```python
import jax
import jax.numpy as jnp

def _softmax(x, axis=-1):
    return jax.nn.softmax(x, axis=axis)

def _gelu(x):
    return jax.nn.gelu(x, approximate=True)

def _silu(x):
    return jax.nn.silu(x)

def _sigmoid(x):
    return jax.nn.sigmoid(x)

def _layernorm(x, axis=-1, eps=1e-05):
    m = jnp.mean(x, axis=axis, keepdims=True)
    v = jnp.var(x, axis=axis, keepdims=True)
    return (x - m) / jnp.sqrt(v + eps)

def _scatter_add(tgt, idx, src, axis=0):
    return tgt.at[idx].add(src)

def _segment_sum(src, seg, n):
    return jax.ops.segment_sum(src, seg, n)

class _Rng:

    def __init__(self, key):
        self._k = key

    def _next(self):
        self._k, sub = jax.random.split(self._k)
        return sub

    def normal(self, shape):
        return jax.random.normal(self._next(), shape, dtype=jnp.bfloat16)

    def randint(self, lo, hi, shape):
        return jax.random.randint(self._next(), shape, lo, hi, dtype=jnp.int32)

    def uniform(self, shape, lo=0.0, hi=1.0):
        return jax.random.uniform(self._next(), shape, jnp.bfloat16, lo, hi)

    def permutation(self, n):
        return jax.random.permutation(self._next(), n)
kernel_name = 'adaLN_cond__spectral_gfnet__mixer_token_mlp__prompt'

def setup_inputs():
    _rng = _Rng(jax.random.key(int.from_bytes(__import__("os").urandom(4), "little")))
    _w = lambda a: (lambda t: t.astype(jnp.bfloat16) if jnp.issubdtype(t.dtype, jnp.floating) else t)(jnp.asarray(a))

    def _A_setup():
        B, S, D = (1, 2048, 576)
        Df = D // 2 + 1
        return {'x': _w((lambda *s: _rng.normal(s) * 0.05)(B, S, D)), 'w_r': _w((lambda *s: _rng.normal(s) * 0.05)(S, Df) * 0.02), 'w_i': _w((lambda *s: _rng.normal(s) * 0.05)(S, Df) * 0.02)}
    _A_in = _A_setup()

    def _B_setup():
        B, S, D, F = (1, 2048, 576, 4608)
        return {'x': _w((lambda *s: _rng.normal(s) * 0.05)(B, S, D)), 'w1': _w((lambda *s: _rng.normal(s) * 0.05)(S, F) * S ** (-0.5)), 'b1': _w((lambda *s: _rng.normal(s) * 0.05)(F) * 0.02), 'w2': _w((lambda *s: _rng.normal(s) * 0.05)(F, S) * F ** (-0.5)), 'b2': _w((lambda *s: _rng.normal(s) * 0.05)(S) * 0.02)}
    _B_in = _B_setup()
    return {'A_x': _A_in['x'], 'A_w_r': _A_in['w_r'], 'A_w_i': _A_in['w_i'], 'B_x': _B_in['x'], 'B_w1': _B_in['w1'], 'B_b1': _B_in['b1'], 'B_w2': _B_in['w2'], 'B_b2': _B_in['b2'], 'c': _w((lambda *s: _rng.normal(s) * 0.05)(1, 576)), 'w_mod': _w((lambda *s: _rng.normal(s) * 0.05)(576, 6 * 576) * 576 ** (-0.5))}

def reference(A_x, A_w_r, A_w_i, B_x, B_w1, B_b1, B_w2, B_b2, c, w_mod):

    def _A_ref(x, w_r, w_i):
        B, S, D = x.shape
        X = (lambda x, axes=(-2, -1): jnp.fft.rfft2(x.astype(jnp.float32), axes=axes))(x, axes=(-2, -1))
        W = w_r + 1j * w_i
        X = X * W
        y = (lambda x, s, axes=(-2, -1): jnp.fft.irfft2(x, s=s, axes=axes).astype(jnp.bfloat16))(X, (S, D), axes=(-2, -1))
        return y

    def _B_ref(x, w1, b1, w2, b2):
        B, S, D = x.shape
        h = _layernorm(x, axis=-1)
        u = jnp.einsum('bsd,sf->bdf', h, w1) + b1
        u = _gelu(u)
        y = jnp.einsum('bdf,fs->bds', u, w2) + b2
        return (lambda x, *d: x.transpose(*d))(y, 0, 2, 1)
    x = A_x
    mod = (_silu(c) @ w_mod).reshape(c.shape[0], 6, 1, -1)
    sa, ca, ga, sb, cb, gb = (mod[:, 0].copy(), mod[:, 1].copy(), mod[:, 2].copy(), mod[:, 3].copy(), mod[:, 4].copy(), mod[:, 5].copy())
    h = _layernorm(x, axis=-1) * (1 + ca) + sa
    x = x + ga * _A_ref(h, A_w_r, A_w_i)
    h = _layernorm(x, axis=-1) * (1 + cb) + sb
    x = x + gb * _B_ref(h, B_w1, B_b1, B_w2, B_b2)
    return x
```

```python
import numpy as np
import jax
import jax.numpy as jnp
import jax.experimental.pallas as pl
import jax.experimental.pallas.tpu as pltpu

S, D, F = 2048, 576, 4608
DF = D // 2 + 1
NP = 49
MB = D // 4
NCH = F // 512
NRG = (8, 8, 8, 8, 5)
W2_ROWS = F // 2
W1_ROWS = S // 2

f32, u32, bf16 = jnp.float32, jnp.uint32, jnp.bfloat16


def _interleave(a, b):
    n = a.shape[0] // 8
    return np.stack([a.reshape(n, 8, -1), b.reshape(n, 8, -1)], axis=1).reshape(16 * n, -1)


def _constants():
    d0 = np.arange(64)
    fd = np.zeros((5, 128, 128))
    fi = np.zeros((5, 128, 128))
    scale = 1.0 / (S * D)
    for k1 in range(1, 5):
        k = np.array([k1 + 9 * m for m in range(32)] + [9 - k1 + 9 * m for m in range(32)])
        sg = np.array([1.0] * 32 + [-1.0] * 32)[:, None]
        ang = 2 * np.pi * np.outer(k, d0) / D
        c, s = np.cos(ang), np.sin(ang)
        q = np.sqrt(3.0) / 2 if k1 == 3 else 1.0
        re = _interleave(c.T, (-q * sg * s).T).T
        im = _interleave(-s.T, (-q * sg * c).T).T
        fd[k1 - 1] = _interleave(re, im)
        fi[k1 - 1] = 2 * scale * fd[k1 - 1].T
    ang = 2 * np.pi * np.outer(9 * np.arange(33), d0) / D
    re, im = np.zeros((40, 64)), np.zeros((40, 64))
    re[:33], im[:33] = np.cos(ang), -np.sin(ang)
    im[0] = im[32] = 0.0
    w = np.full((40, 1), 2.0)
    w[0] = w[32] = 1.0
    fd[4, :80, :64] = _interleave(re, im)
    fi[4, :64, :80] = scale * _interleave(w * re, w * im).T
    s0 = np.arange(128)
    gf = np.zeros((16, 2, 128, 128))
    gi = np.zeros((16, 2, 128, 128))
    for j1 in range(16):
        lane = (np.arange(128) - j1) % 128
        ang = 2 * np.pi * np.outer(s0, j1 + 16 * (8 * (lane % 16) + lane // 16)) / S
        gf[j1, 0], gf[j1, 1] = np.cos(ang), -np.sin(ang)
        gi[j1, 0], gi[j1, 1] = np.cos(ang).T, np.sin(ang).T
    to = lambda a: a.astype(np.float32).astype(jnp.bfloat16)
    return to(np.concatenate([fd, fi])), to(np.concatenate([gf, gi]).reshape(64, 128, 128))


_DMAT, _GMAT = _constants()

_C1, _C2, _C4 = (float(np.cos(2 * np.pi * k / 9)) for k in (1, 2, 4))
_S1, _S4, _S3 = float(np.sin(2 * np.pi / 9)), float(np.sin(8 * np.pi / 9)), float(np.sqrt(3.0) / 2)


def _dft9(x):
    e1, e2, e3, e4 = x[1] + x[8], x[2] + x[7], x[3] + x[6], x[4] + x[5]
    o1, o2, o3, o4 = x[1] - x[8], x[2] - x[7], x[3] - x[6], x[4] - x[5]
    t = x[0] - 0.5 * e3
    sm = e1 + e2 + e4
    p = x[0] + e3
    d1, d2 = e1 - e4, e2 - e4
    q1 = _C1 * d1 + _C2 * d2
    q2 = _C2 * d1 + _C4 * d2
    a, b, c = o1 + o2, o2 + o4, o1 - o4
    r1 = _S1 * a + _S4 * b
    r2 = _S1 * c + _S4 * a
    v = _S3 * o3
    return (p + sm, (t + q1, r1 + v), (t + q2, r2 - v), (p - 0.5 * sm, (o1 - o2) + o4),
            ((t - q1) - q2, (r2 - r1) + v))


def _idft9(a0, z1, z2, z3, z4):
    (a1, b1), (a2, b2), (a3, b3), (a4, b4) = z1, z2, z3, z4
    o3 = _S3 * ((b1 - b2) + b4)
    r1, r2 = b1 - b4, b2 + b4
    a, b, c = _S1 * r1 + _S4 * r2, _S4 * r1, _S1 * r2
    o1, o2, o4 = (a + c) + b3, (a + b) - b3, (b - c) + b3
    t = (a1 + a2) + a4
    q1, q2 = a1 - a4, a2 - a4
    d1 = _C1 * q1 + _C2 * q2
    d2 = _C2 * q1 + _C4 * q2
    p, sm = a0 + a3, a0 - 0.5 * a3
    e1, e2, e4 = sm + d1, sm + d2, (sm - d1) - d2
    e3 = p - 0.5 * t
    return [t + p, e1 + o1, e2 + o2, e3 + o3, e4 + o4, e4 - o4, e3 - o3, e2 - o2, e1 - o1]


def _radix4(x, sign):
    t0 = (x[0][0] + x[2][0], x[0][1] + x[2][1])
    t1 = (x[0][0] - x[2][0], x[0][1] - x[2][1])
    t2 = (x[1][0] + x[3][0], x[1][1] + x[3][1])
    t3 = (x[1][0] - x[3][0], x[1][1] - x[3][1])
    plus = (t1[0] - t3[1], t1[1] + t3[0])
    minus = (t1[0] + t3[1], t1[1] - t3[0])
    y1, y3 = (plus, minus) if sign > 0 else (minus, plus)
    return [(t0[0] + t2[0], t0[1] + t2[1]), y1, (t0[0] - t2[0], t0[1] - t2[1]), y3]


def _twiddle(z, n, sign):
    re, im = z
    if n == 0:
        return z
    if n == 4:
        return (-im, re) if sign > 0 else (im, -re)
    c, s = float(np.cos(np.pi * n / 8)), sign * float(np.sin(np.pi * n / 8))
    if n in (2, 6):
        if c * s > 0:
            return (c * (re - im), c * (im + re))
        return (c * (re + im), c * (im - re))
    return (c * re - s * im, c * im + s * re)


_A_TERMS = (((0, 0), 1, (1, 1)), ((1, 0), 1, (1, 1)), ((0, 0), 0, None), ((1, 1), 0, None),
            ((0, 0), 1, (0, 1)), ((1, 0), -1, (0, 0)), ((0, 1), -1, (1, 1)))
_B_TERMS = (((0, 0), 1, (1, 1)), ((0, 0), 0, None), ((0, 1), -1, (1, 1)), ((1, 0), -1, (0, 0)),
            ((1, 1), 0, None), ((0, 0), 1, (0, 1)), ((1, 0), 1, (1, 1)))


def _add2(x, y):
    return [[x[i][j] + y[i][j] for j in range(2)] for i in range(2)]


def _sub2(x, y):
    return [[x[i][j] - y[i][j] for j in range(2)] for i in range(2)]


def _outer_operand(ld, term):
    a, s, b = term
    x = [[ld(2 * a[0] + i, 2 * a[1] + j) for j in range(2)] for i in range(2)]
    if s == 0:
        return x
    y = [[ld(2 * b[0] + i, 2 * b[1] + j) for j in range(2)] for i in range(2)]
    return _add2(x, y) if s > 0 else _sub2(x, y)


def _inner_operand(x, term):
    a, s, b = term
    if s == 0:
        return x[a[0]][a[1]]
    return x[a[0]][a[1]] + x[b[0]][b[1]] if s > 0 else x[a[0]][a[1]] - x[b[0]][b[1]]


def _inner_result(m):
    m1, m4, m2 = m(0), m(3), m(1)
    c21, c22, c11 = m2 + m4, m1 - m2, m1 + m4
    m5, m3 = m(4), m(2)
    c12, c11, c22 = m3 + m5, c11 - m5, c22 + m3
    return [[c11 + m(6), c12], [c21, c22 + m(5)]]


def _recombine(load, bias, finish, tag):
    def inner(p1, col=None):
        def m(p2):
            v = load(7 * p1 + p2)
            if col is not None and p2 in (3, 2):
                v = v + bias(2 * col + (0 if p2 == 3 else 1))
            return v
        return _inner_result(m)

    def done(c, bi, bj):
        for i in range(2):
            for j in range(2):
                finish(2 * bi + i, 2 * bj + j, c[i][j])

    yield tag
    m2 = inner(1)
    yield tag
    m4 = inner(3, col=0)
    done(_add2(m2, m4), 1, 0)
    yield tag
    m1 = inner(0)
    c22, c11 = _sub2(m1, m2), _add2(m1, m4)
    yield tag
    m5 = inner(4)
    c11 = _sub2(c11, m5)
    yield tag
    m3 = inner(2, col=1)
    c22 = _add2(c22, m3)
    done(_add2(m3, m5), 0, 1)
    yield tag
    done(_add2(c11, inner(6)), 0, 0)
    yield tag
    done(_add2(c22, inner(5)), 1, 1)


def _gelu2(x):
    c0 = float(np.sqrt(2.0 / np.pi))
    return x + x * jnp.tanh(x * (c0 + (c0 * 0.044715) * (x * x)))


def _merge(*streams):
    units = []
    for k, us in enumerate(streams):
        units += [((i + 0.5) / len(us), k, u) for i, u in enumerate(us)]
    units.sort(key=lambda t: t[:2])

    def chain():
        for u in units:
            yield from u[2][1]

    return sum(u[2][0] for u in units), chain()


def _pack(a, b):
    return jnp.concatenate([a, b], axis=0).astype(bf16)


def _colsum(v):
    return jnp.broadcast_to(jnp.sum(v, axis=0, keepdims=True), v.shape)


def _kernel(x_hbm, wr_hbm, wi_hbm, w1_hbm, b1_ref, w2_hbm, b2_ref, c_ref, wmod_hbm, dmat_hbm, gmat_hbm,
            out_hbm,
            zero_s, w2_v, uc_v, bc0, bc1, mm0, mm1, uu_v, x2_v, mod_v, io_v, sem_w2, sem_out):
    zero_s[0] = 0
    zero = zero_s[0]

    def tick(ref, row, val):
        ref[pl.ds(pl.multiple_of(row + zero, 8), 8), :] = val

    def as_bf16(v):
        return pltpu.bitcast(v, bf16)

    w2_copies = [pltpu.make_async_copy(w2_hbm.bitcast(u32).at[:, pl.ds(128 * t, 128)],
                                       w2_v.at[pl.ds(t * W2_ROWS, W2_ROWS)], sem_w2.at[t])
                 for t in range(16)]

    def weight_unit(src, row_of, ru, bc):
        raw = lambda k, j: src[pl.ds(row_of(k, j, ru), 8), :]
        ld = lambda k, j: as_bf16(raw(k, j)).astype(f32)
        for p1, t1 in enumerate(_B_TERMS):
            yield "w"
            x = _outer_operand(ld, t1)
            for p2, t2 in enumerate(_B_TERMS):
                if t1[1] == 0 and t2[1] == 0:
                    bc.bitcast(u32)[7 * p1 + p2, pl.ds(8 * ru, 8), :] = raw(
                        2 * t1[0][0] + t2[0][0], 2 * t1[0][1] + t2[0][1])
                else:
                    bc[7 * p1 + p2, pl.ds(16 * ru, 16), :] = _inner_operand(x, t2).astype(bf16)

    def weight_units(src, row_of, bc):
        return [(7, weight_unit(src, row_of, ru, bc)) for ru in range(32)]

    def lhs_unit(src, dst, slot, r, tag):
        ld = lambda i, j: src[pl.ds((4 * i + j) * MB + 16 * r, 16), :]
        for p1, t1 in enumerate(_A_TERMS):
            yield tag
            x = _outer_operand(ld, t1)
            for p2, t2 in enumerate(_A_TERMS):
                dst[slot(7 * p1 + p2), pl.ds(16 * r, 16), :] = _inner_operand(x, t2).astype(bf16)

    def hidden_units(mm, c):
        def first(r8):
            def finish(i, j, v):
                uu_v[pl.ds((4 * i + j) * MB + 8 * r8, 8), :] = _gelu2(v)
            return _recombine(lambda p: mm[pl.ds(p * MB + 8 * r8, 8), :],
                              lambda j: mod_v[pl.ds(pl.multiple_of(6 * D + 8 * (4 * c + j), 8), 8), :],
                              finish, "o")
        units = []
        for r in range(MB // 16):
            units += [(7, first(2 * r)), (7, first(2 * r + 1)),
                      (7, lhs_unit(uu_v, uc_v, lambda p: p * NCH + c, r, "u"))]
        return units

    def output_units(mm, n):
        def unit(r8):
            def finish(i, j, v):
                row = i * MB + 8 * r8
                res = x2_v[pl.ds(pl.multiple_of((4 * n + j) * D + row, 8), 8), :]
                io_v[4 * n + j, pl.ds(row, 8), :] = (res + mod_v[pl.ds(5 * D + row, 8), :] * v).astype(bf16)
            return _recombine(lambda p: mm[pl.ds(p * MB + 8 * r8, 8), :],
                              lambda j: mod_v[pl.ds(pl.multiple_of(6 * D + 8 * (36 + 4 * n + j), 8), 8), :],
                              finish, "o")
        return [(7, unit(r8)) for r8 in range(MB // 8)]

    def step(product, side, w_src, w_row, o_src):
        total, gen = side
        pending, done = next(gen, None), 0
        for _ in range(3):
            if pending is not None:
                pending, done = next(gen, None), done + 1
        points = NP * (MB // 16) - 12
        pt = 0
        for p in range(NP):
            for v in product(p):
                pt += 1
                seen = set()
                while pending is not None and done * points < pt * total:
                    if pending not in seen:
                        seen.add(pending)
                        if pending == "w":
                            tick(w_src, w_row, pltpu.bitcast(v, u32))
                        elif pending == "o":
                            tick(o_src, NP * MB, v)
                        else:
                            tick(uu_v, 16 * MB, v)
                    pending, done = next(gen, None), done + 1
        assert pending is None

    def deep_product(lhs_ref, slot, bc, dst, init=None):
        lhs_u, bc_u = lhs_ref.bitcast(u32), bc.bitcast(u32)

        def product(p):
            lhs = jnp.concatenate([as_bf16(lhs_u[slot(p, t)]) for t in range(4)], axis=1)
            v = jnp.dot(lhs, as_bf16(bc_u[p]), preferred_element_type=f32)
            for r in range(MB // 16):
                blk = v[16 * r:16 * r + 16]
                if init is not None:
                    blk = blk + init(p, r)
                dst[pl.ds(p * MB + 16 * r, 16), :] = blk
                yield blk[:8]
        return product

    w1_row = lambda c: (lambda k, j, ru: pl.multiple_of((4 * c + j) * W1_ROWS + 256 * k + 8 * ru, 8))
    w2_row_wide = lambda k, j, ru: (4 * (ru // 8) + j) * W2_ROWS + 64 * k + 8 * (ru % 8)
    w2_row = lambda n, h: (lambda k, j, ru: pl.multiple_of(
        (4 * n + j) * W2_ROWS + 256 * (1 + 4 * h + ru // 8) + 64 * k + 8 * (ru % 8), 8))

    def first_half(w1_v, ac_v, wmod_v, dmat_v, gmat_v, wf_v, wt_v, ha_v, ra_v, uv_v, tl_v,
                   zl_v, pp_v, qq_v, sem, sem_x, sem_w1):
        x_copies = [pltpu.make_async_copy(x_hbm.at[:, pl.ds(128 * t, 128)], io_v.at[t], sem_x.at[t])
                    for t in range(16)]
        wmod_copies = [pltpu.make_async_copy(wmod_hbm.at[:, pl.ds(1152 * h, 1152 * (h + 1))],
                                             wmod_v.at[:, pl.ds(1152 * h, 1152 * (h + 1))], sem.at[h])
                       for h in range(2)]
        dmat_copy = pltpu.make_async_copy(dmat_hbm, dmat_v, sem.at[2])
        gmat_copy = pltpu.make_async_copy(gmat_hbm, gmat_v, sem.at[3])
        wf_copies = [pltpu.make_async_copy(src, wf_v.at[a], sem.at[4 + a])
                     for a, src in enumerate((wr_hbm, wi_hbm))]
        w1_copies = [pltpu.make_async_copy(w1_hbm.bitcast(u32).at[:, pl.ds(128 * t, 128)],
                                           w1_v.at[pl.ds(t * W1_ROWS, W1_ROWS)], sem_w1.at[t])
                     for t in range(36)]

        wmod_copies[0].start()
        for a in range(4):
            for b in range(4):
                x_copies[a + 4 * b].start()
            if a == 0:
                dmat_copy.start()

        cv = c_ref[...].astype(f32)
        sc = jnp.broadcast_to(cv * jax.nn.sigmoid(cv), (16, D)).astype(bf16)
        b1 = b1_ref[...].astype(f32).reshape(1, F)
        for t in range(36):
            mod_v[pl.ds(6 * D + 8 * t, 8), :] = jnp.broadcast_to(b1[:, 128 * t:128 * t + 128], (8, 128))
        b2 = 2.0 * b2_ref[...].astype(f32).reshape(1, S)
        for t in range(16):
            mod_v[pl.ds(6 * D + 8 * (36 + t), 8), :] = jnp.broadcast_to(b2[:, 128 * t:128 * t + 128], (8, 128))

        def modulation(t0, t1):
            m = jnp.dot(sc, wmod_v[:, pl.ds(128 * t0, 128 * (t1 - t0))], preferred_element_type=f32)[:8]
            for t in range(t0, t1):
                col = 128 * t + jax.lax.broadcasted_iota(jnp.int32, (8, 128), 1)
                v = m[:, 128 * (t - t0):128 * (t - t0 + 1)]
                scale = ((col >= D) & (col < 2 * D)) | ((col >= 4 * D) & (col < 5 * D))
                v = jnp.where(scale, 1.0 + v, v)
                v = jnp.where(col >= 5 * D, 0.5 * v, v)
                mod_v[pl.ds(128 * t, 128), :] = jnp.concatenate([v] * 16, axis=0).T

        wmod_copies[0].wait()
        modulation(0, 9)
        dmat_copy.wait()
        dmat_u, io_u = dmat_v.bitcast(u32), io_v.bitcast(u32)

        for a in range(4):
            for b in range(4):
                x_copies[a + 4 * b].wait()
            if a == 1:
                for cp in wf_copies:
                    cp.start()
                gmat_copy.start()
            if a == 3:
                wmod_copies[1].start()
                for cp in w1_copies[:8]:
                    cp.start()
            for b in range(4):
                t = a + 4 * b
                xf = as_bf16(io_u[t]).astype(f32)
                ha_v[pl.ds(b * D, D), :] = xf
                acc = xf[0:8]
                for r in range(1, D // 8):
                    acc = acc + xf[8 * r:8 * r + 8]
                mean = _colsum(acc) * (1.0 / D)
                acc = None
                for r in range(D // 8):
                    d = ha_v[pl.ds(b * D + 8 * r, 8), :] - mean
                    acc = d * d if acc is None else acc + d * d
                rstd = 1.0 / jnp.sqrt(_colsum(acc) * (1.0 / D) + 1e-5)
                held = None
                for r in range(8):
                    h = []
                    for i in range(9):
                        row = 64 * i + 8 * r
                        xn = (ha_v[pl.ds(b * D + row, 8), :] - mean) * rstd
                        h.append(xn * mod_v[pl.ds(D + row, 8), :] + mod_v[pl.ds(row, 8), :])
                    z = _dft9(h)
                    for g in range(4):
                        ra_v[5 * b + g, pl.ds(16 * r, 16), :] = _pack(*z[g + 1])
                    if r % 2 == 0:
                        held = z[0]
                    else:
                        ra_v[5 * b + 4, pl.ds(8 * (r - 1), 16), :] = _pack(held, z[0])
            ra_u = ra_v.bitcast(u32)
            for g in range(5):
                if g < 4:
                    lhs = as_bf16(dmat_u[g])
                    rhs = jnp.concatenate([as_bf16(ra_u[5 * b + g]) for b in range(4)], axis=1)
                else:
                    lhs = as_bf16(dmat_u[4, pl.ds(0, 40), pl.ds(0, 64)])
                    rhs = jnp.concatenate([as_bf16(ra_u[5 * b + 4, pl.ds(0, 32), :]) for b in range(4)], axis=1)
                v = jnp.dot(lhs, rhs, preferred_element_type=f32)
                for r in range(NRG[g]):
                    z = [(v[16 * r:16 * r + 8, 128 * b:128 * b + 128], v[16 * r + 8:16 * r + 16, 128 * b:128 * b + 128])
                         for b in range(4)]
                    for c, y in enumerate(_radix4(z, -1)):
                        y = _twiddle(y, a * c, -1)
                        uv_v[4 * c + a, pl.ds(128 * g + 16 * r, 8), :] = y[0]
                        uv_v[4 * c + a, pl.ds(128 * g + 16 * r + 8, 8), :] = y[1]

        for cp in wf_copies:
            cp.wait()
        lane = jax.lax.broadcasted_iota(jnp.int32, (8, 128), 1)
        masks = [(lane & (1 << i)) != 0 for i in range(4)]

        def regroup(tiles):
            t = [pltpu.roll(v, b, 1) if b else v for b, v in enumerate(tiles)]
            t = [t[-i % 16] for i in range(16)]
            for i in range(4):
                t = [jnp.where(masks[i], t[(j - (1 << i)) % 16], t[j]) for j in range(16)]
            return t

        for a in range(2):
            for r in range(18):
                tiles = [pltpu.bitcast(wf_v[a, pl.ds(16 * r, 16), pl.ds(128 * b, 128)], u32) for b in range(16)]
                for j1, v in enumerate(regroup(tiles)):
                    wt_v[16 * a + j1, pl.ds(16 * r, 16), :] = as_bf16(v).astype(f32)
            last = jnp.broadcast_to(wf_v[a, pl.ds(288, 1), :].astype(f32), (8, S))
            for j1, v in enumerate(regroup([last[:, 128 * b:128 * b + 128] for b in range(16)])):
                wt_v[16 * a + j1, pl.ds(288, 8), :] = v
        gmat_copy.wait()
        for cp in w1_copies[8:]:
            cp.start()
        for cp in w2_copies:
            cp.start()
        gmat_u = gmat_v.bitcast(u32)

        def filt(a, j1, g, r):
            if g < 4:
                first = (g + 1 if r < 4 else 8 - g) + 72 * (r % 4)
                return wt_v[16 * a + j1, pl.ds(first, 8, stride=9), :]
            if r < 4:
                return wt_v[16 * a + j1, pl.ds(72 * r, 8, stride=9), :]
            return wt_v[16 * a + j1, pl.ds(288, 8), :]

        def cmul(v, r):
            top, bot = v[16 * r:16 * r + 8], v[16 * r + 8:16 * r + 16]
            return top[:, :128] - bot[:, 128:], top[:, 128:] + bot[:, :128]

        tl_u, zl_u, qq_u = tl_v.bitcast(u32), zl_v.bitcast(u32), qq_v.bitcast(u32)
        for g in range(5):
            n = NRG[g]
            o = 16 * (g % 2)
            for r in range(n):
                row = 128 * g + 16 * r
                for c in range(4):
                    z = [(uv_v[4 * c + a, pl.ds(row, 8), :], uv_v[4 * c + a, pl.ds(row + 8, 8), :]) for a in range(4)]
                    for e, y in enumerate(_radix4(z, -1)):
                        tl_v[o + c + 4 * e, pl.ds(16 * r, 16), :] = _pack(*y)
            for j1 in range(16):
                rhs = jnp.concatenate([as_bf16(gmat_u[2 * j1 + i]) for i in range(2)], axis=1)
                v = jnp.dot(as_bf16(tl_u[o + j1, pl.ds(0, 8 * n), :]), rhs, preferred_element_type=f32)
                for r in range(n):
                    yr, yi = cmul(v, r)
                    wr, wi = filt(0, j1, g, r), filt(1, j1, g, r)
                    zl_v[o + j1, pl.ds(16 * r, 16), :] = _pack(yr * wr - yi * wi, yr * wi + yi * wr)
            for j1 in range(16):
                rhs = jnp.concatenate([as_bf16(gmat_u[32 + 2 * j1 + i]) for i in range(2)], axis=1)
                v = jnp.dot(as_bf16(zl_u[o + j1, pl.ds(0, 8 * n), :]), rhs, preferred_element_type=f32)
                for r in range(n):
                    yr, yi = cmul(v, r)
                    pp_v[o + j1, pl.ds(16 * r, 8), :] = yr
                    pp_v[o + j1, pl.ds(16 * r + 8, 8), :] = yi
            for r in range(n):
                mid = [[None] * 4 for _ in range(4)]
                for c in range(4):
                    z = [(pp_v[o + c + 4 * e, pl.ds(16 * r, 8), :], pp_v[o + c + 4 * e, pl.ds(16 * r + 8, 8), :])
                         for e in range(4)]
                    for a, y in enumerate(_radix4(z, 1)):
                        mid[a][c] = _twiddle(y, a * c, 1)
                for a in range(4):
                    for b, y in enumerate(_radix4(mid[a], 1)):
                        qq_v[o + a + 4 * b, pl.ds(16 * r, 16), :] = _pack(*y)
            for a in range(4):
                if g < 4:
                    lhs = as_bf16(dmat_u[5 + g])
                else:
                    lhs = as_bf16(dmat_u[9, pl.ds(0, 32), pl.ds(0, 80)])
                rhs = jnp.concatenate([as_bf16(qq_u[o + a + 4 * b, pl.ds(0, 8 * n), :]) for b in range(4)], axis=1)
                v = jnp.dot(lhs, rhs, preferred_element_type=f32)
                for b in range(4):
                    uv_v[a + 4 * b, pl.ds(128 * g, v.shape[0]), :] = v[:, 128 * b:128 * b + 128]

        wmod_copies[1].wait()
        modulation(9, 27)
        for cp in w1_copies[:8]:
            cp.wait()
        for _ in _merge(weight_units(w1_v, w1_row(0), bc0))[1]:
            pass

        for a in range(4):
            for b in range(4):
                t = a + 4 * b
                acc = None
                for r2 in range(4):
                    xres = [as_bf16(io_u[t, pl.ds(32 * i + 8 * r2, 8), :]).astype(f32) for i in range(9)]
                    for hh in range(2):
                        r = 2 * r2 + hh
                        z = [(uv_v[t, pl.ds(128 * g + 16 * r, 8), :], uv_v[t, pl.ds(128 * g + 16 * r + 8, 8), :])
                             for g in range(4)]
                        y = _idft9(uv_v[t, pl.ds(512 + 8 * r, 8), :], *z)
                        for i in range(9):
                            row = 64 * i + 8 * r
                            x2 = xres[i][8 * hh:8 * hh + 8] + mod_v[pl.ds(2 * D + row, 8), :] * y[i]
                            x2_v[pl.ds(t * D + row, 8), :] = x2
                            acc = x2 if acc is None else acc + x2
                mean = _colsum(acc) * (1.0 / D)
                acc = None
                for r in range(D // 8):
                    d = x2_v[pl.ds(t * D + 8 * r, 8), :] - mean
                    acc = d * d if acc is None else acc + d * d
                rstd = 1.0 / jnp.sqrt(_colsum(acc) * (1.0 / D) + 1e-5)
                acc = None
                for r in range(D // 8):
                    xn = (x2_v[pl.ds(t * D + 8 * r, 8), :] - mean) * rstd
                    h = xn * mod_v[pl.ds(4 * D + 8 * r, 8), :] + mod_v[pl.ds(3 * D + 8 * r, 8), :]
                    ha_v[pl.ds(b * D + 8 * r, 8), :] = h
                    acc = h if acc is None else acc + h
                mean = _colsum(acc) * (1.0 / D)
                acc = None
                for r in range(D // 8):
                    d = ha_v[pl.ds(b * D + 8 * r, 8), :] - mean
                    acc = d * d if acc is None else acc + d * d
                rstd = 1.0 / jnp.sqrt(_colsum(acc) * (1.0 / D) + 1e-5)
                for r in range(D // 8):
                    i, rr = divmod(8 * r, MB)
                    uu_v[pl.ds((4 * i + b) * MB + rr, 8), :] = (ha_v[pl.ds(b * D + 8 * r, 8), :] - mean) * rstd
            for r in range(MB // 16):
                for _ in lhs_unit(uu_v, ac_v, lambda p: 4 * p + a, r, "u"):
                    pass

        for cp in w1_copies[8:]:
            cp.wait()
        w1_tick = 36 * W1_ROWS
        slot = lambda p, t: 4 * p + t

        def mm1_step(c, odd, w_units, with_hidden=True):
            bc, mm, prev = (bc1, mm1, mm0) if odd else (bc0, mm0, mm1)
            w_src, w_tick, units = w_units
            streams = [units] + ([hidden_units(prev, c - 1)] if with_hidden else [])
            step(deep_product(ac_v, slot, bc, mm), _merge(*streams), w_src, w_tick, prev)

        next_w1 = lambda c, bc: (w1_v, w1_tick, weight_units(w1_v, w1_row(c), bc))
        mm1_step(0, False, next_w1(1, bc1), with_hidden=False)

        def pair(i, carry):
            mm1_step(2 * i + 1, True, next_w1(2 * i + 2, bc0))
            mm1_step(2 * i + 2, False, next_w1(2 * i + 3, bc1))
            return carry

        jax.lax.fori_loop(0, 3, pair, 0)
        for cp in w2_copies:
            cp.wait()
        mm1_step(7, True, next_w1(8, bc0))
        mm1_step(8, False, (w2_v, 16 * W2_ROWS, weight_units(w2_v, w2_row_wide, bc1)))

    pl.run_scoped(
        first_half,
        pltpu.VMEM((36 * W1_ROWS + 8, 128), u32),
        pltpu.VMEM((4 * NP, MB, 128), bf16),
        pltpu.VMEM((D, 6 * D), bf16),
        pltpu.VMEM((10, 128, 128), bf16),
        pltpu.VMEM((64, 128, 128), bf16),
        pltpu.VMEM((2, DF, S), bf16),
        pltpu.VMEM((32, 296, 128), f32),
        pltpu.VMEM((4 * D, 128), f32),
        pltpu.VMEM((20, 128, 128), bf16),
        pltpu.VMEM((16, 592, 128), f32),
        pltpu.VMEM((32, 128, 128), bf16),
        pltpu.VMEM((32, 128, 128), bf16),
        pltpu.VMEM((32, 128, 128), f32),
        pltpu.VMEM((32, 128, 128), bf16),
        pltpu.SemaphoreType.DMA((6,)),
        pltpu.SemaphoreType.DMA((16,)),
        pltpu.SemaphoreType.DMA((36,)),
    )

    def second_half(acc_v):
        w2_tick = 16 * W2_ROWS
        uc_u = uc_v.bitcast(u32)

        def wide_product(p):
            rhs = jnp.concatenate([as_bf16(bc1.bitcast(u32)[p, pl.ds(64 * n, 64), :]) for n in range(4)], axis=1)
            v = jnp.dot(as_bf16(uc_u[p * NCH]), rhs, preferred_element_type=f32)
            for r in range(MB // 16):
                for n in range(4):
                    acc_v[pl.ds((n * NP + p) * MB + 16 * r, 16), :] = v[16 * r:16 * r + 16, 128 * n:128 * n + 128]
                yield v[16 * r:16 * r + 8, :128]

        step(wide_product, _merge(weight_units(w2_v, w2_row(0, 0), bc0), hidden_units(mm0, NCH - 1)),
             w2_v, w2_tick, mm0)

        def out_copies(n):
            return [pltpu.make_async_copy(io_v.at[4 * n + j],
                                          out_hbm.at[:, pl.ds(pl.multiple_of(128 * (4 * n + j), 128), 128)],
                                          sem_out.at[4 * n + j]) for j in range(4)]

        def half0(n, with_output):
            init = lambda p, r: acc_v[pl.ds(pl.multiple_of((n * NP + p) * MB + 16 * r, 8), 16), :]
            streams = [weight_units(w2_v, w2_row(n, 1), bc1)] + ([output_units(mm1, n - 1)] if with_output else [])
            step(deep_product(uc_v, lambda p, t: p * NCH + 1 + t, bc0, mm0, init), _merge(*streams),
                 w2_v, w2_tick, mm1)

        def half1(n, with_weights):
            init = lambda p, r: mm0[pl.ds(p * MB + 16 * r, 16), :]
            streams = [weight_units(w2_v, w2_row(n + 1, 0), bc0)] if with_weights else []
            step(deep_product(uc_v, lambda p, t: p * NCH + 5 + t, bc1, mm1, init), _merge(*streams),
                 w2_v, w2_tick, mm1)

        half0(0, False)

        def pair(n, carry):
            half1(n, True)
            half0(n + 1, True)
            for cp in out_copies(n):
                cp.start()
            return carry

        jax.lax.fori_loop(0, 3, pair, 0)
        half1(3, False)
        for _ in _merge(output_units(mm1, 3))[1]:
            pass
        for cp in out_copies(3):
            cp.start()
        for n in range(4):
            for cp in out_copies(n):
                cp.wait()

    pl.run_scoped(second_half, pltpu.VMEM((4 * NP * MB, 128), f32))


@jax.jit
def pallas_adaLN_cond__spectral_gfnet__mixer_token_mlp__prompt_kernel(
    A_x: jax.Array,
    A_w_r: jax.Array,
    A_w_i: jax.Array,
    B_x: jax.Array,
    B_w1: jax.Array,
    B_b1: jax.Array,
    B_w2: jax.Array,
    B_b2: jax.Array,
    c: jax.Array,
    w_mod: jax.Array,
):
    del B_x
    hbm = pl.BlockSpec(memory_space=pl.ANY)
    vmem = pl.BlockSpec(memory_space=pltpu.VMEM)
    out = pl.pallas_call(
        _kernel,
        out_shape=jax.ShapeDtypeStruct((D, S), bf16),
        in_specs=[hbm, hbm, hbm, hbm, vmem, hbm, vmem, vmem, hbm, hbm, hbm],
        out_specs=hbm,
        scratch_shapes=[
            pltpu.SMEM((1,), jnp.int32),
            pltpu.VMEM((16 * W2_ROWS + 8, 128), u32),
            pltpu.VMEM((NP * NCH, MB, 128), bf16),
            pltpu.VMEM((NP, 512, 128), bf16),
            pltpu.VMEM((NP, 512, 128), bf16),
            pltpu.VMEM((NP * MB + 8, 128), f32),
            pltpu.VMEM((NP * MB + 8, 128), f32),
            pltpu.VMEM((16 * MB + 8, 128), f32),
            pltpu.VMEM((16 * D, 128), f32),
            pltpu.VMEM((6 * D + 8 * 52, 128), f32),
            pltpu.VMEM((16, D, 128), bf16),
            pltpu.SemaphoreType.DMA((16,)),
            pltpu.SemaphoreType.DMA((16,)),
        ],
        compiler_params=pltpu.CompilerParams(vmem_limit_bytes=126 * 1024 * 1024),
        name="adaln_gfnet_mixer",
    )(A_x.reshape(S, D).T, A_w_r.T, A_w_i.T, B_w1, B_b1, B_w2, B_b2, c, w_mod, _DMAT, _GMAT)
    return out.T.reshape(1, S, D)
```

```python
import numpy as np
import jax
import jax.numpy as jnp
import jax.experimental.pallas as pl
import jax.experimental.pallas.tpu as pltpu

S, D, F = 2048, 576, 4608
DF = D // 2 + 1
NP = 49
MB = D // 4
NCH = F // 512
NRG = (8, 8, 8, 8, 5)
W2_ROWS = F // 2
W1_ROWS = S // 2

f32, u32, bf16 = jnp.float32, jnp.uint32, jnp.bfloat16


def _interleave(a, b):
    n = a.shape[0] // 8
    return np.stack([a.reshape(n, 8, -1), b.reshape(n, 8, -1)], axis=1).reshape(16 * n, -1)


def _constants():
    d0 = np.arange(64)
    fd = np.zeros((5, 128, 128))
    fi = np.zeros((5, 128, 128))
    scale = 1.0 / (S * D)
    for k1 in range(1, 5):
        k = np.array([k1 + 9 * m for m in range(32)] + [9 - k1 + 9 * m for m in range(32)])
        sg = np.array([1.0] * 32 + [-1.0] * 32)[:, None]
        ang = 2 * np.pi * np.outer(k, d0) / D
        c, s = np.cos(ang), np.sin(ang)
        q = np.sqrt(3.0) / 2 if k1 == 3 else 1.0
        re = _interleave(c.T, (-q * sg * s).T).T
        im = _interleave(-s.T, (-q * sg * c).T).T
        fd[k1 - 1] = _interleave(re, im)
        fi[k1 - 1] = 2 * scale * fd[k1 - 1].T
    ang = 2 * np.pi * np.outer(9 * np.arange(33), d0) / D
    re, im = np.zeros((40, 64)), np.zeros((40, 64))
    re[:33], im[:33] = np.cos(ang), -np.sin(ang)
    im[0] = im[32] = 0.0
    w = np.full((40, 1), 2.0)
    w[0] = w[32] = 1.0
    fd[4, :80, :64] = _interleave(re, im)
    fi[4, :64, :80] = scale * _interleave(w * re, w * im).T
    s0 = np.arange(128)
    gf = np.zeros((16, 2, 128, 128))
    gi = np.zeros((16, 2, 128, 128))
    for j1 in range(16):
        lane = (np.arange(128) - j1) % 128
        ang = 2 * np.pi * np.outer(s0, j1 + 16 * (8 * (lane % 16) + lane // 16)) / S
        gf[j1, 0], gf[j1, 1] = np.cos(ang), -np.sin(ang)
        gi[j1, 0], gi[j1, 1] = np.cos(ang).T, np.sin(ang).T
    to = lambda a: a.astype(np.float32).astype(jnp.bfloat16)
    return to(np.concatenate([fd, fi])), to(np.concatenate([gf, gi]).reshape(64, 128, 128))


_DMAT, _GMAT = _constants()

_C1, _C2, _C4 = (float(np.cos(2 * np.pi * k / 9)) for k in (1, 2, 4))
_S1, _S4, _S3 = float(np.sin(2 * np.pi / 9)), float(np.sin(8 * np.pi / 9)), float(np.sqrt(3.0) / 2)


def _dft9(x):
    e1, e2, e3, e4 = x[1] + x[8], x[2] + x[7], x[3] + x[6], x[4] + x[5]
    o1, o2, o3, o4 = x[1] - x[8], x[2] - x[7], x[3] - x[6], x[4] - x[5]
    t = x[0] - 0.5 * e3
    sm = e1 + e2 + e4
    p = x[0] + e3
    d1, d2 = e1 - e4, e2 - e4
    q1 = _C1 * d1 + _C2 * d2
    q2 = _C2 * d1 + _C4 * d2
    a, b, c = o1 + o2, o2 + o4, o1 - o4
    r1 = _S1 * a + _S4 * b
    r2 = _S1 * c + _S4 * a
    v = _S3 * o3
    return (p + sm, (t + q1, r1 + v), (t + q2, r2 - v), (p - 0.5 * sm, (o1 - o2) + o4),
            ((t - q1) - q2, (r2 - r1) + v))


def _idft9(a0, z1, z2, z3, z4):
    (a1, b1), (a2, b2), (a3, b3), (a4, b4) = z1, z2, z3, z4
    o3 = _S3 * ((b1 - b2) + b4)
    r1, r2 = b1 - b4, b2 + b4
    a, b, c = _S1 * r1 + _S4 * r2, _S4 * r1, _S1 * r2
    o1, o2, o4 = (a + c) + b3, (a + b) - b3, (b - c) + b3
    t = (a1 + a2) + a4
    q1, q2 = a1 - a4, a2 - a4
    d1 = _C1 * q1 + _C2 * q2
    d2 = _C2 * q1 + _C4 * q2
    p, sm = a0 + a3, a0 - 0.5 * a3
    e1, e2, e4 = sm + d1, sm + d2, (sm - d1) - d2
    e3 = p - 0.5 * t
    return [t + p, e1 + o1, e2 + o2, e3 + o3, e4 + o4, e4 - o4, e3 - o3, e2 - o2, e1 - o1]


def _radix4(x, sign):
    t0 = (x[0][0] + x[2][0], x[0][1] + x[2][1])
    t1 = (x[0][0] - x[2][0], x[0][1] - x[2][1])
    t2 = (x[1][0] + x[3][0], x[1][1] + x[3][1])
    t3 = (x[1][0] - x[3][0], x[1][1] - x[3][1])
    plus = (t1[0] - t3[1], t1[1] + t3[0])
    minus = (t1[0] + t3[1], t1[1] - t3[0])
    y1, y3 = (plus, minus) if sign > 0 else (minus, plus)
    return [(t0[0] + t2[0], t0[1] + t2[1]), y1, (t0[0] - t2[0], t0[1] - t2[1]), y3]


def _twiddle(z, n, sign):
    re, im = z
    if n == 0:
        return z
    if n == 4:
        return (-im, re) if sign > 0 else (im, -re)
    c, s = float(np.cos(np.pi * n / 8)), sign * float(np.sin(np.pi * n / 8))
    if n in (2, 6):
        if c * s > 0:
            return (c * (re - im), c * (im + re))
        return (c * (re + im), c * (im - re))
    return (c * re - s * im, c * im + s * re)


_A_TERMS = (((0, 0), 1, (1, 1)), ((1, 0), 1, (1, 1)), ((0, 0), 0, None), ((1, 1), 0, None),
            ((0, 0), 1, (0, 1)), ((1, 0), -1, (0, 0)), ((0, 1), -1, (1, 1)))
_B_TERMS = (((0, 0), 1, (1, 1)), ((0, 0), 0, None), ((0, 1), -1, (1, 1)), ((1, 0), -1, (0, 0)),
            ((1, 1), 0, None), ((0, 0), 1, (0, 1)), ((1, 0), 1, (1, 1)))


def _add2(x, y):
    return [[x[i][j] + y[i][j] for j in range(2)] for i in range(2)]


def _sub2(x, y):
    return [[x[i][j] - y[i][j] for j in range(2)] for i in range(2)]


def _outer_operand(ld, term):
    a, s, b = term
    x = [[ld(2 * a[0] + i, 2 * a[1] + j) for j in range(2)] for i in range(2)]
    if s == 0:
        return x
    y = [[ld(2 * b[0] + i, 2 * b[1] + j) for j in range(2)] for i in range(2)]
    return _add2(x, y) if s > 0 else _sub2(x, y)


def _inner_operand(x, term):
    a, s, b = term
    if s == 0:
        return x[a[0]][a[1]]
    return x[a[0]][a[1]] + x[b[0]][b[1]] if s > 0 else x[a[0]][a[1]] - x[b[0]][b[1]]


def _inner_result(m):
    m1, m4, m2 = m(0), m(3), m(1)
    c21, c22, c11 = m2 + m4, m1 - m2, m1 + m4
    m5, m3 = m(4), m(2)
    c12, c11, c22 = m3 + m5, c11 - m5, c22 + m3
    return [[c11 + m(6), c12], [c21, c22 + m(5)]]


def _recombine(load, bias, finish, tag):
    def inner(p1, col=None):
        def m(p2):
            v = load(7 * p1 + p2)
            if col is not None and p2 in (3, 2):
                v = v + bias(2 * col + (0 if p2 == 3 else 1))
            return v
        return _inner_result(m)

    def done(c, bi, bj):
        for i in range(2):
            for j in range(2):
                finish(2 * bi + i, 2 * bj + j, c[i][j])

    yield tag
    m2 = inner(1)
    yield tag
    m4 = inner(3, col=0)
    done(_add2(m2, m4), 1, 0)
    yield tag
    m1 = inner(0)
    c22, c11 = _sub2(m1, m2), _add2(m1, m4)
    yield tag
    m5 = inner(4)
    c11 = _sub2(c11, m5)
    yield tag
    m3 = inner(2, col=1)
    c22 = _add2(c22, m3)
    done(_add2(m3, m5), 0, 1)
    yield tag
    done(_add2(c11, inner(6)), 0, 0)
    yield tag
    done(_add2(c22, inner(5)), 1, 1)


def _gelu2(x):
    c0 = float(np.sqrt(2.0 / np.pi))
    return x + x * jnp.tanh(x * (c0 + (c0 * 0.044715) * (x * x)))


def _merge(*streams):
    units = []
    for k, us in enumerate(streams):
        units += [((i + 0.5) / len(us), k, u) for i, u in enumerate(us)]
    units.sort(key=lambda t: t[:2])

    def chain():
        for u in units:
            yield from u[2][1]

    return sum(u[2][0] for u in units), chain()


def _pack(a, b):
    return jnp.concatenate([a, b], axis=0).astype(bf16)


def _colsum(v):
    return jnp.broadcast_to(jnp.sum(v, axis=0, keepdims=True), v.shape)


def _kernel(x_hbm, wr_hbm, wi_hbm, w1_hbm, b1_ref, w2_hbm, b2_ref, c_ref, wmod_hbm, dmat_hbm, gmat_hbm,
            zero_s, out_hbm,
            w2_v, uc_v, bc0, bc1, mm0, mm1, uu_v, x2_v, mod_v, io_v, sem_w2, sem_out):
    zero = zero_s[0]

    def tick(ref, row, val):
        ref[pl.ds(pl.multiple_of(row + zero, 8), 8), :] = val

    def as_bf16(v):
        return pltpu.bitcast(v, bf16)

    w2_copies = [pltpu.make_async_copy(w2_hbm.bitcast(u32).at[:, pl.ds(128 * t, 128)],
                                       w2_v.at[pl.ds(t * W2_ROWS, W2_ROWS)], sem_w2.at[t])
                 for t in range(16)]

    def weight_unit(src, row_of, ru, bc):
        raw = lambda k, j: src[pl.ds(row_of(k, j, ru), 8), :]
        ld = lambda k, j: as_bf16(raw(k, j)).astype(f32)
        for p1, t1 in enumerate(_B_TERMS):
            yield "w"
            x = _outer_operand(ld, t1)
            for p2, t2 in enumerate(_B_TERMS):
                if t1[1] == 0 and t2[1] == 0:
                    bc.bitcast(u32)[7 * p1 + p2, pl.ds(8 * ru, 8), :] = raw(
                        2 * t1[0][0] + t2[0][0], 2 * t1[0][1] + t2[0][1])
                else:
                    bc[7 * p1 + p2, pl.ds(16 * ru, 16), :] = _inner_operand(x, t2).astype(bf16)

    def weight_units(src, row_of, bc):
        return [(7, weight_unit(src, row_of, ru, bc)) for ru in range(32)]

    def lhs_unit(src, dst, slot, r, tag):
        ld = lambda i, j: src[pl.ds((4 * i + j) * MB + 16 * r, 16), :]
        for p1, t1 in enumerate(_A_TERMS):
            yield tag
            x = _outer_operand(ld, t1)
            for p2, t2 in enumerate(_A_TERMS):
                dst[slot(7 * p1 + p2), pl.ds(16 * r, 16), :] = _inner_operand(x, t2).astype(bf16)

    def hidden_units(mm, c):
        def first(r8):
            def finish(i, j, v):
                uu_v[pl.ds((4 * i + j) * MB + 8 * r8, 8), :] = _gelu2(v)
            return _recombine(lambda p: mm[pl.ds(p * MB + 8 * r8, 8), :],
                              lambda j: mod_v[pl.ds(pl.multiple_of(6 * D + 8 * (4 * c + j), 8), 8), :],
                              finish, "o")
        units = []
        for r in range(MB // 16):
            units += [(7, first(2 * r)), (7, first(2 * r + 1)),
                      (7, lhs_unit(uu_v, uc_v, lambda p: p * NCH + c, r, "u"))]
        return units

    def output_units(mm, n):
        def unit(r8):
            def finish(i, j, v):
                row = i * MB + 8 * r8
                res = x2_v[pl.ds(pl.multiple_of((4 * n + j) * D + row, 8), 8), :]
                io_v[4 * n + j, pl.ds(row, 8), :] = (res + mod_v[pl.ds(5 * D + row, 8), :] * v).astype(bf16)
            return _recombine(lambda p: mm[pl.ds(p * MB + 8 * r8, 8), :],
                              lambda j: mod_v[pl.ds(pl.multiple_of(6 * D + 8 * (36 + 4 * n + j), 8), 8), :],
                              finish, "o")
        return [(7, unit(r8)) for r8 in range(MB // 8)]

    def step(product, side, w_src, w_row, o_src):
        total, gen = side
        pending, done = next(gen, None), 0
        for _ in range(3):
            if pending is not None:
                pending, done = next(gen, None), done + 1
        points = NP * (MB // 16) - 12
        pt = 0
        for p in range(NP):
            for v in product(p):
                pt += 1
                seen = set()
                while pending is not None and done * points < pt * total:
                    if pending not in seen:
                        seen.add(pending)
                        if pending == "w":
                            tick(w_src, w_row, pltpu.bitcast(v, u32))
                        elif pending == "o":
                            tick(o_src, NP * MB, v)
                        else:
                            tick(uu_v, 16 * MB, v)
                    pending, done = next(gen, None), done + 1
        assert pending is None

    def deep_product(lhs_ref, slot, bc, dst, init=None):
        lhs_u, bc_u = lhs_ref.bitcast(u32), bc.bitcast(u32)

        def product(p):
            lhs = jnp.concatenate([as_bf16(lhs_u[slot(p, t)]) for t in range(4)], axis=1)
            v = jnp.dot(lhs, as_bf16(bc_u[p]), preferred_element_type=f32)
            for r in range(MB // 16):
                blk = v[16 * r:16 * r + 16]
                if init is not None:
                    blk = blk + init(p, r)
                dst[pl.ds(p * MB + 16 * r, 16), :] = blk
                yield blk[:8]
        return product

    w1_row = lambda c: (lambda k, j, ru: pl.multiple_of((4 * c + j) * W1_ROWS + 256 * k + 8 * ru, 8))
    w2_row_wide = lambda k, j, ru: (4 * (ru // 8) + j) * W2_ROWS + 64 * k + 8 * (ru % 8)
    w2_row = lambda n, h: (lambda k, j, ru: pl.multiple_of(
        (4 * n + j) * W2_ROWS + 256 * (1 + 4 * h + ru // 8) + 64 * k + 8 * (ru % 8), 8))

    def first_half(w1_v, ac_v, wmod_v, dmat_v, gmat_v, wf_v, wt_v, ha_v, ra_v, uv_v, tl_v,
                   zl_v, pp_v, qq_v, sem, sem_x, sem_w1):
        x_copies = [pltpu.make_async_copy(x_hbm.at[:, pl.ds(128 * t, 128)], io_v.at[t], sem_x.at[t])
                    for t in range(16)]
        wmod_copies = [pltpu.make_async_copy(wmod_hbm.at[:, pl.ds(1152 * h, 1152 * (h + 1))],
                                             wmod_v.at[:, pl.ds(1152 * h, 1152 * (h + 1))], sem.at[h])
                       for h in range(2)]
        dmat_copy = pltpu.make_async_copy(dmat_hbm, dmat_v, sem.at[2])
        gmat_copy = pltpu.make_async_copy(gmat_hbm, gmat_v, sem.at[3])
        wf_copies = [pltpu.make_async_copy(src, wf_v.at[a], sem.at[4 + a])
                     for a, src in enumerate((wr_hbm, wi_hbm))]

        def w1_copies(c):
            return [pltpu.make_async_copy(
                w1_hbm.bitcast(u32).at[:, pl.ds(pl.multiple_of(128 * (4 * c + j), 128), 128)],
                w1_v.at[pl.ds(pl.multiple_of((4 * c + j) * W1_ROWS, 8), W1_ROWS)], sem_w1.at[c])
                for j in range(4)]

        def start(copies):
            for cp in copies:
                cp.start()

        def wait(copies):
            for cp in copies:
                cp.wait()

        wmod_copies[0].start()
        for a in range(4):
            for b in range(4):
                x_copies[a + 4 * b].start()
            if a == 0:
                dmat_copy.start()

        cv = c_ref[...].astype(f32)
        sc = jnp.broadcast_to(cv * jax.nn.sigmoid(cv), (16, D)).astype(bf16)
        b1 = b1_ref[...].astype(f32).reshape(1, F)
        for t in range(36):
            mod_v[pl.ds(6 * D + 8 * t, 8), :] = jnp.broadcast_to(b1[:, 128 * t:128 * t + 128], (8, 128))
        b2 = 2.0 * b2_ref[...].astype(f32).reshape(1, S)
        for t in range(16):
            mod_v[pl.ds(6 * D + 8 * (36 + t), 8), :] = jnp.broadcast_to(b2[:, 128 * t:128 * t + 128], (8, 128))

        def modulation(t0, t1):
            m = jnp.dot(sc, wmod_v[:, pl.ds(128 * t0, 128 * (t1 - t0))], preferred_element_type=f32)[:8]
            for t in range(t0, t1):
                col = 128 * t + jax.lax.broadcasted_iota(jnp.int32, (8, 128), 1)
                v = m[:, 128 * (t - t0):128 * (t - t0 + 1)]
                scale = ((col >= D) & (col < 2 * D)) | ((col >= 4 * D) & (col < 5 * D))
                v = jnp.where(scale, 1.0 + v, v)
                v = jnp.where(col >= 5 * D, 0.5 * v, v)
                mod_v[pl.ds(128 * t, 128), :] = jnp.concatenate([v] * 16, axis=0).T

        wmod_copies[0].wait()
        modulation(0, 9)
        dmat_copy.wait()
        dmat_u, io_u = dmat_v.bitcast(u32), io_v.bitcast(u32)

        for a in range(4):
            for b in range(4):
                x_copies[a + 4 * b].wait()
            if a == 1:
                for cp in wf_copies:
                    cp.start()
                gmat_copy.start()
            if a == 3:
                wmod_copies[1].start()
                start(w1_copies(0) + w1_copies(1))
            for b in range(4):
                t = a + 4 * b
                xf = as_bf16(io_u[t]).astype(f32)
                ha_v[pl.ds(b * D, D), :] = xf
                acc = xf[0:8]
                for r in range(1, D // 8):
                    acc = acc + xf[8 * r:8 * r + 8]
                mean = _colsum(acc) * (1.0 / D)
                acc = None
                for r in range(D // 8):
                    d = ha_v[pl.ds(b * D + 8 * r, 8), :] - mean
                    acc = d * d if acc is None else acc + d * d
                rstd = 1.0 / jnp.sqrt(_colsum(acc) * (1.0 / D) + 1e-5)
                held = None
                for r in range(8):
                    h = []
                    for i in range(9):
                        row = 64 * i + 8 * r
                        xn = (ha_v[pl.ds(b * D + row, 8), :] - mean) * rstd
                        h.append(xn * mod_v[pl.ds(D + row, 8), :] + mod_v[pl.ds(row, 8), :])
                    z = _dft9(h)
                    for g in range(4):
                        ra_v[5 * b + g, pl.ds(16 * r, 16), :] = _pack(*z[g + 1])
                    if r % 2 == 0:
                        held = z[0]
                    else:
                        ra_v[5 * b + 4, pl.ds(8 * (r - 1), 16), :] = _pack(held, z[0])
            ra_u = ra_v.bitcast(u32)
            for g in range(5):
                if g < 4:
                    lhs = as_bf16(dmat_u[g])
                    rhs = jnp.concatenate([as_bf16(ra_u[5 * b + g]) for b in range(4)], axis=1)
                else:
                    lhs = as_bf16(dmat_u[4, pl.ds(0, 40), pl.ds(0, 64)])
                    rhs = jnp.concatenate([as_bf16(ra_u[5 * b + 4, pl.ds(0, 32), :]) for b in range(4)], axis=1)
                v = jnp.dot(lhs, rhs, preferred_element_type=f32)
                for r in range(NRG[g]):
                    z = [(v[16 * r:16 * r + 8, 128 * b:128 * b + 128], v[16 * r + 8:16 * r + 16, 128 * b:128 * b + 128])
                         for b in range(4)]
                    for c, y in enumerate(_radix4(z, -1)):
                        y = _twiddle(y, a * c, -1)
                        uv_v[4 * c + a, pl.ds(128 * g + 16 * r, 8), :] = y[0]
                        uv_v[4 * c + a, pl.ds(128 * g + 16 * r + 8, 8), :] = y[1]

        for cp in wf_copies:
            cp.wait()
        lane = jax.lax.broadcasted_iota(jnp.int32, (8, 128), 1)
        masks = [(lane & (1 << i)) != 0 for i in range(4)]

        def regroup(tiles):
            t = [pltpu.roll(v, b, 1) if b else v for b, v in enumerate(tiles)]
            t = [t[-i % 16] for i in range(16)]
            for i in range(4):
                t = [jnp.where(masks[i], t[(j - (1 << i)) % 16], t[j]) for j in range(16)]
            return t

        for a in range(2):
            for r in range(18):
                tiles = [pltpu.bitcast(wf_v[a, pl.ds(16 * r, 16), pl.ds(128 * b, 128)], u32) for b in range(16)]
                for j1, v in enumerate(regroup(tiles)):
                    wt_v[16 * a + j1, pl.ds(16 * r, 16), :] = as_bf16(v).astype(f32)
            last = jnp.broadcast_to(wf_v[a, pl.ds(288, 1), :].astype(f32), (8, S))
            for j1, v in enumerate(regroup([last[:, 128 * b:128 * b + 128] for b in range(16)])):
                wt_v[16 * a + j1, pl.ds(288, 8), :] = v
        gmat_copy.wait()
        for c in range(2, NCH):
            start(w1_copies(c))
        gmat_u = gmat_v.bitcast(u32)

        def filt(a, j1, g, r):
            if g < 4:
                first = (g + 1 if r < 4 else 8 - g) + 72 * (r % 4)
                return wt_v[16 * a + j1, pl.ds(first, 8, stride=9), :]
            if r < 4:
                return wt_v[16 * a + j1, pl.ds(72 * r, 8, stride=9), :]
            return wt_v[16 * a + j1, pl.ds(288, 8), :]

        def cmul(v, r):
            top, bot = v[16 * r:16 * r + 8], v[16 * r + 8:16 * r + 16]
            return top[:, :128] - bot[:, 128:], top[:, 128:] + bot[:, :128]

        tl_u, zl_u, qq_u = tl_v.bitcast(u32), zl_v.bitcast(u32), qq_v.bitcast(u32)
        for g in range(5):
            n = NRG[g]
            o = 16 * (g % 2)
            for r in range(n):
                row = 128 * g + 16 * r
                for c in range(4):
                    z = [(uv_v[4 * c + a, pl.ds(row, 8), :], uv_v[4 * c + a, pl.ds(row + 8, 8), :]) for a in range(4)]
                    for e, y in enumerate(_radix4(z, -1)):
                        tl_v[o + c + 4 * e, pl.ds(16 * r, 16), :] = _pack(*y)
            for j1 in range(16):
                rhs = jnp.concatenate([as_bf16(gmat_u[2 * j1 + i]) for i in range(2)], axis=1)
                v = jnp.dot(as_bf16(tl_u[o + j1, pl.ds(0, 8 * n), :]), rhs, preferred_element_type=f32)
                for r in range(n):
                    yr, yi = cmul(v, r)
                    wr, wi = filt(0, j1, g, r), filt(1, j1, g, r)
                    zl_v[o + j1, pl.ds(16 * r, 16), :] = _pack(yr * wr - yi * wi, yr * wi + yi * wr)
            for j1 in range(16):
                rhs = jnp.concatenate([as_bf16(gmat_u[32 + 2 * j1 + i]) for i in range(2)], axis=1)
                v = jnp.dot(as_bf16(zl_u[o + j1, pl.ds(0, 8 * n), :]), rhs, preferred_element_type=f32)
                for r in range(n):
                    yr, yi = cmul(v, r)
                    pp_v[o + j1, pl.ds(16 * r, 8), :] = yr
                    pp_v[o + j1, pl.ds(16 * r + 8, 8), :] = yi
            for r in range(n):
                mid = [[None] * 4 for _ in range(4)]
                for c in range(4):
                    z = [(pp_v[o + c + 4 * e, pl.ds(16 * r, 8), :], pp_v[o + c + 4 * e, pl.ds(16 * r + 8, 8), :])
                         for e in range(4)]
                    for a, y in enumerate(_radix4(z, 1)):
                        mid[a][c] = _twiddle(y, a * c, 1)
                for a in range(4):
                    for b, y in enumerate(_radix4(mid[a], 1)):
                        qq_v[o + a + 4 * b, pl.ds(16 * r, 16), :] = _pack(*y)
            for a in range(4):
                if g < 4:
                    lhs = as_bf16(dmat_u[5 + g])
                else:
                    lhs = as_bf16(dmat_u[9, pl.ds(0, 32), pl.ds(0, 80)])
                rhs = jnp.concatenate([as_bf16(qq_u[o + a + 4 * b, pl.ds(0, 8 * n), :]) for b in range(4)], axis=1)
                v = jnp.dot(lhs, rhs, preferred_element_type=f32)
                for b in range(4):
                    uv_v[a + 4 * b, pl.ds(128 * g, v.shape[0]), :] = v[:, 128 * b:128 * b + 128]

        wmod_copies[1].wait()
        modulation(9, 27)
        wait(w1_copies(0))
        for _ in _merge(weight_units(w1_v, w1_row(0), bc0))[1]:
            pass

        for a in range(4):
            for b in range(4):
                t = a + 4 * b
                acc = None
                for r2 in range(4):
                    xres = [as_bf16(io_u[t, pl.ds(32 * i + 8 * r2, 8), :]).astype(f32) for i in range(9)]
                    for hh in range(2):
                        r = 2 * r2 + hh
                        z = [(uv_v[t, pl.ds(128 * g + 16 * r, 8), :], uv_v[t, pl.ds(128 * g + 16 * r + 8, 8), :])
                             for g in range(4)]
                        y = _idft9(uv_v[t, pl.ds(512 + 8 * r, 8), :], *z)
                        for i in range(9):
                            row = 64 * i + 8 * r
                            x2 = xres[i][8 * hh:8 * hh + 8] + mod_v[pl.ds(2 * D + row, 8), :] * y[i]
                            x2_v[pl.ds(t * D + row, 8), :] = x2
                            acc = x2 if acc is None else acc + x2
                mean = _colsum(acc) * (1.0 / D)
                acc = None
                for r in range(D // 8):
                    d = x2_v[pl.ds(t * D + 8 * r, 8), :] - mean
                    acc = d * d if acc is None else acc + d * d
                rstd = 1.0 / jnp.sqrt(_colsum(acc) * (1.0 / D) + 1e-5)
                acc = None
                for r in range(D // 8):
                    xn = (x2_v[pl.ds(t * D + 8 * r, 8), :] - mean) * rstd
                    h = xn * mod_v[pl.ds(4 * D + 8 * r, 8), :] + mod_v[pl.ds(3 * D + 8 * r, 8), :]
                    ha_v[pl.ds(b * D + 8 * r, 8), :] = h
                    acc = h if acc is None else acc + h
                mean = _colsum(acc) * (1.0 / D)
                acc = None
                for r in range(D // 8):
                    d = ha_v[pl.ds(b * D + 8 * r, 8), :] - mean
                    acc = d * d if acc is None else acc + d * d
                rstd = 1.0 / jnp.sqrt(_colsum(acc) * (1.0 / D) + 1e-5)
                for r in range(D // 8):
                    i, rr = divmod(8 * r, MB)
                    uu_v[pl.ds((4 * i + b) * MB + rr, 8), :] = (ha_v[pl.ds(b * D + 8 * r, 8), :] - mean) * rstd
            for r in range(MB // 16):
                for _ in lhs_unit(uu_v, ac_v, lambda p: 4 * p + a, r, "u"):
                    pass

        wait(w1_copies(1))
        w1_tick = 36 * W1_ROWS
        slot = lambda p, t: 4 * p + t

        def mm1_step(c, odd, w_units, with_hidden=True):
            bc, mm, prev = (bc1, mm1, mm0) if odd else (bc0, mm0, mm1)
            w_src, w_tick, units = w_units
            streams = [units] + ([hidden_units(prev, c - 1)] if with_hidden else [])
            step(deep_product(ac_v, slot, bc, mm), _merge(*streams), w_src, w_tick, prev)

        next_w1 = lambda c, bc: (w1_v, w1_tick, weight_units(w1_v, w1_row(c), bc))
        mm1_step(0, False, next_w1(1, bc1), with_hidden=False)

        start(w2_copies)

        def pair(i, carry):
            wait(w1_copies(2 * i + 2) + w1_copies(2 * i + 3))
            mm1_step(2 * i + 1, True, next_w1(2 * i + 2, bc0))
            mm1_step(2 * i + 2, False, next_w1(2 * i + 3, bc1))
            return carry

        jax.lax.fori_loop(0, 3, pair, 0)
        wait(w1_copies(8) + w2_copies)
        mm1_step(7, True, next_w1(8, bc0))
        mm1_step(8, False, (w2_v, 16 * W2_ROWS, weight_units(w2_v, w2_row_wide, bc1)))

    pl.run_scoped(
        first_half,
        pltpu.VMEM((36 * W1_ROWS + 8, 128), u32),
        pltpu.VMEM((4 * NP, MB, 128), bf16),
        pltpu.VMEM((D, 6 * D), bf16),
        pltpu.VMEM((10, 128, 128), bf16),
        pltpu.VMEM((64, 128, 128), bf16),
        pltpu.VMEM((2, DF, S), bf16),
        pltpu.VMEM((32, 296, 128), f32),
        pltpu.VMEM((4 * D, 128), f32),
        pltpu.VMEM((20, 128, 128), bf16),
        pltpu.VMEM((16, 592, 128), f32),
        pltpu.VMEM((32, 128, 128), bf16),
        pltpu.VMEM((32, 128, 128), bf16),
        pltpu.VMEM((32, 128, 128), f32),
        pltpu.VMEM((32, 128, 128), bf16),
        pltpu.SemaphoreType.DMA((6,)),
        pltpu.SemaphoreType.DMA((16,)),
        pltpu.SemaphoreType.DMA((NCH,)),
    )

    def second_half(acc_v):
        w2_tick = 16 * W2_ROWS
        uc_u = uc_v.bitcast(u32)

        def wide_product(p):
            rhs = jnp.concatenate([as_bf16(bc1.bitcast(u32)[p, pl.ds(64 * n, 64), :]) for n in range(4)], axis=1)
            v = jnp.dot(as_bf16(uc_u[p * NCH]), rhs, preferred_element_type=f32)
            for r in range(MB // 16):
                for n in range(4):
                    acc_v[pl.ds((n * NP + p) * MB + 16 * r, 16), :] = v[16 * r:16 * r + 16, 128 * n:128 * n + 128]
                yield v[16 * r:16 * r + 8, :128]

        step(wide_product, _merge(weight_units(w2_v, w2_row(0, 0), bc0), hidden_units(mm0, NCH - 1)),
             w2_v, w2_tick, mm0)

        def out_copies(n):
            return [pltpu.make_async_copy(io_v.at[4 * n + j],
                                          out_hbm.at[:, pl.ds(pl.multiple_of(128 * (4 * n + j), 128), 128)],
                                          sem_out.at[4 * n + j]) for j in range(4)]

        def half0(n, with_output):
            init = lambda p, r: acc_v[pl.ds(pl.multiple_of((n * NP + p) * MB + 16 * r, 8), 16), :]
            streams = [weight_units(w2_v, w2_row(n, 1), bc1)] + ([output_units(mm1, n - 1)] if with_output else [])
            step(deep_product(uc_v, lambda p, t: p * NCH + 1 + t, bc0, mm0, init), _merge(*streams),
                 w2_v, w2_tick, mm1)

        def half1(n, with_weights):
            init = lambda p, r: mm0[pl.ds(p * MB + 16 * r, 16), :]
            streams = [weight_units(w2_v, w2_row(n + 1, 0), bc0)] if with_weights else []
            step(deep_product(uc_v, lambda p, t: p * NCH + 5 + t, bc1, mm1, init), _merge(*streams),
                 w2_v, w2_tick, mm1)

        half0(0, False)

        def pair(n, carry):
            half1(n, True)
            half0(n + 1, True)
            for cp in out_copies(n):
                cp.start()
            return carry

        jax.lax.fori_loop(0, 3, pair, 0)
        half1(3, False)
        for _ in _merge(output_units(mm1, 3))[1]:
            pass
        for cp in out_copies(3):
            cp.start()
        for n in range(4):
            for cp in out_copies(n):
                cp.wait()

    pl.run_scoped(second_half, pltpu.VMEM((4 * NP * MB, 128), f32))


@jax.jit
def pallas_adaLN_cond__spectral_gfnet__mixer_token_mlp__prompt_kernel(
    A_x: jax.Array,
    A_w_r: jax.Array,
    A_w_i: jax.Array,
    B_x: jax.Array,
    B_w1: jax.Array,
    B_b1: jax.Array,
    B_w2: jax.Array,
    B_b2: jax.Array,
    c: jax.Array,
    w_mod: jax.Array,
):
    del B_x
    hbm = pl.BlockSpec(memory_space=pl.ANY)
    vmem = pl.BlockSpec(memory_space=pltpu.VMEM)
    out = pl.pallas_call(
        _kernel,
        out_shape=jax.ShapeDtypeStruct((D, S), bf16),
        in_specs=[hbm, hbm, hbm, hbm, vmem, hbm, vmem, vmem, hbm, hbm, hbm,
                  pl.BlockSpec(memory_space=pltpu.SMEM)],
        out_specs=hbm,
        scratch_shapes=[
            pltpu.VMEM((16 * W2_ROWS + 8, 128), u32),
            pltpu.VMEM((NP * NCH, MB, 128), bf16),
            pltpu.VMEM((NP, 512, 128), bf16),
            pltpu.VMEM((NP, 512, 128), bf16),
            pltpu.VMEM((NP * MB + 8, 128), f32),
            pltpu.VMEM((NP * MB + 8, 128), f32),
            pltpu.VMEM((16 * MB + 8, 128), f32),
            pltpu.VMEM((16 * D, 128), f32),
            pltpu.VMEM((6 * D + 8 * 52, 128), f32),
            pltpu.VMEM((16, D, 128), bf16),
            pltpu.SemaphoreType.DMA((16,)),
            pltpu.SemaphoreType.DMA((16,)),
        ],
        compiler_params=pltpu.CompilerParams(vmem_limit_bytes=126 * 1024 * 1024),
        name="adaln_gfnet_mixer",
    )(A_x.reshape(S, D).T, A_w_r.T, A_w_i.T, B_w1, B_b1, B_w2, B_b2, c, w_mod, _DMAT, _GMAT,
      np.zeros((1,), np.int32))
    return out.T.reshape(1, S, D)
```

```python
import numpy as np
import jax
import jax.numpy as jnp
import jax.experimental.pallas as pl
import jax.experimental.pallas.tpu as pltpu

S, D, F = 2048, 576, 4608
DF = D // 2 + 1
NP = 49
MB = D // 4
NCH = F // 512
NRG = (8, 8, 8, 8, 5)
STAGE = 1024

f32, u32, bf16 = jnp.float32, jnp.uint32, jnp.bfloat16


def _interleave(a, b):
    n = a.shape[0] // 8
    return np.stack([a.reshape(n, 8, -1), b.reshape(n, 8, -1)], axis=1).reshape(16 * n, -1)


def _constants():
    d0 = np.arange(64)
    fd = np.zeros((5, 128, 128))
    fi = np.zeros((5, 128, 128))
    scale = 1.0 / (S * D)
    for k1 in range(1, 5):
        k = np.array([k1 + 9 * m for m in range(32)] + [9 - k1 + 9 * m for m in range(32)])
        sg = np.array([1.0] * 32 + [-1.0] * 32)[:, None]
        ang = 2 * np.pi * np.outer(k, d0) / D
        c, s = np.cos(ang), np.sin(ang)
        q = np.sqrt(3.0) / 2 if k1 == 3 else 1.0
        re = _interleave(c.T, (-q * sg * s).T).T
        im = _interleave(-s.T, (-q * sg * c).T).T
        fd[k1 - 1] = _interleave(re, im)
        fi[k1 - 1] = 2 * scale * fd[k1 - 1].T
    ang = 2 * np.pi * np.outer(9 * np.arange(33), d0) / D
    re, im = np.zeros((40, 64)), np.zeros((40, 64))
    re[:33], im[:33] = np.cos(ang), -np.sin(ang)
    im[0] = im[32] = 0.0
    w = np.full((40, 1), 2.0)
    w[0] = w[32] = 1.0
    fd[4, :80, :64] = _interleave(re, im)
    fi[4, :64, :80] = scale * _interleave(w * re, w * im).T
    return np.concatenate([fd, fi]).astype(np.float32).astype(jnp.bfloat16)


_DMAT = _constants()

_C1, _C2, _C4 = (float(np.cos(2 * np.pi * k / 9)) for k in (1, 2, 4))
_S1, _S4, _S3 = float(np.sin(2 * np.pi / 9)), float(np.sin(8 * np.pi / 9)), float(np.sqrt(3.0) / 2)


def _dft9(x):
    e1, e2, e3, e4 = x[1] + x[8], x[2] + x[7], x[3] + x[6], x[4] + x[5]
    o1, o2, o3, o4 = x[1] - x[8], x[2] - x[7], x[3] - x[6], x[4] - x[5]
    t = x[0] - 0.5 * e3
    sm = e1 + e2 + e4
    p = x[0] + e3
    d1, d2 = e1 - e4, e2 - e4
    q1 = _C1 * d1 + _C2 * d2
    q2 = _C2 * d1 + _C4 * d2
    a, b, c = o1 + o2, o2 + o4, o1 - o4
    r1 = _S1 * a + _S4 * b
    r2 = _S1 * c + _S4 * a
    v = _S3 * o3
    return (p + sm, (t + q1, r1 + v), (t + q2, r2 - v), (p - 0.5 * sm, (o1 - o2) + o4),
            ((t - q1) - q2, (r2 - r1) + v))


def _idft9(a0, z1, z2, z3, z4):
    (a1, b1), (a2, b2), (a3, b3), (a4, b4) = z1, z2, z3, z4
    o3 = _S3 * ((b1 - b2) + b4)
    r1, r2 = b1 - b4, b2 + b4
    a, b, c = _S1 * r1 + _S4 * r2, _S4 * r1, _S1 * r2
    o1, o2, o4 = (a + c) + b3, (a + b) - b3, (b - c) + b3
    t = (a1 + a2) + a4
    q1, q2 = a1 - a4, a2 - a4
    d1 = _C1 * q1 + _C2 * q2
    d2 = _C2 * q1 + _C4 * q2
    p, sm = a0 + a3, a0 - 0.5 * a3
    e1, e2, e4 = sm + d1, sm + d2, (sm - d1) - d2
    e3 = p - 0.5 * t
    return [t + p, e1 + o1, e2 + o2, e3 + o3, e4 + o4, e4 - o4, e3 - o3, e2 - o2, e1 - o1]


def _radix4(x, sign):
    t0 = (x[0][0] + x[2][0], x[0][1] + x[2][1])
    t1 = (x[0][0] - x[2][0], x[0][1] - x[2][1])
    t2 = (x[1][0] + x[3][0], x[1][1] + x[3][1])
    t3 = (x[1][0] - x[3][0], x[1][1] - x[3][1])
    plus = (t1[0] - t3[1], t1[1] + t3[0])
    minus = (t1[0] + t3[1], t1[1] - t3[0])
    y1, y3 = (plus, minus) if sign > 0 else (minus, plus)
    return [(t0[0] + t2[0], t0[1] + t2[1]), y1, (t0[0] - t2[0], t0[1] - t2[1]), y3]


def _twiddle(z, n, sign):
    re, im = z
    if n == 0:
        return z
    if n == 4:
        return (-im, re) if sign > 0 else (im, -re)
    c, s = float(np.cos(np.pi * n / 8)), sign * float(np.sin(np.pi * n / 8))
    if n in (2, 6):
        if c * s > 0:
            return (c * (re - im), c * (im + re))
        return (c * (re + im), c * (im - re))
    return (c * re - s * im, c * im + s * re)


_A_TERMS = (((0, 0), 1, (1, 1)), ((1, 0), 1, (1, 1)), ((0, 0), 0, None), ((1, 1), 0, None),
            ((0, 0), 1, (0, 1)), ((1, 0), -1, (0, 0)), ((0, 1), -1, (1, 1)))
_B_TERMS = (((0, 0), 1, (1, 1)), ((0, 0), 0, None), ((0, 1), -1, (1, 1)), ((1, 0), -1, (0, 0)),
            ((1, 1), 0, None), ((0, 0), 1, (0, 1)), ((1, 0), 1, (1, 1)))


def _add2(x, y):
    return [[x[i][j] + y[i][j] for j in range(2)] for i in range(2)]


def _sub2(x, y):
    return [[x[i][j] - y[i][j] for j in range(2)] for i in range(2)]


def _outer_operand(ld, term):
    a, s, b = term
    x = [[ld(2 * a[0] + i, 2 * a[1] + j) for j in range(2)] for i in range(2)]
    if s == 0:
        return x
    y = [[ld(2 * b[0] + i, 2 * b[1] + j) for j in range(2)] for i in range(2)]
    return _add2(x, y) if s > 0 else _sub2(x, y)


def _inner_operand(x, term):
    a, s, b = term
    if s == 0:
        return x[a[0]][a[1]]
    return x[a[0]][a[1]] + x[b[0]][b[1]] if s > 0 else x[a[0]][a[1]] - x[b[0]][b[1]]


def _inner_result(m):
    m1, m4, m2 = m(0), m(3), m(1)
    c21, c22, c11 = m2 + m4, m1 - m2, m1 + m4
    m5, m3 = m(4), m(2)
    c12, c11, c22 = m3 + m5, c11 - m5, c22 + m3
    return [[c11 + m(6), c12], [c21, c22 + m(5)]]


def _inner_block(load, bias, p1):
    def m(p2):
        v = load(7 * p1 + p2)
        if p1 in (3, 2) and p2 in (3, 2):
            v = v + bias(2 * (3 - p1) + (3 - p2))
        return v
    return _inner_result(m)


def _finish_block(finish, c, bi, bj):
    for i in range(2):
        for j in range(2):
            finish(2 * bi + i, 2 * bj + j, c[i][j])


def _recombine(load, bias, finish, tag):
    yield tag
    m2 = _inner_block(load, bias, 1)
    yield tag
    m4 = _inner_block(load, bias, 3)
    _finish_block(finish, _add2(m2, m4), 1, 0)
    yield tag
    m1 = _inner_block(load, bias, 0)
    c22, c11 = _sub2(m1, m2), _add2(m1, m4)
    yield tag
    m5 = _inner_block(load, bias, 4)
    c11 = _sub2(c11, m5)
    yield tag
    m3 = _inner_block(load, bias, 2)
    c22 = _add2(c22, m3)
    _finish_block(finish, _add2(m3, m5), 0, 1)
    yield tag
    _finish_block(finish, _add2(c11, _inner_block(load, bias, 6)), 0, 0)
    yield tag
    _finish_block(finish, _add2(c22, _inner_block(load, bias, 5)), 1, 1)


def _gelu2(x):
    c0 = float(np.sqrt(2.0 / np.pi))
    return x + x * jnp.tanh(x * (c0 + (c0 * 0.044715) * (x * x)))


def _merge(*streams, fine=False):
    streams = [us for us in streams if us]

    def whole():
        order = sorted(((i + 0.5) / len(us), k, i) for k, us in enumerate(streams) for i in range(len(us)))
        for _, k, i in order:
            costs, gen = streams[k][i]
            yield from zip(gen, costs + [None])

    def pieces():
        order = []
        for k, us in enumerate(streams):
            costs = np.array([c for u in us for c in u[0]])
            order += [(float(q) / costs.sum(), k, int(c)) for q, c in zip(np.cumsum(costs) - 0.5 * costs, costs)]
        gens = [(tag for u in us for tag in u[1]) for us in streams]
        heads = [next(g) for g in gens]
        for _, k, c in sorted(order):
            yield heads[k], c
            heads[k] = next(gens[k], None)

    return sum(sum(u[0]) for us in streams for u in us), (pieces() if fine else whole())


def _run(units):
    for _, gen in units:
        for _ in gen:
            pass


def _pack(a, b):
    return jnp.concatenate([a, b], axis=0).astype(bf16)


def _colmean(v):
    return jnp.sum(v, axis=0, keepdims=True) * (1.0 / D)


def _rows(start, n):
    return pl.ds(start if isinstance(start, int) else pl.multiple_of(start, 8), n)


def _lanes(tile):
    return pl.ds(128 * tile if isinstance(tile, int) else pl.multiple_of(128 * tile, 128), 128)


def _as_bf16(v):
    return pltpu.bitcast(v, bf16)


def _tile(v, t):
    return v[:, 128 * t:128 * t + 128]


def _start(copies):
    for cp in copies:
        cp.start()


def _wait(copies):
    for cp in copies:
        cp.wait()


def _operand_costs(terms, groups, unpack):
    out, have = [], set()
    for keep, group in groups:
        have, n = have & set(keep), 0
        for p1 in group:
            a, s, b = terms[p1]
            need = {(2 * q[0] + i, 2 * q[1] + j) for q in ((a, b) if s else (a,)) for i in range(2) for j in range(2)}
            n += unpack * len(need - have) + (8 if s else 0) + 17
            have |= need
        out.append(n)
    return out


def _quad(*blocks):
    return [(2 * a + i, 2 * b + j) for a, b in blocks for i in range(2) for j in range(2)]


_SINGLE = [((), (p,)) for p in range(7)]
_SHARED = [((), (1,)), (_quad((0, 0), (1, 1)), (5,)), (_quad((0, 0), (1, 1), (0, 1)), (4, 2)),
           (_quad((0, 0), (1, 1)), (0, 6)), (_quad((0, 0), (1, 1), (1, 0)), (3,))]
_OUTER_ORDER = (1, 3, 0, 4, 2, 6, 5)

_B1, _B2 = 6 * D, 6 * D + 8 * 36
_HA = _B2 + 8 * 16
_AR_TICK = _HA + 4 * D
_S_SMALL, _S_X, _S_MOD, _S_DMAT, _S_WF, _S_STAGE, _S_WIDE, _S_OUT, _N_SEM = 0, 1, 5, 10, 12, 15, 17, 18, 19


def _kernel(x_hbm, wr_hbm, wi_hbm, w1_hbm, b1_hbm, w2_hbm, b2_hbm, c_hbm, wmod_hbm, dmat_hbm, zero_hbm,
            out_hbm,
            zero_s, st0, st1, uc_v, bc0, bc1, mm0, mm1, uu_v, x2_v, ar_v, io_v, sem):
    copy = pltpu.make_async_copy
    state = {}

    def tick(target, val):
        ref, idx, row = target
        val = pltpu.bitcast(val, ref.dtype)
        n = val.shape[0]
        ref[idx + (pl.ds(pl.multiple_of(row + state["zero"], n), n), pl.ds(0, 128))] = val

    def paced(main, points, side, lead):
        total, gen = side
        pending, done = next(gen, None), 0
        for _ in range(lead):
            if pending is not None:
                pending, done = next(gen, None), done + pending[1]
        for pt, v in enumerate(main, 1):
            seen = []
            while pending is not None and done * points < pt * total:
                if not any(pending[0] is t for t in seen):
                    seen.append(pending[0])
                    tick(pending[0], v)
                pending, done = next(gen, None), done + pending[1]
        assert pending is None

    def chained(units, target, lag):
        late = []
        for k, unit in enumerate(units):
            if k >= lag:
                for v in late[k - lag]:
                    tick(target, v)
            late.append(unit())

    t_uu, t_ar = (uu_v, (), 16 * MB), (ar_v, (), _AR_TICK)
    t_mm = [(mm0, (), NP * MB), (mm1, (), NP * MB)]
    t_st = [(st0, (), 4 * STAGE), (st1, (), 4 * STAGE)]
    bcs = (bc0, bc1)

    def stage_copies(par, src, row, tile):
        return [copy(src.bitcast(u32).at[_rows(row, STAGE), _lanes(tile + j)],
                     t_st[par][0].at[pl.ds(j * STAGE, STAGE)], sem.at[_S_STAGE + par]) for j in range(4)]

    def stage_wait(par):
        whole = t_st[par][0].at[pl.ds(0, 4 * STAGE)]
        copy(whole, whole, sem.at[_S_STAGE + par]).wait()

    def operand_unit(target, raw, load, terms, groups, put):
        cache = {}
        for keep, group in groups:
            yield target
            cache = {k: v for k, v in cache.items() if k in keep}

            def ld(i, j):
                if (i, j) not in cache:
                    cache[i, j] = load(i, j)
                return cache[i, j]

            for p1 in group:
                t1 = terms[p1]
                x = _outer_operand(ld, t1)
                for p2, t2 in enumerate(terms):
                    if raw is not None and t1[1] == 0 and t2[1] == 0:
                        put(7 * p1 + p2, raw(2 * t1[0][0] + t2[0][0], 2 * t1[0][1] + t2[0][1]))
                    else:
                        put(7 * p1 + p2, _inner_operand(x, t2).astype(bf16))

    def weight_units(par, groups, source=None):
        target, bc = source or t_st[par], bcs[par]

        def unit(ru):
            def raw(k, j):
                return target[0][pl.ds(j * STAGE + 256 * (ru // 8) + 64 * k + 8 * (ru % 8), 8), :]

            def put(p, v):
                if v.dtype == u32:
                    bc.bitcast(u32)[p, pl.ds(8 * ru, 8), :] = v
                else:
                    bc[p, pl.ds(16 * ru, 16), :] = v
            return operand_unit(target, raw, lambda k, j: _as_bf16(raw(k, j)).astype(f32), _B_TERMS, groups, put)
        return [(_operand_costs(_B_TERMS, groups, 2), unit(ru)) for ru in range(32)]

    def hidden_units(c, par):
        target = t_mm[par]

        def first(r8):
            def finish(i, j, v):
                uu_v[pl.ds((4 * i + j) * MB + 8 * r8, 8), :] = _gelu2(v)
            return _recombine(lambda p: target[0][pl.ds(p * MB + 8 * r8, 8), :],
                              lambda j: ar_v[_rows(_B1 + 8 * (4 * c + j), 8), :], finish, target)

        def second(r):
            def put(p, v):
                uc_v[p * NCH + c, pl.ds(16 * r, 16), :] = v
            return operand_unit(t_uu, None, lambda i, j: uu_v[pl.ds((4 * i + j) * MB + 16 * r, 16), :],
                                _A_TERMS, _SINGLE, put)

        units, cost = [], [8, 38, 16, 12, 42, 36, 36]
        for r in range(MB // 16):
            units += [(cost, first(2 * r)), (cost, first(2 * r + 1)),
                      (_operand_costs(_A_TERMS, _SINGLE, 0), second(r))]
        return units

    def products(product, outer, side):
        main = (v for p1 in outer for p2 in range(7) for v in product(7 * p1 + p2))
        points = 7 * len(outer) * (MB // 16)
        paced(main, points - max(2, points // 40), side, lead=3 if len(outer) == 7 else 1)

    def deep_product(lhs_ref, slot, bc, dst, init=None):
        lhs_u, bc_u = lhs_ref.bitcast(u32), bc.bitcast(u32)

        def product(p):
            lhs = jnp.concatenate([_as_bf16(lhs_u[slot(p, t)]) for t in range(4)], axis=1)
            v = jnp.dot(lhs, _as_bf16(bc_u[p]), preferred_element_type=f32)
            for r in range(MB // 16):
                blk = v[16 * r:16 * r + 16]
                if init is not None:
                    blk = blk + init(p, r)
                dst[pl.ds(p * MB + 16 * r, 16), :] = blk
                yield blk[:8]
        return product

    def first_half(wide_v, ac_v, wmod_v, dmat_v, gmat_v, wf_v, wt_v, uv_v, bb_v, ee_v, sa_v, c_v, b1_v, b2_v):
        small_copies = [copy(c_hbm, c_v, sem.at[_S_SMALL]), copy(zero_hbm, zero_s, sem.at[_S_SMALL]),
                        copy(b1_hbm, b1_v, sem.at[_S_SMALL]), copy(b2_hbm, b2_v, sem.at[_S_SMALL])]
        x_copies = lambda a: [copy(x_hbm.at[:, _lanes(a + 4 * b)], io_v.at[a + 4 * b], sem.at[_S_X + a])
                              for b in range(4)]
        mod_tiles = ((4, 9), (0, 4), (9, 14), (14, 23), (23, 27))
        wmod_copies = [copy(wmod_hbm.at[:, pl.ds(128 * t0, 128 * (t1 - t0))],
                            wmod_v.at[:, pl.ds(128 * t0, 128 * (t1 - t0))], sem.at[_S_MOD + h])
                       for h, (t0, t1) in enumerate(mod_tiles)]
        dmat_copies = [copy(dmat_hbm.at[pl.ds(5 * h, 5)], dmat_v.at[pl.ds(5 * h, 5)], sem.at[_S_DMAT + h])
                       for h in range(2)]
        wf_rows = ((0, 96), (96, 96), (192, DF - 192))
        wf_copies = [[copy(src.at[pl.ds(*rows)], wf_v.at[a, pl.ds(*rows)], sem.at[_S_WF + h])
                      for a, src in enumerate((wr_hbm, wi_hbm))] for h, rows in enumerate(wf_rows)]
        G = {"S": _SINGLE, "H": _SHARED}

        def mm1_step(c, par):
            products(deep_product(ac_v, lambda p, t: 4 * p + t, bcs[par], t_mm[par][0]), range(7),
                     _merge(weight_units(1 - par, G["S"]), hidden_units(c - 1, 1 - par),
                            fine=bool(0)))

        late_copies = [wmod_copies[1]] + sum(wf_copies, []) + [dmat_copies[1]] + wmod_copies[2:]
        _start(small_copies + [wmod_copies[0], dmat_copies[0]] + x_copies(0) + x_copies(1) + x_copies(2)
               + x_copies(3) + ([] if 0 else late_copies))

        _wait(small_copies)
        state["zero"] = zero_s[0]
        s0 = jax.lax.broadcasted_iota(jnp.int32, (16, 128), 0)
        j0 = jax.lax.broadcasted_iota(jnp.int32, (16, 128), 1)
        j0 = 8 * (j0 & 15) + (j0 >> 4)
        phasor = lambda n, period: (jnp.cos(n.astype(f32) * (-2 * np.pi / period)),
                                    jnp.sin(n.astype(f32) * (-2 * np.pi / period)))
        cmul = lambda x, y: (x[0] * y[0] - x[1] * y[1], x[0] * y[1] + x[1] * y[0])
        base, rot, down = phasor((s0 * j0) & 127, 128), phasor(s0, S), phasor(j0[:1] & 7, 8)

        def generate(r, carry):
            g = carry[:2]
            for j1 in range(16):
                for i in range(2):
                    v = pltpu.bitcast(g[i].astype(bf16), u32)
                    gmat_v[2 * j1 + i, pl.ds(pl.multiple_of(16 * r, 16), 16), :] = _as_bf16(
                        pltpu.roll(v, j1, 1) if j1 else v)
                g = cmul(g, carry[2:])
            return cmul(carry[:2], down) + cmul(carry[2:], (float(np.cos(np.pi / 64)), float(-np.sin(np.pi / 64))))

        jax.lax.fori_loop(0, 8, generate, base + rot)
        for t in range(20, 24):
            io_v[t] = jnp.zeros((D, 128), bf16)
        gmat_u, bb_u = gmat_v.bitcast(u32), bb_v.bitcast(u32)


        cv = c_v[...].astype(f32)
        sc = jnp.broadcast_to(cv * jax.nn.sigmoid(cv), (16, D)).astype(bf16)
        b1 = b1_v[...].astype(f32).reshape(1, F)
        for t in range(36):
            ar_v[pl.ds(_B1 + 8 * t, 8), :] = jnp.broadcast_to(_tile(b1, t), (8, 128))
        b2 = 2.0 * b2_v[...].astype(f32).reshape(1, S)
        for t in range(16):
            ar_v[pl.ds(_B2 + 8 * t, 8), :] = jnp.broadcast_to(_tile(b2, t), (8, 128))

        def modulation(h):
            t0, t1 = mod_tiles[h]
            m = jnp.dot(sc, wmod_v[:, pl.ds(128 * t0, 128 * (t1 - t0))], preferred_element_type=f32)[:8]
            for t in range(t0, t1):
                col = 128 * t + jax.lax.broadcasted_iota(jnp.int32, (8, 128), 1)
                v = _tile(m, t - t0)
                scale = ((col >= D) & (col < 2 * D)) | ((col >= 4 * D) & (col < 5 * D))
                v = jnp.where(scale, 1.0 + v, v)
                v = jnp.where(col >= 5 * D, 0.5 * v, v)
                ar_v[pl.ds(128 * t, 128), :] = jnp.concatenate([v] * 16, axis=0).T

        wmod_copies[0].wait()
        modulation(0)
        dmat_u, io_u = dmat_v.bitcast(u32), io_v.bitcast(u32)
        t_io, t_uv, t_x2 = (io_v, (24,), 0), (uv_v, (16,), 0), (x2_v, (), 16 * D)

        fold = lambda v: v.reshape(8, 8, 128).sum(axis=0)

        def dft9_tiles(h, r, held):
            z = _dft9(h)
            out = [(128 * g + 16 * r, _pack(*z[g + 1])) for g in range(4)]
            if r % 2:
                out.append((512 + 8 * (r - 1), _pack(held.pop(), z[0])))
            else:
                held.append(z[0])
            return out

        def put(slot, tiles):
            for row, v in tiles:
                io_v[slot, pl.ds(row, 16), :] = v

        def channel_dft(g, slots):
            n = 64 if g < 4 else 32
            lhs = _as_bf16(dmat_u[g] if g < 4 else dmat_u[4, pl.ds(0, 40), pl.ds(0, 64)])
            rhs = jnp.concatenate([_as_bf16(io_u[t, pl.ds(64 * g, n), :]) for t in slots], axis=1)
            return jnp.dot(lhs, rhs, preferred_element_type=f32)

        def spectrum(a, rstd, ordered=True):
            slots = [16 + 4 * (a % 2) + b for b in range(4)]
            nxt = channel_dft(0, slots)
            for g in range(5):
                yield
                v, nxt = nxt, (channel_dft(g + 1, slots) if g < 4 else None)
                for half in range(2):
                    yield
                    for r in range(4 * half, min(4 * half + 4, NRG[g])):
                        z = [(_tile(v[16 * r:16 * r + 8], b) * rstd[b], _tile(v[16 * r + 8:16 * r + 16], b) * rstd[b])
                             for b in range(4)]
                        for c, y in enumerate(_radix4(z, -1)):
                            uv_v[4 * a + c, pl.ds(128 * g + 16 * r, 16), :] = jnp.concatenate(y, axis=0)
                        if ordered and r % 2 == 2 - 1:
                            tick(t_io, y[1])

        def phase_a(a, rstd_prev):
            _wait(x_copies(a))
            behind = spectrum((a + 3) % 4, rstd_prev)
            next(behind, None)
            for q in range(8):
                gmat_v[32 + 8 * a + q] = _as_bf16(gmat_u[8 * a + q]).T
            mean = [_colmean(fold(_as_bf16(io_u[a + 4 * b]).astype(f32).reshape(9, 64, 128).sum(axis=0)))
                    for b in range(4)]
            sq, queue = [0.0] * 4, []
            for b in range(4):
                held, slot = [], 16 + 4 * (a % 2) + b
                if b:
                    tick(t_ar, sq[b - 1])
                for r in range(8):
                    if r % 2 == 0:
                        xp = [io_u[a + 4 * b, pl.ds(32 * i + 4 * r, 8), :] for i in range(9)]
                        for emit in queue:
                            emit()
                        queue = []
                        next(behind, None)
                        xp = [_as_bf16(v).astype(f32) for v in xp]
                    h = []
                    for i in range(9):
                        d = xp[i][8 * (r % 2):8 * (r % 2) + 8] - mean[b]
                        sq[b] = sq[b] + d * d
                        h.append(d * ar_v[pl.ds(D + 64 * i + 8 * r, 8), :])
                    tiles = dft9_tiles(h, r, held)
                    if r % 2 == 0:
                        put(slot, tiles)
                    else:
                        queue.append(lambda slot=slot, tiles=tiles, q=sq[b]: (put(slot, tiles), tick(t_io, q)))
            assert next(behind, 1) == 1
            for emit in queue:
                emit()
            return tuple(jnp.broadcast_to(jax.lax.rsqrt(_colmean(q) + 1e-5), (8, 128)) for q in sq)

        dmat_copies[0].wait()
        rstd_last = jax.lax.fori_loop(0, 4, phase_a, (jnp.zeros((8, 128), f32),) * 4)
        wmod_copies[1].wait()
        modulation(1)
        held = []
        for r in range(8):
            put(16, dft9_tiles([float(S) * ar_v[pl.ds(64 * i + 8 * r, 8), :] for i in range(9)], r, held))
        for g in range(5):
            v = channel_dft(g, [16])
            first = jax.lax.broadcasted_iota(jnp.int32, v.shape, 1) == 0
            sa_v[pl.ds(128 * g, 16 * NRG[g]), :] = jnp.where(first, v, 0.0)

        for _ in spectrum(3, rstd_last, ordered=False):
            pass

        def pair_at(j, row):
            return uv_v[j, pl.ds(row, 8), :], uv_v[j, pl.ds(row + 8, 8), :]

        def butterflies(g, r):
            row = 128 * g + 16 * r
            for c in range(4):
                yield t_uv
                z = [_twiddle(pair_at(4 * a + c, row), a * c, -1) for a in range(4)]
                for e, y in enumerate(_radix4(z, -1)):
                    bb_v[c + 4 * e, pl.ds(row, 16), :] = _pack(*y)

        def token_dft(g, inverse):
            n = NRG[g]
            for j1 in range(16):
                rhs = jnp.concatenate([_as_bf16(gmat_u[32 * inverse + 2 * j1 + i]) for i in range(2)], axis=1)
                v = jnp.dot(_as_bf16(bb_u[j1, pl.ds(64 * g, 8 * n), :]), rhs, preferred_element_type=f32)
                for r in range(n):
                    top, bot = v[16 * r:16 * r + 8], v[16 * r + 8:16 * r + 16]
                    if inverse:
                        re, im = _tile(top, 0) + _tile(bot, 1), _tile(bot, 0) - _tile(top, 1)
                    else:
                        re, im = _tile(top, 0) - _tile(bot, 1), _tile(bot, 0) + _tile(top, 1)
                    uv_v[j1, pl.ds(128 * g + 16 * r, 16), :] = jnp.concatenate([re, im], axis=0)
                    yield re

        lane = jax.lax.broadcasted_iota(jnp.int32, (8, 128), 1)

        def filt(a, j1, g, r):
            if g < 4:
                first = (g + 1 if r < 4 else 8 - g) + 72 * (r % 4)
                return wt_v[16 * a + j1, pl.ds(first, 8, stride=9), :]
            if r < 4:
                return wt_v[16 * a + j1, pl.ds(72 * r, 8, stride=9), :]
            return wt_v[16 * a + j1, pl.ds(288, 8), :]

        def filtering(g, j1):
            for r in range(NRG[g]):
                if r % 4 == 0:
                    yield t_uv
                row = 128 * g + 16 * r
                yr, yi = pair_at(j1, row)
                if j1 == 0:
                    yr, yi = yr + sa_v[pl.ds(row, 8), :], yi + sa_v[pl.ds(row + 8, 8), :]
                wr, wi = filt(0, j1, g, r), filt(1, j1, g, r)
                bb_v[j1, pl.ds(row, 16), :] = _pack(yr * wr - yi * wi, yr * wi + yi * wr)

        def inverse_butterflies(g, r):
            row = 128 * g + 16 * r
            mid = [[None] * 4 for _ in range(4)]
            for c in range(4):
                yield t_uv
                for a, y in enumerate(_radix4([pair_at(c + 4 * e, row) for e in range(4)], 1)):
                    mid[a][c] = _twiddle(y, a * c, 1)
            for a in range(4):
                for b, y in enumerate(_radix4(mid[a], 1)):
                    bb_v[a + 4 * b, pl.ds(row, 16), :] = _pack(*y)

        bfly = lambda g: [([20, 36, 28, 36], butterflies(g, r)) for r in range(NRG[g])] if g < 5 else []
        filts = lambda g: [([28, 7 * (NRG[g] - 4)], filtering(g, j1)) for j1 in range(16)] if g < 5 else []
        ibfly = lambda g: [([16, 32, 24, 112], inverse_butterflies(g, r)) for r in range(NRG[g])] if g >= 0 else []

        masks = [(lane & (1 << i)) != 0 for i in range(4)]

        def regroup(tiles):
            t = [pltpu.roll(v, b, 1) if b else v for b, v in enumerate(tiles)]
            t = [t[-i % 16] for i in range(16)]
            for i in range(4):
                t = [jnp.where(masks[i], t[(j - (1 << i)) % 16], t[j]) for j in range(16)]
            return t

        def regroup_unit(a, r):
            yield t_wf
            if r < 18:
                tiles = [pltpu.bitcast(wf_v[a, pl.ds(16 * r, 16), pl.ds(128 * b, 128)], u32) for b in range(16)]
                for j1, v in enumerate(regroup(tiles)):
                    wt_v[16 * a + j1, pl.ds(16 * r, 16), :] = _as_bf16(v).astype(f32)
            else:
                last = jnp.broadcast_to(wf_v[a, pl.ds(288, 1), :].astype(f32), (8, S))
                for j1, v in enumerate(regroup([_tile(last, b) for b in range(16)])):
                    wt_v[16 * a + j1, pl.ds(288, 8), :] = v

        t_wf = (wf_v, (2,), 0)
        regroups = lambda h: [([112], regroup_unit(a, r)) for r in range(6 * h, 6 * h + 6 + h // 2) for a in range(2)]
        when = {int(q): h for h, q in enumerate("234")}

        _run(bfly(0))
        for g in range(5):
            if g in when:
                _wait(wf_copies[when[g]])
            paced(token_dft(g, 0), 16 * NRG[g] - 8,
                  _merge(bfly(g + 1), regroups(when[g]) if g in when else [], fine=True), lead=1)
        if 5 in when:
            _wait(wf_copies[2])
            _run(regroups(2))
        first_rows = wide_v.at[pl.ds(0, 4 * STAGE)]
        _start([copy(w1_hbm.bitcast(u32).at[:, _lanes(j)], wide_v.at[pl.ds(j * STAGE, STAGE)], sem.at[_S_WIDE])
                for j in range(4)] + stage_copies(1, w1_hbm, 0, 4) + stage_copies(0, w1_hbm, 0, 8))

        _run(filts(0))
        for g in range(5):
            paced(token_dft(g, 1), 16 * NRG[g] - 8, _merge(filts(g + 1), ibfly(g - 1), fine=bool(0)), lead=1)
        _wait([dmat_copies[1]] + wmod_copies[2:])
        modulation(2)
        _run(ibfly(4))
        modulation(3)
        modulation(4)
        shift = ar_v[pl.ds(3 * D, D), :]
        ar_v[pl.ds(3 * D, D), :] = shift - _colmean(fold(shift.reshape(9, 64, 128).sum(axis=0)))

        for a in range(4):
            rhs = jnp.concatenate([_as_bf16(bb_u[4 * a + b, pl.ds(256, 40), :]) for b in range(4)], axis=1)
            v = jnp.dot(_as_bf16(dmat_u[9, pl.ds(0, 32), pl.ds(0, 80)]), rhs, preferred_element_type=f32)
            for b in range(4):
                ee_v[pl.ds(64 * (4 * a + b), 64), :] = _tile(v, b)

        def phase_c(a, carry):
            acc = [0.0] * 4
            for b in range(4):
                t = 4 * a + b
                v = [jnp.dot(_as_bf16(dmat_u[5 + g]), _as_bf16(bb_u[4 * a + b, pl.ds(64 * g, 64), :]),
                             preferred_element_type=f32) for g in range(4)]
                for r in range(8):
                    if r % 2 == 0:
                        xres = [_as_bf16(io_u[t, pl.ds(32 * i + 4 * r, 8), :]).astype(f32) for i in range(9)]
                    z = [(q[16 * r:16 * r + 8], q[16 * r + 8:16 * r + 16]) for q in v]
                    y = _idft9(ee_v[_rows(64 * (4 * a + b) + 8 * r, 8), :], *z)
                    for i in range(9):
                        row = 64 * i + 8 * r
                        x2 = xres[i][8 * (r % 2):8 * (r % 2) + 8] + ar_v[pl.ds(2 * D + row, 8), :] * y[i]
                        x2_v[_rows(t * D + row, 8), :] = x2
                        acc[b] = acc[b] + x2
                    if r % 2 == 0:
                        tick(t_io, acc[b])
            mean = [_colmean(v) for v in acc]
            sq, lin, sq2 = [0.0] * 4, [0.0] * 4, [0.0] * 4

            def second(b, i):
                d = x2_v[_rows((4 * a + b) * D + 64 * i, 64), :] - mean[b]
                w = d * ar_v[pl.ds(4 * D + 64 * i, 64), :]
                ar_v[pl.ds(_HA + b * D + 64 * i, 64), :] = w
                sq[b], lin[b] = sq[b] + fold(d * d), lin[b] + fold(w)
                return sq[b], lin[b]

            chained([lambda b=b, i=i: second(b, i) for b in range(4) for i in range(9)], t_x2, lag=5)
            rstd = [jax.lax.rsqrt(_colmean(v) + 1e-5) for v in sq]
            mean = [_colmean(v) for v in lin]

            def third(b, i):
                h = ((ar_v[pl.ds(_HA + b * D + 64 * i, 64), :] - mean[b]) * rstd[b]
                     + ar_v[pl.ds(3 * D + 64 * i, 64), :])
                uu_v[pl.ds(b * D + 64 * i, 64), :] = h
                sq2[b] = sq2[b] + fold(h * h)
                return sq2[b],

            chained([lambda b=b, i=i: third(b, i) for b in range(4) for i in range(9)], t_ar, lag=5)
            rstd = [jax.lax.rsqrt(_colmean(v) + 1e-5) for v in sq2]

            def operands(r):
                blk = [[uu_v[pl.ds(k * D + i * MB + 16 * r, 16), :] * rstd[k] for k in range(4)] for i in range(4)]
                for p1, t1 in enumerate(_A_TERMS):
                    x = _outer_operand(lambda i, k: blk[i][k], t1)
                    for p2, t2 in enumerate(_A_TERMS):
                        v = _inner_operand(x, t2)
                        ac_v[4 * (7 * p1 + p2) + a, pl.ds(16 * r, 16), :] = v.astype(bf16)
                    if p1 == 2:
                        late = v[:8]
                return late,

            chained([lambda r=r: operands(r) for r in range(MB // 16)], t_uu, lag=1)
            return carry

        jax.lax.fori_loop(0, 4, phase_c, 0)

        copy(first_rows, first_rows, sem.at[_S_WIDE]).wait()
        stage_wait(1)
        own = lambda k: (weight_units(0, [((), (_OUTER_ORDER[k],))], source=(wide_v, (), 4 * STAGE))
                         if k < 7 else [])
        ahead = weight_units(1, G['H'])
        product = deep_product(ac_v, lambda p, t: 4 * p + t, bc0, mm0)
        _run(own(0))
        for k, p1 in enumerate(_OUTER_ORDER):
            tick((bc0, (NP,), 0), jnp.zeros((8, 128), f32))
            products(product, [p1], _merge(own(k + 1) + (ahead[4 * k:4 * k + 4] if k < 6 else ahead[24:])))

        def mm1_pair(i, carry):
            c = 2 * i + 1

            @pl.when(i < 3)
            def _():
                _start(stage_copies(1, w1_hbm, 0, 4 * (c + 2)))

            @pl.when(i == 3)
            def _():
                _start([copy(w2_hbm.bitcast(u32).at[pl.ds(0, 256), _lanes(4 * n + j)],
                             st1.at[pl.ds(j * STAGE + 256 * n, 256)], sem.at[_S_STAGE + 1])
                        for j in range(4) for n in range(4)])

            stage_wait(0)
            mm1_step(c, 1)

            @pl.when(i < 3)
            def _():
                _start(stage_copies(0, w1_hbm, 0, 4 * (c + 3)))

            @pl.when(i == 3)
            def _():
                _start(stage_copies(0, w2_hbm, 256, 0))

            stage_wait(1)
            mm1_step(c + 1, 0)
            return carry

        jax.lax.fori_loop(0, 4, mm1_pair, 0)

    pl.run_scoped(
        first_half,
        pltpu.VMEM((4 * STAGE + 8, 128), u32),
        pltpu.VMEM((4 * NP, MB, 128), bf16),
        pltpu.VMEM((D, 6 * D), bf16),
        pltpu.VMEM((10, 128, 128), bf16),
        pltpu.VMEM((64, 128, 128), bf16),
        pltpu.VMEM((3, DF, S), bf16),
        pltpu.VMEM((32, 296, 128), f32),
        pltpu.VMEM((17, 592, 128), f32),
        pltpu.VMEM((16, 592, 128), bf16),
        pltpu.VMEM((16 * 64, 128), f32),
        pltpu.VMEM((592, 128), f32),
        pltpu.VMEM((1, D), bf16),
        pltpu.VMEM((F,), bf16),
        pltpu.VMEM((S,), bf16),
    )

    def second_half(acc_v):
        state["zero"] = zero_s[0]
        uc_u = uc_v.bitcast(u32)

        def wide_product(p):
            rhs = jnp.concatenate([_as_bf16(bc1.bitcast(u32)[p, pl.ds(64 * n, 64), :]) for n in range(4)], axis=1)
            v = jnp.dot(_as_bf16(uc_u[p * NCH]), rhs, preferred_element_type=f32)
            for r in range(MB // 16):
                for n in range(4):
                    acc_v[pl.ds((n * NP + p) * MB + 16 * r, 16), :] = _tile(v[16 * r:16 * r + 16], n)
                yield _tile(v[16 * r:16 * r + 8], 0)

        def output_units(n, groups):
            def unit(r8):
                def finish(i, j, v):
                    row = i * MB + 8 * r8
                    res = x2_v[_rows((4 * n + j) * D + row, 8), :]
                    io_v[4 * n + j, pl.ds(row, 8), :] = (res + ar_v[pl.ds(5 * D + row, 8), :] * v).astype(bf16)
                return _recombine(lambda p: mm1[pl.ds(p * MB + 8 * r8, 8), :],
                                  lambda j: ar_v[_rows(_B2 + 8 * (4 * n + j), 8), :], finish, t_mm[1])
            return [([8, 26, 16, 12, 30, 24, 24], unit(r8)) for r8 in groups]

        def out_copies(n, rows=((0, D),)):
            return [copy(io_v.at[4 * n + j, pl.ds(*rr)], out_hbm.at[pl.ds(*rr), _lanes(4 * n + j)], sem.at[_S_OUT])
                    for j in range(4) for rr in rows]

        _start(stage_copies(1, w2_hbm, 256 + STAGE, 0))
        stage_wait(0)
        products(wide_product, range(7),
                 _merge(weight_units(0, _SINGLE), hidden_units(NCH - 1, 0), fine=bool(0)))

        def mm2_pair(n, carry):
            @pl.when(n < 3)
            def _():
                _start(stage_copies(0, w2_hbm, 256, 4 * n + 4))

            stage_wait(1)
            first = deep_product(uc_v, lambda p, t: p * NCH + 1 + t, bc0, mm0,
                                 lambda p, r: acc_v[_rows((n * NP + p) * MB + 16 * r, 16), :])
            products(first, range(7), _merge(weight_units(1, _SINGLE),
                                             output_units((n + 3) % 4, range(MB // 8)), fine=bool(0)))

            @pl.when(n > 0)
            def _():
                _start(out_copies(n - 1))

            @pl.when(n < 3)
            def _():
                _start(stage_copies(1, w2_hbm, 256 + STAGE, 4 * n + 4))
                stage_wait(0)

            second = deep_product(uc_v, lambda p, t: p * NCH + 5 + t, bc1, mm1,
                                  lambda p, r: mm0[pl.ds(p * MB + 16 * r, 16), :])
            products(second, range(7), _merge(weight_units(0, _SINGLE)))
            return carry

        jax.lax.fori_loop(0, 4, mm2_pair, 0)
        last = []
        for h in range(2):
            _run(output_units(3, range(9 * h, 9 * h + 9)))
            last += out_copies(3, [(i * MB + 72 * h, 72) for i in range(4)])
            _start(last[16 * h:])
        _wait(out_copies(0) + out_copies(1) + out_copies(2) + last)

    pl.run_scoped(second_half, pltpu.VMEM((4 * NP * MB, 128), f32))


@jax.jit
def pallas_adaLN_cond__spectral_gfnet__mixer_token_mlp__prompt_kernel(
    A_x: jax.Array,
    A_w_r: jax.Array,
    A_w_i: jax.Array,
    B_x: jax.Array,
    B_w1: jax.Array,
    B_b1: jax.Array,
    B_w2: jax.Array,
    B_b2: jax.Array,
    c: jax.Array,
    w_mod: jax.Array,
):
    del B_x
    hbm = pl.BlockSpec(memory_space=pl.ANY)
    out = pl.pallas_call(
        _kernel,
        out_shape=jax.ShapeDtypeStruct((D, S), bf16),
        in_specs=[hbm] * 11,
        out_specs=hbm,
        scratch_shapes=[
            pltpu.SMEM((1,), jnp.int32),
            pltpu.VMEM((4 * STAGE + 8, 128), u32),
            pltpu.VMEM((4 * STAGE + 8, 128), u32),
            pltpu.VMEM((NP * NCH, MB, 128), bf16),
            pltpu.VMEM((NP + 1, 512, 128), bf16),
            pltpu.VMEM((NP, 512, 128), bf16),
            pltpu.VMEM((NP * MB + 8, 128), f32),
            pltpu.VMEM((NP * MB + 8, 128), f32),
            pltpu.VMEM((16 * MB + 8, 128), f32),
            pltpu.VMEM((16 * D + 8, 128), f32),
            pltpu.VMEM((_AR_TICK + 8, 128), f32),
            pltpu.VMEM((25, D, 128), bf16),
            pltpu.SemaphoreType.DMA((_N_SEM,)),
        ],
        compiler_params=pltpu.CompilerParams(vmem_limit_bytes=126 * 1024 * 1024),
        name="adaln_gfnet_mixer",
    )(A_x.reshape(S, D).T, A_w_r.T, A_w_i.T, B_w1, B_b1, B_w2, B_b2, c, w_mod, _DMAT,
      np.zeros((1,), np.int32))
    return out.T.reshape(1, S, D)
```

```python
import numpy as np
import jax
import jax.numpy as jnp
import jax.experimental.pallas as pl
import jax.experimental.pallas.tpu as pltpu

S, D, F = 2048, 576, 4608
DF = D // 2 + 1
NP = 49
MB = D // 4
NCH = F // 512
NRG = (8, 8, 8, 8, 5)
STAGE = 1280

f32, u32, bf16 = jnp.float32, jnp.uint32, jnp.bfloat16


def _interleave(a, b):
    n = a.shape[0] // 8
    return np.stack([a.reshape(n, 8, -1), b.reshape(n, 8, -1)], axis=1).reshape(16 * n, -1)


def _constants():
    d0 = np.arange(64)
    fd = np.zeros((5, 128, 128))
    fi = np.zeros((5, 128, 128))
    scale = 1.0 / (S * D)
    for k1 in range(1, 5):
        k = np.array([k1 + 9 * m for m in range(32)] + [9 - k1 + 9 * m for m in range(32)])
        sg = np.array([1.0] * 32 + [-1.0] * 32)[:, None]
        ang = 2 * np.pi * np.outer(k, d0) / D
        c, s = np.cos(ang), np.sin(ang)
        q = np.sqrt(3.0) / 2 if k1 == 3 else 1.0
        re = _interleave(c.T, (-q * sg * s).T).T
        im = _interleave(-s.T, (-q * sg * c).T).T
        fd[k1 - 1] = _interleave(re, im)
        fi[k1 - 1] = 2 * scale * fd[k1 - 1].T
    ang = 2 * np.pi * np.outer(9 * np.arange(33), d0) / D
    re, im = np.zeros((40, 64)), np.zeros((40, 64))
    re[:33], im[:33] = np.cos(ang), -np.sin(ang)
    im[0] = im[32] = 0.0
    w = np.full((40, 1), 2.0)
    w[0] = w[32] = 1.0
    fd[4, :80, :64] = _interleave(re, im)
    fi[4, :64, :80] = scale * _interleave(w * re, w * im).T
    return np.concatenate([fd, fi]).astype(np.float32).astype(jnp.bfloat16)


_DMAT = _constants()

_C1, _C2, _C4 = (float(np.cos(2 * np.pi * k / 9)) for k in (1, 2, 4))
_S1, _S4, _S3 = float(np.sin(2 * np.pi / 9)), float(np.sin(8 * np.pi / 9)), float(np.sqrt(3.0) / 2)


def _dft9(x):
    e1, e2, e3, e4 = x[1] + x[8], x[2] + x[7], x[3] + x[6], x[4] + x[5]
    o1, o2, o3, o4 = x[1] - x[8], x[2] - x[7], x[3] - x[6], x[4] - x[5]
    t = x[0] - 0.5 * e3
    sm = e1 + e2 + e4
    p = x[0] + e3
    d1, d2 = e1 - e4, e2 - e4
    q1 = _C1 * d1 + _C2 * d2
    q2 = _C2 * d1 + _C4 * d2
    a, b, c = o1 + o2, o2 + o4, o1 - o4
    r1 = _S1 * a + _S4 * b
    r2 = _S1 * c + _S4 * a
    v = _S3 * o3
    return (p + sm, (t + q1, r1 + v), (t + q2, r2 - v), (p - 0.5 * sm, (o1 - o2) + o4),
            ((t - q1) - q2, (r2 - r1) + v))


def _idft9(a0, z1, z2, z3, z4):
    (a1, b1), (a2, b2), (a3, b3), (a4, b4) = z1, z2, z3, z4
    o3 = _S3 * ((b1 - b2) + b4)
    r1, r2 = b1 - b4, b2 + b4
    a, b, c = _S1 * r1 + _S4 * r2, _S4 * r1, _S1 * r2
    o1, o2, o4 = (a + c) + b3, (a + b) - b3, (b - c) + b3
    t = (a1 + a2) + a4
    q1, q2 = a1 - a4, a2 - a4
    d1 = _C1 * q1 + _C2 * q2
    d2 = _C2 * q1 + _C4 * q2
    p, sm = a0 + a3, a0 - 0.5 * a3
    e1, e2, e4 = sm + d1, sm + d2, (sm - d1) - d2
    e3 = p - 0.5 * t
    return [t + p, e1 + o1, e2 + o2, e3 + o3, e4 + o4, e4 - o4, e3 - o3, e2 - o2, e1 - o1]


def _radix4(x, sign):
    t0 = (x[0][0] + x[2][0], x[0][1] + x[2][1])
    t1 = (x[0][0] - x[2][0], x[0][1] - x[2][1])
    t2 = (x[1][0] + x[3][0], x[1][1] + x[3][1])
    t3 = (x[1][0] - x[3][0], x[1][1] - x[3][1])
    plus = (t1[0] - t3[1], t1[1] + t3[0])
    minus = (t1[0] + t3[1], t1[1] - t3[0])
    y1, y3 = (plus, minus) if sign > 0 else (minus, plus)
    return [(t0[0] + t2[0], t0[1] + t2[1]), y1, (t0[0] - t2[0], t0[1] - t2[1]), y3]


def _twiddle(z, n, sign):
    re, im = z
    if n == 0:
        return z
    if n == 4:
        return (-im, re) if sign > 0 else (im, -re)
    c, s = float(np.cos(np.pi * n / 8)), sign * float(np.sin(np.pi * n / 8))
    if n in (2, 6):
        if c * s > 0:
            return (c * (re - im), c * (im + re))
        return (c * (re + im), c * (im - re))
    return (c * re - s * im, c * im + s * re)


_A_TERMS = (((0, 0), 1, (1, 1)), ((1, 0), 1, (1, 1)), ((0, 0), 0, None), ((1, 1), 0, None),
            ((0, 0), 1, (0, 1)), ((1, 0), -1, (0, 0)), ((0, 1), -1, (1, 1)))
_B_TERMS = (((0, 0), 1, (1, 1)), ((0, 0), 0, None), ((0, 1), -1, (1, 1)), ((1, 0), -1, (0, 0)),
            ((1, 1), 0, None), ((0, 0), 1, (0, 1)), ((1, 0), 1, (1, 1)))


def _add2(x, y):
    return [[x[i][j] + y[i][j] for j in range(2)] for i in range(2)]


def _sub2(x, y):
    return [[x[i][j] - y[i][j] for j in range(2)] for i in range(2)]


def _outer_operand(ld, term):
    a, s, b = term
    x = [[ld(2 * a[0] + i, 2 * a[1] + j) for j in range(2)] for i in range(2)]
    if s == 0:
        return x
    y = [[ld(2 * b[0] + i, 2 * b[1] + j) for j in range(2)] for i in range(2)]
    return _add2(x, y) if s > 0 else _sub2(x, y)


def _inner_operand(x, term):
    a, s, b = term
    if s == 0:
        return x[a[0]][a[1]]
    return x[a[0]][a[1]] + x[b[0]][b[1]] if s > 0 else x[a[0]][a[1]] - x[b[0]][b[1]]


def _inner_result(m):
    m1, m4, m2 = m(0), m(3), m(1)
    c21, c22, c11 = m2 + m4, m1 - m2, m1 + m4
    m5, m3 = m(4), m(2)
    c12, c11, c22 = m3 + m5, c11 - m5, c22 + m3
    return [[c11 + m(6), c12], [c21, c22 + m(5)]]


def _inner_block(load, bias, p1):
    def m(p2):
        v = load(7 * p1 + p2)
        if p1 in (3, 2) and p2 in (3, 2):
            v = v + bias(2 * (3 - p1) + (3 - p2))
        return v
    return _inner_result(m)


def _finish_block(finish, c, bi, bj):
    for i in range(2):
        for j in range(2):
            finish(2 * bi + i, 2 * bj + j, c[i][j])


def _recombine(load, bias, finish, tag):
    yield tag
    m2 = _inner_block(load, bias, 1)
    yield tag
    m4 = _inner_block(load, bias, 3)
    _finish_block(finish, _add2(m2, m4), 1, 0)
    yield tag
    m1 = _inner_block(load, bias, 0)
    c22, c11 = _sub2(m1, m2), _add2(m1, m4)
    yield tag
    m5 = _inner_block(load, bias, 4)
    c11 = _sub2(c11, m5)
    yield tag
    m3 = _inner_block(load, bias, 2)
    c22 = _add2(c22, m3)
    _finish_block(finish, _add2(m3, m5), 0, 1)
    yield tag
    _finish_block(finish, _add2(c11, _inner_block(load, bias, 6)), 0, 0)
    yield tag
    _finish_block(finish, _add2(c22, _inner_block(load, bias, 5)), 1, 1)


def _gelu2(x):
    c0 = float(np.sqrt(2.0 / np.pi))
    return x + x * jnp.tanh(x * (c0 + (c0 * 0.044715) * (x * x)))


def _merge(*streams, fine=False):
    streams = [us for us in streams if us]

    def whole():
        order = sorted(((i + 0.5) / len(us), k, i) for k, us in enumerate(streams) for i in range(len(us)))
        for _, k, i in order:
            costs, gen = streams[k][i]
            yield from zip(gen, costs + [None])

    def pieces():
        order = []
        for k, us in enumerate(streams):
            costs = np.array([c for u in us for c in u[0]])
            order += [(float(q) / costs.sum(), k, int(c)) for q, c in zip(np.cumsum(costs) - 0.5 * costs, costs)]
        gens = [(tag for u in us for tag in u[1]) for us in streams]
        heads = [next(g) for g in gens]
        for _, k, c in sorted(order):
            yield heads[k], c
            heads[k] = next(gens[k], None)

    return sum(sum(u[0]) for us in streams for u in us), (pieces() if fine else whole())


def _run(units):
    for _, gen in units:
        for _ in gen:
            pass


def _pack(a, b):
    return jnp.concatenate([a, b], axis=0).astype(bf16)


def _colmean(v):
    return jnp.sum(v, axis=0, keepdims=True) * (1.0 / D)


def _rows(start, n):
    return pl.ds(start if isinstance(start, int) else pl.multiple_of(start, 8), n)


def _lanes(tile):
    return pl.ds(128 * tile if isinstance(tile, int) else pl.multiple_of(128 * tile, 128), 128)


def _as_bf16(v):
    return pltpu.bitcast(v, bf16)


def _tile(v, t):
    return v[:, 128 * t:128 * t + 128]


def _start(copies):
    for cp in copies:
        cp.start()


def _wait(copies):
    for cp in copies:
        cp.wait()


def _operand_costs(terms, groups, unpack):
    out, have = [], set()
    for keep, group in groups:
        have, n = have & set(keep), 0
        for p1 in group:
            a, s, b = terms[p1]
            need = {(2 * q[0] + i, 2 * q[1] + j) for q in ((a, b) if s else (a,)) for i in range(2) for j in range(2)}
            n += unpack * len(need - have) + (8 if s else 0) + 17
            have |= need
        out.append(n)
    return out


def _quad(*blocks):
    return [(2 * a + i, 2 * b + j) for a, b in blocks for i in range(2) for j in range(2)]


_SINGLE = [((), (p,)) for p in range(7)]
_SHARED = [((), (1,)), (_quad((0, 0), (1, 1)), (5,)), (_quad((0, 0), (1, 1), (0, 1)), (4, 2)),
           (_quad((0, 0), (1, 1)), (0, 6)), (_quad((0, 0), (1, 1), (1, 0)), (3,))]
_OUTER_ORDER = (1, 3, 0, 4, 2, 6, 5)
G = {"S": _SINGLE, "H": _SHARED}

_B1, _B2 = 6 * D, 6 * D + 8 * 36
_HA = _B2 + 8 * 16
_AR_TICK = _HA + 4 * D
_S_SMALL, _S_X, _S_MOD, _S_DMAT, _S_WF, _S_STAGE, _S_WIDE, _S_OUT, _N_SEM = 0, 1, 5, 10, 12, 15, 17, 18, 19


def _kernel(x_hbm, wr_hbm, wi_hbm, w1_hbm, b1_hbm, w2_hbm, b2_hbm, c_hbm, wmod_hbm, dmat_hbm, zero_hbm,
            out_hbm,
            zero_s, st0, st1, uc_v, bc0, bc1, mm0, mm1, uu_v, x2_v, ar_v, io_v, sem):
    copy = pltpu.make_async_copy
    state = {}

    def tick(target, val):
        ref, idx, row = target
        if ref.dtype == bf16 and ref.shape[-2] % 2:
            ref[idx + (pl.ds(pl.multiple_of(row + state["zero"], 8), 8), pl.ds(0, 128))] = val.astype(bf16)
            return
        ref = ref.bitcast(u32) if ref.dtype == bf16 else ref
        ref[idx + (pl.ds(pl.multiple_of(row + state["zero"], 8), 8), pl.ds(0, 128))] = pltpu.bitcast(val, ref.dtype)

    def paced(main, points, side, lead):
        total, gen = side
        pending, done = next(gen, None), 0
        for _ in range(lead):
            if pending is not None:
                pending, done = next(gen, None), done + pending[1]
        for pt, v in enumerate(main, 1):
            seen = []
            while pending is not None and done * points < pt * total:
                if not any(pending[0] is t for t in seen):
                    seen.append(pending[0])
                    tick(pending[0], v)
                pending, done = next(gen, None), done + pending[1]
        assert pending is None

    def chained(units, target, lag):
        late = []
        for k, unit in enumerate(units):
            if k >= lag:
                for v in late[k - lag]:
                    tick(target, v)
            late.append(unit())

    t_uu, t_ar = (uu_v, (), 16 * MB), (ar_v, (), _AR_TICK)
    t_mm = [(mm0, (), NP * MB), (mm1, (), NP * MB)]
    t_st = [(st0, (), 4 * STAGE), (st1, (), 4 * STAGE)]
    bcs = (bc0, bc1)

    def stage_copies(par, src, row, tile, depth=4):
        return [copy(src.bitcast(u32).at[pl.ds(row, 256 * depth), _lanes(tile + j)],
                     t_st[par][0].at[pl.ds(j * STAGE, 256 * depth)], sem.at[_S_STAGE + par]) for j in range(4)]

    def stage_wait(par, depth=4):
        whole = t_st[par][0].at[pl.ds(0, 4 * 256 * depth)]
        copy(whole, whole, sem.at[_S_STAGE + par]).wait()

    def operand_unit(target, raw, load, terms, groups, put):
        cache = {}
        for keep, group in groups:
            yield target
            cache = {k: v for k, v in cache.items() if k in keep}

            def ld(i, j):
                if (i, j) not in cache:
                    cache[i, j] = load(i, j)
                return cache[i, j]

            for p1 in group:
                t1 = terms[p1]
                x = _outer_operand(ld, t1)
                for p2, t2 in enumerate(terms):
                    if raw is not None and t1[1] == 0 and t2[1] == 0:
                        put(7 * p1 + p2, raw(2 * t1[0][0] + t2[0][0], 2 * t1[0][1] + t2[0][1]))
                    else:
                        put(7 * p1 + p2, _inner_operand(x, t2).astype(bf16))

    def weight_units(par, groups, source=None, depth=4):
        target, bc = source or t_st[par], bcs[par]

        def unit(ru):
            def raw(k, j):
                return target[0][pl.ds(j * STAGE + 256 * (ru // 8) + 64 * k + 8 * (ru % 8), 8), :]

            def put(p, v):
                if v.dtype == u32:
                    bc.bitcast(u32)[p, pl.ds(8 * ru, 8), :] = v
                else:
                    bc[p, pl.ds(16 * ru, 16), :] = v
            return operand_unit(target, raw, lambda k, j: _as_bf16(raw(k, j)).astype(f32), _B_TERMS, groups, put)
        return [(_operand_costs(_B_TERMS, groups, 2), unit(ru)) for ru in range(8 * depth)]

    def hidden_units(c, par):
        target = t_mm[par]

        def first(r8):
            def finish(i, j, v):
                uu_v[pl.ds((4 * i + j) * MB + 8 * r8, 8), :] = _gelu2(v)
            return _recombine(lambda p: target[0][pl.ds(p * MB + 8 * r8, 8), :],
                              lambda j: ar_v[_rows(_B1 + 8 * (4 * c + j), 8), :], finish, target)

        def second(r):
            def put(p, v):
                uc_v[p * NCH + c, pl.ds(16 * r, 16), :] = v
            return operand_unit(t_uu, None, lambda i, j: uu_v[pl.ds((4 * i + j) * MB + 16 * r, 16), :],
                                _A_TERMS, _SINGLE, put)

        units, cost = [], [8, 38, 16, 12, 42, 36, 36]
        for r in range(MB // 16):
            units += [(cost, first(2 * r)), (cost, first(2 * r + 1)),
                      (_operand_costs(_A_TERMS, _SINGLE, 0), second(r))]
        return units

    def products(product, outer, side):
        main = (v for p1 in outer for p2 in range(7) for v in product(7 * p1 + p2))
        points = 7 * len(outer) * (MB // 16)
        paced(main, points - max(2, points // 40), side, lead=3 if len(outer) == 7 else 1)

    def deep_product(lhs_ref, slot, bc, dst, init=None, depth=4):
        lhs_u, bc_u = lhs_ref.bitcast(u32), bc.bitcast(u32)

        def product(p):
            lhs = jnp.concatenate([_as_bf16(lhs_u[slot(p, t)]) for t in range(depth)], axis=1)
            v = jnp.dot(lhs, _as_bf16(bc_u[p, pl.ds(0, 64 * depth), :]), preferred_element_type=f32)
            for r in range(MB // 16):
                blk = v[16 * r:16 * r + 16]
                if init is not None:
                    blk = blk + init(p, r)
                dst[pl.ds(p * MB + 16 * r, 16), :] = blk
                yield blk[:8]
        return product

    def first_half(wide_v, ac_v, wmod_v, dmat_v, gmat_u, wf_v, wt_v, uv_v, bb_v, ee_v, sa_v, c_v, b1_v, b2_v):
        small_copies = [copy(c_hbm, c_v, sem.at[_S_SMALL]), copy(zero_hbm, zero_s, sem.at[_S_SMALL]),
                        copy(b1_hbm, b1_v, sem.at[_S_SMALL]), copy(b2_hbm, b2_v, sem.at[_S_SMALL])]
        x_copies = lambda a: [copy(x_hbm.at[:, _lanes(a + 4 * b)], io_v.at[a + 4 * b], sem.at[_S_X + a])
                              for b in range(4)]
        mod_tiles = ((4, 9), (0, 4), (9, 27))
        wmod_copies = [copy(wmod_hbm.at[:, pl.ds(128 * t0, 128 * (t1 - t0))],
                            wmod_v.at[:, pl.ds(128 * t0, 128 * (t1 - t0))], sem.at[_S_MOD + h])
                       for h, (t0, t1) in enumerate(mod_tiles)]
        dmat_copies = [copy(dmat_hbm.at[pl.ds(5 * h, 5)], dmat_v.at[pl.ds(5 * h, 5)], sem.at[_S_DMAT + h])
                       for h in range(2)]
        wf_rows = ((0, 96), (96, 96), (192, DF - 192))
        wf_copies = [[copy(src.at[pl.ds(*rows)], wf_v.at[a, pl.ds(*rows)], sem.at[_S_WF + h])
                      for a, src in enumerate((wr_hbm, wi_hbm))] for h, rows in enumerate(wf_rows)]
        def mm1_step(c, par):
            products(deep_product(ac_v, lambda p, t: 4 * p + t, bcs[par], t_mm[par][0]), range(7),
                     _merge(weight_units(1 - par, G["S"]), hidden_units(c - 1, 1 - par),
                            fine=bool(0)))

        late_copies = [wmod_copies[1]] + sum(wf_copies, []) + [dmat_copies[1]] + wmod_copies[2:]
        _start(small_copies + [wmod_copies[0], dmat_copies[0]] + x_copies(0) + x_copies(1) + x_copies(2)
               + x_copies(3) + ([] if 0 else late_copies))

        _wait(small_copies)
        state["zero"] = zero_s[0]
        s0 = jax.lax.broadcasted_iota(jnp.int32, (16, 128), 0)
        j0 = jax.lax.broadcasted_iota(jnp.int32, (16, 128), 1)
        j0 = 8 * (j0 & 15) + (j0 >> 4)
        phasor = lambda n, period: (jnp.cos(n.astype(f32) * (-2 * np.pi / period)),
                                    jnp.sin(n.astype(f32) * (-2 * np.pi / period)))
        cmul = lambda x, y: (x[0] * y[0] - x[1] * y[1], x[0] * y[1] + x[1] * y[0])
        base, rot, down = phasor((s0 * j0) & 127, 128), phasor(s0, S), phasor(j0[:1] & 7, 8)

        def generate(i, carry):
            for r in range(2):
                g, rows = carry[:2], _rows(8 * (2 * i + r), 8)
                for j1 in range(16):
                    for q in range(2):
                        v = pltpu.bitcast(g[q].astype(bf16), u32)
                        gmat_u[2 * j1 + q, rows, :] = pltpu.roll(v, j1, 1) if j1 else v
                    g = cmul(g, carry[2:])
                carry = cmul(carry[:2], down) + cmul(carry[2:], (float(np.cos(np.pi / 64)), float(-np.sin(np.pi / 64))))
            return carry

        jax.lax.fori_loop(0, 8 // 2, generate, base + rot)
        for t in range(20, 24):
            io_v[t] = jnp.zeros((D, 128), bf16)
        bb_u = bb_v.bitcast(u32)


        cv = c_v[...].astype(f32)
        sc = jnp.broadcast_to(cv * jax.nn.sigmoid(cv), (16, D)).astype(bf16)
        b1 = b1_v[...].astype(f32).reshape(1, F)
        for t in range(36):
            ar_v[pl.ds(_B1 + 8 * t, 8), :] = jnp.broadcast_to(_tile(b1, t), (8, 128))
        b2 = 2.0 * b2_v[...].astype(f32).reshape(1, S)
        for t in range(16):
            ar_v[pl.ds(_B2 + 8 * t, 8), :] = jnp.broadcast_to(_tile(b2, t), (8, 128))

        def modulation(t0, n):
            cols = pl.ds(128 * t0 if isinstance(t0, int) else pl.multiple_of(128 * t0, 128), 128 * n)
            m = jnp.dot(sc, wmod_v[:, cols], preferred_element_type=f32)[:8]
            for q in range(n):
                col = 128 * (t0 + q) + jax.lax.broadcasted_iota(jnp.int32, (8, 128), 1)
                v = _tile(m, q)
                scale = ((col >= D) & (col < 2 * D)) | ((col >= 4 * D) & (col < 5 * D))
                v = jnp.where(scale, 1.0 + v, v)
                v = jnp.where(col >= 5 * D, 0.5 * v, v)
                ar_v[_rows(128 * (t0 + q), 128), :] = jnp.concatenate([v] * 16, axis=0).T

        wmod_copies[0].wait()
        modulation(4, 5)
        dmat_u, io_u = dmat_v.bitcast(u32), io_v.bitcast(u32)
        t_io, t_uv, t_x2 = (io_v, (24,), 0), (uv_v, (16,), 0), (x2_v, (), 16 * D)

        fold = lambda v: v.reshape(8, 8, 128).sum(axis=0)

        def dft9_tiles(h, r, held):
            z = _dft9(h)
            out = [(128 * g + 16 * r, _pack(*z[g + 1])) for g in range(4)]
            if r % 2:
                out.append((512 + 8 * (r - 1), _pack(held.pop(), z[0])))
            else:
                held.append(z[0])
            return out

        def put(slot, tiles):
            for row, v in tiles:
                io_v[slot, pl.ds(row, 16), :] = v

        def channel_dft(g, slots):
            n = 64 if g < 4 else 32
            lhs = _as_bf16(dmat_u[g] if g < 4 else dmat_u[4, pl.ds(0, 40), pl.ds(0, 64)])
            rhs = jnp.concatenate([_as_bf16(io_u[t, pl.ds(64 * g, n), :]) for t in slots], axis=1)
            return jnp.dot(lhs, rhs, preferred_element_type=f32)

        def spectrum(a, rstd, ordered=True):
            slots = [16 + 4 * (a % 2) + b for b in range(4)]
            nxt = channel_dft(0, slots)
            for g in range(5):
                yield
                v, nxt = nxt, (channel_dft(g + 1, slots) if g < 4 else None)
                for half in range(2):
                    yield
                    for r in range(4 * half, min(4 * half + 4, NRG[g])):
                        z = [(_tile(v[16 * r:16 * r + 8], b) * rstd[b], _tile(v[16 * r + 8:16 * r + 16], b) * rstd[b])
                             for b in range(4)]
                        for c, y in enumerate(_radix4(z, -1)):
                            uv_v[4 * a + c, pl.ds(128 * g + 16 * r, 16), :] = jnp.concatenate(y, axis=0)
                        if ordered and r % 2 == 2 - 1:
                            tick(t_io, y[1])

        def phase_a(a, rstd_prev):
            _wait(x_copies(a))
            behind = spectrum((a + 3) % 4, rstd_prev)
            if 1:
                total = jnp.dot(jnp.ones((16, D), bf16),
                                jnp.concatenate([_as_bf16(io_u[a + 4 * b]) for b in range(4)], axis=1),
                                preferred_element_type=f32)
                mean = [_tile(total[:8], b) * (1.0 / D) for b in range(4)]
                next(behind, None)
            else:
                next(behind, None)
                mean = [_colmean(fold(_as_bf16(io_u[a + 4 * b]).astype(f32).reshape(9, 64, 128).sum(axis=0)))
                        for b in range(4)]
            sq, queue = [0.0] * 4, []
            for b in range(4):
                held, slot = [], 16 + 4 * (a % 2) + b
                if b:
                    tick(t_ar, sq[b - 1])
                for r in range(8):
                    if r % 2 == 0:
                        xp = [io_u[a + 4 * b, pl.ds(32 * i + 4 * r, 8), :] for i in range(9)]
                        for emit in queue:
                            emit()
                        queue = []
                        if 4 * b + r // 2 >= 1:
                            next(behind, None)
                        xp = [_as_bf16(v).astype(f32) for v in xp]
                    h = []
                    for i in range(9):
                        d = xp[i][8 * (r % 2):8 * (r % 2) + 8] - mean[b]
                        sq[b] = sq[b] + d * d
                        h.append(d * ar_v[pl.ds(D + 64 * i + 8 * r, 8), :])
                    tiles = dft9_tiles(h, r, held)
                    if r % 2 == 0:
                        put(slot, tiles)
                    else:
                        queue.append(lambda slot=slot, tiles=tiles, q=sq[b]: (put(slot, tiles), tick(t_io, q)))
            for _ in behind:
                pass
            for emit in queue:
                emit()
            return tuple(jnp.broadcast_to(jax.lax.rsqrt(_colmean(q) + 1e-5), (8, 128)) for q in sq)

        dmat_copies[0].wait()
        rstd_last = jax.lax.fori_loop(0, 4, phase_a, (jnp.zeros((8, 128), f32),) * 4)
        wmod_copies[1].wait()
        modulation(0, 4)
        for _ in spectrum(3, rstd_last, ordered=False):
            pass
        for q in range(32):
            gmat_u[32 + q] = pltpu.bitcast(_as_bf16(gmat_u[q]).T, u32)
        held = []
        for r in range(8):
            put(16, dft9_tiles([float(S) * ar_v[pl.ds(64 * i + 8 * r, 8), :] for i in range(9)], r, held))
        for g in range(5):
            v = channel_dft(g, [16])
            first = jax.lax.broadcasted_iota(jnp.int32, v.shape, 1) == 0
            sa_v[pl.ds(128 * g, 16 * NRG[g]), :] = jnp.where(first, v, 0.0)


        def pair_at(j, row):
            return uv_v[j, pl.ds(row, 8), :], uv_v[j, pl.ds(row + 8, 8), :]

        def butterflies(g, r):
            row = 128 * g + 16 * r
            for c in range(4):
                yield t_uv
                z = [_twiddle(pair_at(4 * a + c, row), a * c, -1) for a in range(4)]
                for e, y in enumerate(_radix4(z, -1)):
                    bb_v[c + 4 * e, pl.ds(row, 16), :] = _pack(*y)

        def token_dft(g, inverse):
            n = NRG[g]
            for j1 in range(16):
                rhs = jnp.concatenate([_as_bf16(gmat_u[32 * inverse + 2 * j1 + i]) for i in range(2)], axis=1)
                v = jnp.dot(_as_bf16(bb_u[j1, pl.ds(64 * g, 8 * n), :]), rhs, preferred_element_type=f32)
                for r in range(n):
                    top, bot = v[16 * r:16 * r + 8], v[16 * r + 8:16 * r + 16]
                    if inverse:
                        re, im = _tile(top, 0) + _tile(bot, 1), _tile(bot, 0) - _tile(top, 1)
                    else:
                        re, im = _tile(top, 0) - _tile(bot, 1), _tile(bot, 0) + _tile(top, 1)
                    uv_v[j1, pl.ds(128 * g + 16 * r, 16), :] = jnp.concatenate([re, im], axis=0)
                    yield re

        lane = jax.lax.broadcasted_iota(jnp.int32, (8, 128), 1)

        def filt(a, j1, g, r):
            if g < 4:
                first = (g + 1 if r < 4 else 8 - g) + 72 * (r % 4)
                return wt_v[16 * a + j1, pl.ds(first, 8, stride=9), :]
            if r < 4:
                return wt_v[16 * a + j1, pl.ds(72 * r, 8, stride=9), :]
            return wt_v[16 * a + j1, pl.ds(288, 8), :]

        def filtering(g, j1):
            for r in range(NRG[g]):
                if r % 4 == 0:
                    yield t_uv
                row = 128 * g + 16 * r
                yr, yi = pair_at(j1, row)
                if j1 == 0:
                    yr, yi = yr + sa_v[pl.ds(row, 8), :], yi + sa_v[pl.ds(row + 8, 8), :]
                wr, wi = filt(0, j1, g, r), filt(1, j1, g, r)
                bb_v[j1, pl.ds(row, 16), :] = _pack(yr * wr - yi * wi, yr * wi + yi * wr)

        def inverse_butterflies(g, r):
            row = 128 * g + 16 * r
            mid = [[None] * 4 for _ in range(4)]
            for c in range(4):
                yield t_uv
                for a, y in enumerate(_radix4([pair_at(c + 4 * e, row) for e in range(4)], 1)):
                    mid[a][c] = _twiddle(y, a * c, 1)
            for a in range(4):
                for b, y in enumerate(_radix4(mid[a], 1)):
                    bb_v[a + 4 * b, pl.ds(row, 16), :] = _pack(*y)

        bfly = lambda g: [([20, 36, 28, 36], butterflies(g, r)) for r in range(NRG[g])] if g < 5 else []
        filts = lambda g: [([28, 7 * (NRG[g] - 4)], filtering(g, j1)) for j1 in range(16)] if g < 5 else []
        ibfly = lambda g: [([16, 32, 24, 112], inverse_butterflies(g, r)) for r in range(NRG[g])] if g >= 0 else []

        masks = [(lane & (1 << i)) != 0 for i in range(4)]

        def regroup(tiles):
            t = [pltpu.roll(v, b, 1) if b else v for b, v in enumerate(tiles)]
            t = [t[-i % 16] for i in range(16)]
            for i in range(4):
                t = [jnp.where(masks[i], t[(j - (1 << i)) % 16], t[j]) for j in range(16)]
            return t

        def regroup_unit(a, r):
            yield t_wf
            if r < 18:
                tiles = [pltpu.bitcast(wf_v[a, pl.ds(16 * r, 16), pl.ds(128 * b, 128)], u32) for b in range(16)]
                for j1, v in enumerate(regroup(tiles)):
                    wt_v[16 * a + j1, pl.ds(16 * r, 16), :] = _as_bf16(v).astype(f32)
            else:
                last = jnp.broadcast_to(wf_v[a, pl.ds(288, 1), :].astype(f32), (8, S))
                for j1, v in enumerate(regroup([_tile(last, b) for b in range(16)])):
                    wt_v[16 * a + j1, pl.ds(288, 8), :] = v

        t_wf = (wf_v, (2,), 0)
        regroups = lambda h: [([112], regroup_unit(a, r)) for r in range(6 * h, 6 * h + 6 + h // 2) for a in range(2)]
        when = {int(q): h for h, q in enumerate("123")}

        _run(bfly(0))
        for g in range(5):
            if g in when:
                _wait(wf_copies[when[g]])
            if str(g) in "":
                tick((bb_v, (16,), 0), jnp.zeros((8, 128), f32))
            paced(token_dft(g, 0), 16 * NRG[g] - 24,
                  _merge(bfly(g + 1) or filts(0), regroups(when[g]) if g in when else [], fine=bool(1)), lead=1)
        first_rows = wide_v.at[pl.ds(0, 4096)]
        _start([copy(w1_hbm.bitcast(u32).at[:, _lanes(j)], wide_v.at[pl.ds(j * STAGE, 1024)], sem.at[_S_WIDE])
                for j in range(4)] + stage_copies(1, w1_hbm, 0, 4) + stage_copies(0, w1_hbm, 0, 8))

        for g in range(5):
            if str(g) in "":
                tick((bb_v, (16,), 0), jnp.zeros((8, 128), f32))
            side = (_merge(filts(g + 1) + ibfly(g - 1)) if 2 == 2 else
                    _merge(filts(g + 1), ibfly(g - 1), fine=bool(2)))
            paced(token_dft(g, 1), 16 * NRG[g] - 8, side, lead=1)
        _wait([dmat_copies[1]] + wmod_copies[2:])
        modulation(9, 18)
        _run(ibfly(4))
        shift = ar_v[pl.ds(3 * D, D), :]
        ar_v[pl.ds(3 * D, D), :] = shift - _colmean(fold(shift.reshape(9, 64, 128).sum(axis=0)))

        for a in range(4):
            rhs = jnp.concatenate([_as_bf16(bb_u[4 * a + b, pl.ds(256, 40), :]) for b in range(4)], axis=1)
            v = jnp.dot(_as_bf16(dmat_u[9, pl.ds(0, 32), pl.ds(0, 80)]), rhs, preferred_element_type=f32)
            for b in range(4):
                ee_v[pl.ds(64 * (4 * a + b), 64), :] = _tile(v, b)

        def phase_c(a, carry):
            acc = [0.0] * 4
            for b in range(4):
                t = 4 * a + b
                v = [jnp.dot(_as_bf16(dmat_u[5 + g]), _as_bf16(bb_u[4 * a + b, pl.ds(64 * g, 64), :]),
                             preferred_element_type=f32) for g in range(4)]
                for r in range(8):
                    if r % 2 == 0:
                        xres = [_as_bf16(io_u[t, pl.ds(32 * i + 4 * r, 8), :]).astype(f32) for i in range(9)]
                    z = [(q[16 * r:16 * r + 8], q[16 * r + 8:16 * r + 16]) for q in v]
                    y = _idft9(ee_v[_rows(64 * (4 * a + b) + 8 * r, 8), :], *z)
                    for i in range(9):
                        row = 64 * i + 8 * r
                        x2 = xres[i][8 * (r % 2):8 * (r % 2) + 8] + ar_v[pl.ds(2 * D + row, 8), :] * y[i]
                        x2_v[_rows(t * D + row, 8), :] = x2
                        acc[b] = acc[b] + x2
                    if r % 2 == 0:
                        tick(t_io, acc[b])
            mean = [_colmean(v) for v in acc]
            sq, lin, sq2 = [0.0] * 4, [0.0] * 4, [0.0] * 4

            def second(b, i):
                d = x2_v[_rows((4 * a + b) * D + 64 * i, 64), :] - mean[b]
                w = d * ar_v[pl.ds(4 * D + 64 * i, 64), :]
                ar_v[pl.ds(_HA + b * D + 64 * i, 64), :] = w
                sq[b], lin[b] = sq[b] + fold(d * d), lin[b] + fold(w)
                return sq[b], lin[b]

            chained([lambda b=b, i=i: second(b, i) for b in range(4) for i in range(9)], t_x2, lag=5)
            rstd = [jax.lax.rsqrt(_colmean(v) + 1e-5) for v in sq]
            mean = [_colmean(v) for v in lin]

            def third(b, i):
                h = ((ar_v[pl.ds(_HA + b * D + 64 * i, 64), :] - mean[b]) * rstd[b]
                     + ar_v[pl.ds(3 * D + 64 * i, 64), :])
                uu_v[pl.ds(b * D + 64 * i, 64), :] = h
                sq2[b] = sq2[b] + fold(h * h)
                return sq2[b],

            chained([lambda b=b, i=i: third(b, i) for b in range(4) for i in range(9)], t_ar, lag=5)
            rstd = [jax.lax.rsqrt(_colmean(v) + 1e-5) for v in sq2]

            def operands(r):
                blk = [[uu_v[pl.ds(k * D + i * MB + 16 * r, 16), :] * rstd[k] for k in range(4)] for i in range(4)]
                for p1, t1 in enumerate(_A_TERMS):
                    x = _outer_operand(lambda i, k: blk[i][k], t1)
                    for p2, t2 in enumerate(_A_TERMS):
                        v = _inner_operand(x, t2)
                        ac_v[4 * (7 * p1 + p2) + a, pl.ds(16 * r, 16), :] = v.astype(bf16)
                    if p1 == 2:
                        late = v[:8]
                return late,

            chained([lambda r=r: operands(r) for r in range(MB // 16)], t_uu, lag=1)
            return carry

        jax.lax.fori_loop(0, 4, phase_c, 0)

        copy(first_rows, first_rows, sem.at[_S_WIDE]).wait()
        stage_wait(1)
        own = lambda k: (weight_units(0, [((), (_OUTER_ORDER[k],))], source=(wide_v, (), 4 * STAGE))
                         if k < 7 else [])
        ahead = weight_units(1, G['H'])
        product = deep_product(ac_v, lambda p, t: 4 * p + t, bc0, mm0)
        _run(own(0))
        for k, p1 in enumerate(_OUTER_ORDER):
            tick((bc0, (NP,), 0), jnp.zeros((8, 128), f32))
            products(product, [p1], _merge(own(k + 1) + (ahead[4 * k:4 * k + 4] if k < 6 else ahead[24:])))

        def mm1_pair(i, carry):
            c = 2 * i + 1

            @pl.when(i < 3)
            def _():
                _start(stage_copies(1, w1_hbm, 0, 4 * (c + 2)))

            @pl.when(i == 3)
            def _():
                _start(stage_copies(1, w2_hbm, 0, 0))

            stage_wait(0)
            mm1_step(c, 1)

            @pl.when(i < 3)
            def _():
                _start(stage_copies(0, w1_hbm, 0, 4 * (c + 3)))

            @pl.when(i == 3)
            def _():
                _start(stage_copies(0, w2_hbm, 1024, 0, 5))

            stage_wait(1)
            mm1_step(c + 1, 0)
            return carry

        jax.lax.fori_loop(0, 4, mm1_pair, 0)

    pl.run_scoped(
        first_half,
        pltpu.VMEM((4 * STAGE + 8, 128), u32),
        pltpu.VMEM((4 * NP, MB, 128), bf16),
        pltpu.VMEM((D, 6 * D), bf16),
        pltpu.VMEM((10, 128, 128), bf16),
        pltpu.VMEM((64, 64, 128), u32),
        pltpu.VMEM((3, DF, S), bf16),
        pltpu.VMEM((32, 296, 128), f32),
        pltpu.VMEM((17, 592, 128), f32),
        pltpu.VMEM((17, 592, 128), bf16),
        pltpu.VMEM((16 * 64, 128), f32),
        pltpu.VMEM((592, 128), f32),
        pltpu.VMEM((1, D), bf16),
        pltpu.VMEM((F,), bf16),
        pltpu.VMEM((S,), bf16),
    )

    state["zero"] = zero_s[0]

    def quadrant(n, which, r8):
        def finish(i, j, v):
            row = i * MB + 8 * r8
            res = x2_v[_rows((4 * n + j) * D + row, 8), :]
            io_v[4 * n + j, pl.ds(row, 8), :] = (res + ar_v[pl.ds(5 * D + row, 8), :] * v).astype(bf16)

        m = lambda p1: _inner_block(lambda p: mm0[pl.ds(p * MB + 8 * r8, 8), :],
                                    lambda j: ar_v[_rows(_B2 + 8 * (4 * n + j), 8), :], p1)
        spot = lambda i, j: pl.ds((2 * i + j) * MB + 8 * r8, 8)
        yield t_mm[0]
        if which == 0:
            _finish_block(finish, _add2(m(1), m(3)), 1, 0)
        elif which == 1:
            m3 = m(2)
            _finish_block(finish, _add2(m3, m(4)), 0, 1)
            yield t_mm[0]
            part = _add2(_sub2(m(0), m(1)), m3)
            for i in range(2):
                for j in range(2):
                    uu_v[spot(i, j), :] = part[i][j]
        elif which == 2:
            part = _add2(m(0), m(3))
            yield t_mm[0]
            _finish_block(finish, _add2(_sub2(part, m(4)), m(6)), 0, 0)
        else:
            part = [[uu_v[spot(i, j), :] for j in range(2)] for i in range(2)]
            _finish_block(finish, _add2(part, m(5)), 1, 1)

    def quadrants(n, which):
        return [([[34], [34, 24], [20, 36], [24]][which], quadrant(n, which, r8)) for r8 in range(MB // 8)]

    def out_copies(n, which):
        bi, bj = ((1, 0), (0, 1), (0, 0), (1, 1))[which]
        rows = pl.ds(bi * (D // 2), D // 2)
        return [copy(io_v.at[4 * n + 2 * bj + j, rows], out_hbm.at[rows, _lanes(4 * n + 2 * bj + j)], sem.at[_S_OUT])
                for j in range(2)]

    def mm2_pair(n, carry):
        @pl.when(n < 3)
        def _():
            _start(stage_copies(1, w2_hbm, 0, 4 * n + 4))

        stage_wait(0, 5)
        first = deep_product(uc_v, lambda p, t: p * NCH + t, bc1, mm1)

        @pl.when(n == 0)
        def _():
            products(first, range(7), _merge(weight_units(0, G["S"], depth=5), hidden_units(NCH - 1, 0),
                                             fine=bool(1)))

        @pl.when(n > 0)
        def _():
            products(first, range(7), _merge(weight_units(0, G["S"], depth=5), quadrants(n - 1, 3),
                                             fine=bool(1)))
            _start(out_copies(n - 1, 3))

        @pl.when(n < 3)
        def _():
            _start(stage_copies(0, w2_hbm, 1024, 4 * n + 4, 5))
            stage_wait(1)

        second = deep_product(uc_v, lambda p, t: p * NCH + 4 + t, bc0, mm0,
                              lambda p, r: mm1[pl.ds(p * MB + 16 * r, 16), :], depth=5)
        ahead = weight_units(1, G["S"])
        fine = bool(0)
        products(second, _OUTER_ORDER[:2], _merge(ahead[:11]))
        products(second, _OUTER_ORDER[2:5], _merge(ahead[11:25], quadrants(n, 0), fine=fine))
        products(second, _OUTER_ORDER[5:6], _merge(ahead[25:28], quadrants(n, 1), fine=fine))
        products(second, _OUTER_ORDER[6:], _merge(ahead[28:], quadrants(n, 2), fine=fine))
        _start(out_copies(n, 0) + out_copies(n, 1) + out_copies(n, 2))
        return carry

    jax.lax.fori_loop(0, 4, mm2_pair, 0)
    _run(quadrants(3, 3))
    _start(out_copies(3, 3))
    copy(out_hbm, out_hbm, sem.at[_S_OUT]).wait()


@jax.jit
def pallas_adaLN_cond__spectral_gfnet__mixer_token_mlp__prompt_kernel(
    A_x: jax.Array,
    A_w_r: jax.Array,
    A_w_i: jax.Array,
    B_x: jax.Array,
    B_w1: jax.Array,
    B_b1: jax.Array,
    B_w2: jax.Array,
    B_b2: jax.Array,
    c: jax.Array,
    w_mod: jax.Array,
):
    del B_x
    hbm = pl.BlockSpec(memory_space=pl.ANY)
    out = pl.pallas_call(
        _kernel,
        out_shape=jax.ShapeDtypeStruct((D, S), bf16),
        in_specs=[hbm] * 11,
        out_specs=hbm,
        scratch_shapes=[
            pltpu.SMEM((1,), jnp.int32),
            pltpu.VMEM((4 * STAGE + 8, 128), u32),
            pltpu.VMEM((4 * STAGE + 8, 128), u32),
            pltpu.VMEM((NP * NCH, MB, 128), bf16),
            pltpu.VMEM((NP + 1, 640, 128), bf16),
            pltpu.VMEM((NP, 512, 128), bf16),
            pltpu.VMEM((NP * MB + 8, 128), f32),
            pltpu.VMEM((NP * MB + 8, 128), f32),
            pltpu.VMEM((16 * MB + 8, 128), f32),
            pltpu.VMEM((16 * D + 8, 128), f32),
            pltpu.VMEM((_AR_TICK + 8, 128), f32),
            pltpu.VMEM((25, D, 128), bf16),
            pltpu.SemaphoreType.DMA((_N_SEM,)),
        ],
        compiler_params=pltpu.CompilerParams(vmem_limit_bytes=126 * 1024 * 1024),
        name="adaln_gfnet_mixer",
    )(A_x.reshape(S, D).T, A_w_r.T, A_w_i.T, B_w1, B_b1, B_w2, B_b2, c, w_mod, _DMAT,
      np.zeros((1,), np.int32))
    return out.T.reshape(1, S, D)
```

```python
import numpy as np
import jax
import jax.numpy as jnp
import jax.experimental.pallas as pl
import jax.experimental.pallas.tpu as pltpu

S, D, F = 2048, 576, 4608
DF = D // 2 + 1
NP = 49
MB = D // 4
NCH = F // 512
NRG = (8, 8, 8, 8, 5)
STAGE = 1280

f32, u32, bf16 = jnp.float32, jnp.uint32, jnp.bfloat16


def _interleave(a, b):
    n = a.shape[0] // 8
    return np.stack([a.reshape(n, 8, -1), b.reshape(n, 8, -1)], axis=1).reshape(16 * n, -1)


def _constants():
    d0 = np.arange(64)
    fd = np.zeros((5, 128, 128))
    fi = np.zeros((5, 128, 128))
    scale = 1.0 / (S * D)
    for k1 in range(1, 5):
        k = np.array([k1 + 9 * m for m in range(32)] + [9 - k1 + 9 * m for m in range(32)])
        sg = np.array([1.0] * 32 + [-1.0] * 32)[:, None]
        ang = 2 * np.pi * np.outer(k, d0) / D
        c, s = np.cos(ang), np.sin(ang)
        q = np.sqrt(3.0) / 2 if k1 == 3 else 1.0
        re = _interleave(c.T, (-q * sg * s).T).T
        im = _interleave(-s.T, (-q * sg * c).T).T
        fd[k1 - 1] = _interleave(re, im)
        fi[k1 - 1] = 2 * scale * fd[k1 - 1].T
    ang = 2 * np.pi * np.outer(9 * np.arange(33), d0) / D
    re, im = np.zeros((40, 64)), np.zeros((40, 64))
    re[:33], im[:33] = np.cos(ang), -np.sin(ang)
    im[0] = im[32] = 0.0
    w = np.full((40, 1), 2.0)
    w[0] = w[32] = 1.0
    fd[4, :80, :64] = _interleave(re, im)
    fi[4, :64, :80] = scale * _interleave(w * re, w * im).T
    return np.concatenate([fd, fi]).astype(np.float32).astype(jnp.bfloat16)


_DMAT = _constants()

_C1, _C2, _C4 = (float(np.cos(2 * np.pi * k / 9)) for k in (1, 2, 4))
_S1, _S4, _S3 = float(np.sin(2 * np.pi / 9)), float(np.sin(8 * np.pi / 9)), float(np.sqrt(3.0) / 2)


def _dft9(x):
    e1, e2, e3, e4 = x[1] + x[8], x[2] + x[7], x[3] + x[6], x[4] + x[5]
    o1, o2, o3, o4 = x[1] - x[8], x[2] - x[7], x[3] - x[6], x[4] - x[5]
    t = x[0] - 0.5 * e3
    sm = e1 + e2 + e4
    p = x[0] + e3
    d1, d2 = e1 - e4, e2 - e4
    q1 = _C1 * d1 + _C2 * d2
    q2 = _C2 * d1 + _C4 * d2
    a, b, c = o1 + o2, o2 + o4, o1 - o4
    r1 = _S1 * a + _S4 * b
    r2 = _S1 * c + _S4 * a
    v = _S3 * o3
    return (p + sm, (t + q1, r1 + v), (t + q2, r2 - v), (p - 0.5 * sm, (o1 - o2) + o4),
            ((t - q1) - q2, (r2 - r1) + v))


def _idft9(a0, z1, z2, z3, z4):
    (a1, b1), (a2, b2), (a3, b3), (a4, b4) = z1, z2, z3, z4
    o3 = _S3 * ((b1 - b2) + b4)
    r1, r2 = b1 - b4, b2 + b4
    a, b, c = _S1 * r1 + _S4 * r2, _S4 * r1, _S1 * r2
    o1, o2, o4 = (a + c) + b3, (a + b) - b3, (b - c) + b3
    t = (a1 + a2) + a4
    q1, q2 = a1 - a4, a2 - a4
    d1 = _C1 * q1 + _C2 * q2
    d2 = _C2 * q1 + _C4 * q2
    p, sm = a0 + a3, a0 - 0.5 * a3
    e1, e2, e4 = sm + d1, sm + d2, (sm - d1) - d2
    e3 = p - 0.5 * t
    return [t + p, e1 + o1, e2 + o2, e3 + o3, e4 + o4, e4 - o4, e3 - o3, e2 - o2, e1 - o1]


def _radix4(x, sign):
    t0 = (x[0][0] + x[2][0], x[0][1] + x[2][1])
    t1 = (x[0][0] - x[2][0], x[0][1] - x[2][1])
    t2 = (x[1][0] + x[3][0], x[1][1] + x[3][1])
    t3 = (x[1][0] - x[3][0], x[1][1] - x[3][1])
    plus = (t1[0] - t3[1], t1[1] + t3[0])
    minus = (t1[0] + t3[1], t1[1] - t3[0])
    y1, y3 = (plus, minus) if sign > 0 else (minus, plus)
    return [(t0[0] + t2[0], t0[1] + t2[1]), y1, (t0[0] - t2[0], t0[1] - t2[1]), y3]


def _twiddle(z, n, sign):
    re, im = z
    if n == 0:
        return z
    if n == 4:
        return (-im, re) if sign > 0 else (im, -re)
    c, s = float(np.cos(np.pi * n / 8)), sign * float(np.sin(np.pi * n / 8))
    if n in (2, 6):
        if c * s > 0:
            return (c * (re - im), c * (im + re))
        return (c * (re + im), c * (im - re))
    return (c * re - s * im, c * im + s * re)


_A_TERMS = (((0, 0), 1, (1, 1)), ((1, 0), 1, (1, 1)), ((0, 0), 0, None), ((1, 1), 0, None),
            ((0, 0), 1, (0, 1)), ((1, 0), -1, (0, 0)), ((0, 1), -1, (1, 1)))
_B_TERMS = (((0, 0), 1, (1, 1)), ((0, 0), 0, None), ((0, 1), -1, (1, 1)), ((1, 0), -1, (0, 0)),
            ((1, 1), 0, None), ((0, 0), 1, (0, 1)), ((1, 0), 1, (1, 1)))


def _add2(x, y):
    return [[x[i][j] + y[i][j] for j in range(2)] for i in range(2)]


def _sub2(x, y):
    return [[x[i][j] - y[i][j] for j in range(2)] for i in range(2)]


def _outer_operand(ld, term):
    a, s, b = term
    x = [[ld(2 * a[0] + i, 2 * a[1] + j) for j in range(2)] for i in range(2)]
    if s == 0:
        return x
    y = [[ld(2 * b[0] + i, 2 * b[1] + j) for j in range(2)] for i in range(2)]
    return _add2(x, y) if s > 0 else _sub2(x, y)


def _inner_operand(x, term):
    a, s, b = term
    if s == 0:
        return x[a[0]][a[1]]
    return x[a[0]][a[1]] + x[b[0]][b[1]] if s > 0 else x[a[0]][a[1]] - x[b[0]][b[1]]


def _inner_result(m):
    m1, m4, m2 = m(0), m(3), m(1)
    c21, c22, c11 = m2 + m4, m1 - m2, m1 + m4
    m5, m3 = m(4), m(2)
    c12, c11, c22 = m3 + m5, c11 - m5, c22 + m3
    return [[c11 + m(6), c12], [c21, c22 + m(5)]]


def _inner_block(load, bias, p1):
    def m(p2):
        v = load(7 * p1 + p2)
        if p1 in (3, 2) and p2 in (3, 2):
            v = v + bias(2 * (3 - p1) + (3 - p2))
        return v
    return _inner_result(m)


def _finish_block(finish, c, bi, bj):
    for i in range(2):
        for j in range(2):
            finish(2 * bi + i, 2 * bj + j, c[i][j])


def _recombine(load, bias, finish, tag):
    yield tag
    m2 = _inner_block(load, bias, 1)
    yield tag
    m4 = _inner_block(load, bias, 3)
    _finish_block(finish, _add2(m2, m4), 1, 0)
    yield tag
    m1 = _inner_block(load, bias, 0)
    c22, c11 = _sub2(m1, m2), _add2(m1, m4)
    yield tag
    m5 = _inner_block(load, bias, 4)
    c11 = _sub2(c11, m5)
    yield tag
    m3 = _inner_block(load, bias, 2)
    c22 = _add2(c22, m3)
    _finish_block(finish, _add2(m3, m5), 0, 1)
    yield tag
    _finish_block(finish, _add2(c11, _inner_block(load, bias, 6)), 0, 0)
    yield tag
    _finish_block(finish, _add2(c22, _inner_block(load, bias, 5)), 1, 1)


def _gelu2(x):
    c0 = float(np.sqrt(2.0 / np.pi))
    return x + x * jnp.tanh(x * (c0 + (c0 * 0.044715) * (x * x)))


def _merge(*streams, fine=False):
    streams = [us for us in streams if us]

    def whole():
        order = sorted(((i + 0.5) / len(us), k, i) for k, us in enumerate(streams) for i in range(len(us)))
        for _, k, i in order:
            costs, gen = streams[k][i]
            yield from zip(gen, costs + [None])

    def pieces():
        order = []
        for k, us in enumerate(streams):
            costs = np.array([c for u in us for c in u[0]])
            order += [(float(q) / costs.sum(), k, int(c)) for q, c in zip(np.cumsum(costs) - 0.5 * costs, costs)]
        gens = [(tag for u in us for tag in u[1]) for us in streams]
        heads = [next(g) for g in gens]
        for _, k, c in sorted(order):
            yield heads[k], c
            heads[k] = next(gens[k], None)

    return sum(sum(u[0]) for us in streams for u in us), (pieces() if fine else whole())


def _run(units):
    for _, gen in units:
        for _ in gen:
            pass


def _pack(a, b):
    return jnp.concatenate([a, b], axis=0).astype(bf16)


def _colmean(v):
    return jnp.sum(v, axis=0, keepdims=True) * (1.0 / D)


def _rows(start, n):
    return pl.ds(start if isinstance(start, int) else pl.multiple_of(start, 8), n)


def _lanes(tile):
    return pl.ds(128 * tile if isinstance(tile, int) else pl.multiple_of(128 * tile, 128), 128)


def _as_bf16(v):
    return pltpu.bitcast(v, bf16)


def _tile(v, t):
    return v[:, 128 * t:128 * t + 128]


def _start(copies):
    for cp in copies:
        cp.start()


def _wait(copies):
    for cp in copies:
        cp.wait()


def _operand_costs(terms, groups, unpack):
    out, have = [], set()
    for keep, group in groups:
        have, n = have & set(keep), 0
        for p1 in group:
            a, s, b = terms[p1]
            need = {(2 * q[0] + i, 2 * q[1] + j) for q in ((a, b) if s else (a,)) for i in range(2) for j in range(2)}
            n += unpack * len(need - have) + (8 if s else 0) + 17
            have |= need
        out.append(n)
    return out


def _quad(*blocks):
    return [(2 * a + i, 2 * b + j) for a, b in blocks for i in range(2) for j in range(2)]


_SINGLE = [((), (p,)) for p in range(7)]
_SHARED = [((), (1,)), (_quad((0, 0), (1, 1)), (5,)), (_quad((0, 0), (1, 1), (0, 1)), (4, 2)),
           (_quad((0, 0), (1, 1)), (0, 6)), (_quad((0, 0), (1, 1), (1, 0)), (3,))]
_OUTER_ORDER = (1, 3, 0, 4, 2, 6, 5)
G = {"S": _SINGLE, "H": _SHARED}

_HA = 6 * D
_AR_TICK = _HA + 4 * D
_S_SMALL, _S_X, _S_MOD, _S_DMAT, _S_WF, _S_STAGE, _S_WIDE, _S_OUT, _N_SEM = 0, 1, 5, 10, 12, 15, 17, 18, 19


def _kernel(x_hbm, wr_hbm, wi_hbm, w1_hbm, b1_hbm, w2_hbm, b2_hbm, c_hbm, wmod_hbm, dmat_hbm, zero_hbm,
            out_hbm,
            zero_s, st0, st1, wide_v, uc_v, bc0, bc1, mm0, mm1, uu_v, x2_v, ar_v, bias_v, io_v, sem):
    copy = pltpu.make_async_copy
    state = {}

    def tick(target, val):
        ref, idx, row = target
        if ref.dtype == bf16 and ref.shape[-2] % 2:
            ref[idx + (pl.ds(pl.multiple_of(row + state["zero"], 8), 8), pl.ds(0, 128))] = val.astype(bf16)
            return
        ref = ref.bitcast(u32) if ref.dtype == bf16 else ref
        ref[idx + (pl.ds(pl.multiple_of(row + state["zero"], 8), 8), pl.ds(0, 128))] = pltpu.bitcast(val, ref.dtype)

    def paced(main, points, side, lead):
        total, gen = side
        pending, done = next(gen, None), 0
        for _ in range(lead):
            if pending is not None:
                pending, done = next(gen, None), done + pending[1]
        seen = []
        for pt, v in enumerate(main, 1):
            if pt % 1 == 0:
                seen = []
            while pending is not None and done * points < pt * total:
                if not any(pending[0] is t for t in seen):
                    seen.append(pending[0])
                    tick(pending[0], v)
                pending, done = next(gen, None), done + pending[1]
        assert pending is None

    def chained(units, target, lag):
        late = []
        for k, unit in enumerate(units):
            if k >= lag:
                for v in late[k - lag]:
                    tick(target, v)
            late.append(unit())

    t_uu, t_ar = (uu_v, (), 16 * MB), (ar_v, (), _AR_TICK)
    t_mm = [(mm0, (), NP * MB), (mm1, (), NP * MB)]
    t_st = [(st0, (), 4 * STAGE), (st1, (), 4 * STAGE)]
    bcs = (bc0, bc1)

    def stage_copies(par, src, row, tile, depth=4):
        return [copy(src.bitcast(u32).at[pl.ds(row, 256 * depth), _lanes(tile + j)],
                     t_st[par][0].at[pl.ds(j * STAGE, 256 * depth)], sem.at[_S_STAGE + par]) for j in range(4)]

    def stage_wait(par, depth=4):
        whole = t_st[par][0].at[pl.ds(0, 4 * 256 * depth)]
        copy(whole, whole, sem.at[_S_STAGE + par]).wait()

    def operand_unit(target, raw, load, terms, groups, put):
        cache = {}
        for keep, group in groups:
            yield target
            cache = {k: v for k, v in cache.items() if k in keep}

            def ld(i, j):
                if (i, j) not in cache:
                    cache[i, j] = load(i, j)
                return cache[i, j]

            for p1 in group:
                t1 = terms[p1]
                x = _outer_operand(ld, t1)
                for p2, t2 in enumerate(terms):
                    if raw is not None and t1[1] == 0 and t2[1] == 0:
                        put(7 * p1 + p2, raw(2 * t1[0][0] + t2[0][0], 2 * t1[0][1] + t2[0][1]))
                    else:
                        put(7 * p1 + p2, _inner_operand(x, t2).astype(bf16))

    def weight_units(par, groups, source=None, depth=4):
        target, bc = source or t_st[par], bcs[par]

        def unit(ru):
            def raw(k, j):
                return target[0][pl.ds(j * STAGE + 256 * (ru // 8) + 64 * k + 8 * (ru % 8), 8), :]

            def put(p, v):
                if v.dtype == u32:
                    bc.bitcast(u32)[p, pl.ds(8 * ru, 8), :] = v
                else:
                    bc[p, pl.ds(16 * ru, 16), :] = v
            return operand_unit(target, raw, lambda k, j: _as_bf16(raw(k, j)).astype(f32), _B_TERMS, groups, put)
        return [(_operand_costs(_B_TERMS, groups, 2), unit(ru)) for ru in range(8 * depth)]

    def hidden_units(c, par):
        target = t_mm[par]
        c = par if 0 else c

        t_hid = (t_uu, (ar_v, (), _AR_TICK)) if 1 else (t_uu, t_uu)
        spot = lambda i, j, r, row, n: pl.ds((4 * i + j) * MB + row + (_HA if t_hid[r % 2] is not t_uu else 0), n)

        def first(r8):
            def finish(i, j, v):
                t_hid[r8 // 2 % 2][0][spot(i, j, r8 // 2, 8 * r8, 8), :] = _gelu2(v)
            return _recombine(lambda p: target[0][pl.ds(p * MB + 8 * r8, 8), :],
                              lambda j: bias_v[_rows(8 * (4 * c + j), 8), :], finish, target)

        def second(r):
            def put(p, v):
                uc_v[p * NCH + c, pl.ds(16 * r, 16), :] = v
            return operand_unit(t_hid[r % 2], None, lambda i, j: t_hid[r % 2][0][spot(i, j, r, 16 * r, 16), :],
                                _A_TERMS, _SINGLE, put)

        units, cost, lag = [], [8, 38, 16, 12, 42, 36, 36], 1
        for r in range(MB // 16 + lag):
            if r < MB // 16:
                units += [(cost, first(2 * r)), (cost, first(2 * r + 1))]
            if r >= lag:
                units += [(_operand_costs(_A_TERMS, _SINGLE, 0), second(r - lag))]
        return units

    def products(product, outer, side):
        main = (v for p1 in outer for p2 in range(7) for v in product(7 * p1 + p2))
        points = 7 * len(outer) * (MB // 16)
        paced(main, points - max(2, points // 40), side, lead=2 if len(outer) == 7 else 1)

    def deep_product(lhs_ref, slot, bc, dst, init=None, depth=4, hooks=None):
        lhs_u, bc_u = lhs_ref.bitcast(u32), bc.bitcast(u32)

        def product(p):
            lhs = jnp.concatenate([_as_bf16(lhs_u[slot(p, t)]) for t in range(depth)], axis=1)
            v = jnp.dot(lhs, _as_bf16(bc_u[p, pl.ds(0, 64 * depth), :]), preferred_element_type=f32)
            if hooks and p in hooks:
                hooks[p]()
            for r in range(MB // 16):
                blk = v[16 * r:16 * r + 16]
                if init is not None:
                    blk = blk + init(p, r)
                dst[pl.ds(p * MB + 16 * r, 16), :] = blk
                yield blk[:8]
        return product

    def first_half(ac_v, wmod_v, dmat_v, gmat_u, wf_v, wt_v, uv_v, yv_v, pv_v, bb_v, ee_v, sa_v, c_v, b1_v, b2_v):
        small_copies = [copy(c_hbm, c_v, sem.at[_S_SMALL]), copy(zero_hbm, zero_s, sem.at[_S_SMALL]),
                        copy(b1_hbm, b1_v, sem.at[_S_SMALL]), copy(b2_hbm, b2_v, sem.at[_S_SMALL])]
        x_copies = lambda a: [copy(x_hbm.at[:, _lanes(a + 4 * b)], io_v.at[a + 4 * b], sem.at[_S_X + a])
                              for b in range(4)]
        mod_tiles = ((0, 4), (4, 9), (9, 27))
        wmod_copies = [copy(wmod_hbm.at[:, pl.ds(128 * t0, 128 * (t1 - t0))],
                            wmod_v.at[:, pl.ds(128 * t0, 128 * (t1 - t0))], sem.at[_S_MOD + h])
                       for h, (t0, t1) in enumerate(mod_tiles)]
        dmat_copies = [copy(dmat_hbm.at[pl.ds(5 * h, 5)], dmat_v.at[pl.ds(5 * h, 5)], sem.at[_S_DMAT + h])
                       for h in range(2)]
        wf_rows = ((0, 96), (96, 96), (192, DF - 192))
        wf_copies = [[copy(src.at[pl.ds(*rows)], wf_v.at[a, pl.ds(*rows)], sem.at[_S_WF + h])
                      for a, src in enumerate((wr_hbm, wi_hbm))] for h, rows in enumerate(wf_rows)]
        def mm1_step(c, par, hooks=None):
            products(deep_product(ac_v, lambda p, t: 4 * p + t, bcs[par], t_mm[par][0], hooks=hooks), range(7),
                     _merge(weight_units(1 - par, G["S"])[:32], hidden_units(c - 1, 1 - par)[:27],
                            fine=bool(0)))

        late_copies = [wmod_copies[0]] + sum(wf_copies, []) + [dmat_copies[1]] + wmod_copies[2:]
        _start(small_copies + [wmod_copies[1], dmat_copies[0]] + x_copies(0) + x_copies(1) + x_copies(2)
               + x_copies(3) + ([] if 0 else late_copies))

        _wait(small_copies)
        state["zero"] = zero_s[0]
        s0 = jax.lax.broadcasted_iota(jnp.int32, (16, 128), 0)
        j0 = jax.lax.broadcasted_iota(jnp.int32, (16, 128), 1)
        j0 = 8 * (j0 & 15) + (j0 >> 4)
        phasor = lambda n, period: (jnp.cos(n.astype(f32) * (-2 * np.pi / period)),
                                    jnp.sin(n.astype(f32) * (-2 * np.pi / period)))
        cmul = lambda x, y: (x[0] * y[0] - x[1] * y[1], x[0] * y[1] + x[1] * y[0])
        base, rot, down = phasor((s0 * j0) & 127, 128), phasor(s0, S), phasor(j0[:1] & 7, 8)

        def generate(i, carry):
            for r in range(2):
                g, rows = carry[:2], _rows(8 * (2 * i + r), 8)
                for j1 in range(16):
                    for q in range(2):
                        v = pltpu.bitcast(g[q].astype(bf16), u32)
                        gmat_u[2 * j1 + q, rows, :] = pltpu.roll(v, j1, 1) if j1 else v
                    g = cmul(g, carry[2:])
                carry = cmul(carry[:2], down) + cmul(carry[2:], (float(np.cos(np.pi / 64)), float(-np.sin(np.pi / 64))))
            return carry

        jax.lax.fori_loop(0, 8 // 2, generate, base + rot)
        for t in range(20, 24):
            io_v[t] = jnp.zeros((D, 128), bf16)
        bb_u = bb_v.bitcast(u32)


        cv = c_v[...].astype(f32)
        sc = jnp.broadcast_to(cv * jax.nn.sigmoid(cv), (16, D)).astype(bf16)
        b1 = b1_v[...].astype(f32).reshape(1, F)
        for t in range(36):
            bias_v[pl.ds(8 * t, 8), :] = jnp.broadcast_to(_tile(b1, t), (8, 128))
        b2 = 2.0 * b2_v[...].astype(f32).reshape(1, S)
        for t in range(16):
            bias_v[pl.ds(8 * (36 + t), 8), :] = jnp.broadcast_to(_tile(b2, t), (8, 128))

        def modulation(t0, n):
            cols = pl.ds(128 * t0 if isinstance(t0, int) else pl.multiple_of(128 * t0, 128), 128 * n)
            m = jnp.dot(sc, wmod_v[:, cols], preferred_element_type=f32)[:8]
            for q in range(n):
                col = 128 * (t0 + q) + jax.lax.broadcasted_iota(jnp.int32, (8, 128), 1)
                v = _tile(m, q)
                scale = ((col >= D) & (col < 2 * D)) | ((col >= 4 * D) & (col < 5 * D))
                v = jnp.where(scale, 1.0 + v, v)
                v = jnp.where(col >= 5 * D, 0.5 * v, v)
                ar_v[_rows(128 * (t0 + q), 128), :] = jnp.concatenate([v] * 16, axis=0).T

        wmod_copies[1].wait()
        modulation(4, 5)
        dmat_u, io_u = dmat_v.bitcast(u32), io_v.bitcast(u32)
        t_io, t_uv, t_x2 = (io_v, (24,), 0), (uv_v, (16,), 0), (x2_v, (), 16 * D)

        fold = lambda v: v.reshape(8, 8, 128).sum(axis=0)

        def dft9_tiles(h, r, held):
            z = _dft9(h)
            out = [(128 * g + 16 * r, _pack(*z[g + 1])) for g in range(4)]
            if r % 2:
                out.append((512 + 8 * (r - 1), _pack(held.pop(), z[0])))
            else:
                held.append(z[0])
            return out

        def put(slot, tiles):
            for row, v in tiles:
                io_v[slot, pl.ds(row, 16), :] = v

        def channel_dft(g, slots):
            n = 64 if g < 4 else 32
            lhs = _as_bf16(dmat_u[g] if g < 4 else dmat_u[4, pl.ds(0, 40), pl.ds(0, 64)])
            rhs = jnp.concatenate([_as_bf16(io_u[t, pl.ds(64 * g, n), :]) for t in slots], axis=1)
            return jnp.dot(lhs, rhs, preferred_element_type=f32)

        def spectrum(a, rstd, ordered=True):
            slots = [16 + 4 * (a % 2) + b for b in range(4)]
            nxt = channel_dft(0, slots)
            for g in range(5):
                yield
                v, nxt = nxt, (channel_dft(g + 1, slots) if g < 4 else None)
                for half in range(2):
                    yield
                    for r in range(4 * half, min(4 * half + 4, NRG[g])):
                        z = [(_tile(v[16 * r:16 * r + 8], b) * rstd[b], _tile(v[16 * r + 8:16 * r + 16], b) * rstd[b])
                             for b in range(4)]
                        for c, y in enumerate(_radix4(z, -1)):
                            uv_v[4 * a + c, pl.ds(128 * g + 16 * r, 16), :] = jnp.concatenate(y, axis=0)
                        if ordered and r % 2 == 2 - 1:
                            tick(t_io, y[1])

        def token_means(a):
            total = jnp.dot(jnp.ones((16, D), bf16),
                            jnp.concatenate([_as_bf16(io_u[a + 4 * b]) for b in range(4)], axis=1),
                            preferred_element_type=f32)
            return tuple(_tile(total[:8], b) * (1.0 / D) for b in range(4))

        def phase_a(a, rstd_prev):
            _wait(x_copies(a))
            behind = spectrum((a + 3) % 4, rstd_prev)
            mean = token_means(a)
            next(behind)
            sq, queue = [0.0] * 4, []
            for b in range(4):
                held, slot = [], 16 + 4 * (a % 2) + b
                if b:
                    tick(t_ar, sq[b - 1])
                for r in range(8):
                    if r % 2 == 0:
                        xp = [io_u[a + 4 * b, pl.ds(32 * i + 4 * r, 8), :] for i in range(9)]
                        for emit in queue:
                            emit()
                        queue = []
                        if 4 * b + r // 2 >= 1:
                            next(behind, None)
                        xp = [_as_bf16(v).astype(f32) for v in xp]
                    h = []
                    for i in range(9):
                        d = xp[i][8 * (r % 2):8 * (r % 2) + 8] - mean[b]
                        sq[b] = sq[b] + d * d
                        h.append(d * ar_v[pl.ds(D + 64 * i + 8 * r, 8), :])
                    tiles = dft9_tiles(h, r, held)
                    if r % 2 == 0:
                        put(slot, tiles)
                    else:
                        queue.append(lambda slot=slot, tiles=tiles, q=sq[b]: (put(slot, tiles), tick(t_io, q)))
            for _ in behind:
                pass
            for emit in queue:
                emit()
            return tuple(jnp.broadcast_to(jax.lax.rsqrt(_colmean(q) + 1e-5), (8, 128)) for q in sq)

        dmat_copies[0].wait()
        rstd_last = jax.lax.fori_loop(0, 4, phase_a, (jnp.zeros((8, 128), f32),) * 4)
        wmod_copies[0].wait()
        modulation(0, 4)
        for _ in spectrum(3, rstd_last, ordered=False):
            pass
        for q in range(32):
            gmat_u[32 + q] = pltpu.bitcast(_as_bf16(gmat_u[q]).T, u32)
        held = []
        for r in range(8):
            put(16, dft9_tiles([float(S) * ar_v[pl.ds(64 * i + 8 * r, 8), :] for i in range(9)], r, held))
        for g in range(5):
            v = channel_dft(g, [16])
            first = jax.lax.broadcasted_iota(jnp.int32, v.shape, 1) == 0
            sa_v[pl.ds(128 * g, 16 * NRG[g]), :] = jnp.where(first, v, 0.0)


        def pair_at(ref, j, row):
            return ref[j, pl.ds(row, 8), :], ref[j, pl.ds(row + 8, 8), :]

        t_yv, t_pv = (yv_v, (16,), 0), [t_uv, (pv_v, (16,), 0)]

        def butterflies(g, r):
            row = 128 * g + 16 * r
            for c in range(4):
                yield t_uv
                z = [_twiddle(pair_at(uv_v, 4 * a + c, row), a * c, -1) for a in range(4)]
                for e, y in enumerate(_radix4(z, -1)):
                    bb_v[c + 4 * e, pl.ds(row, 16), :] = _pack(*y)

        def token_dft(g, inverse):
            n = NRG[g]
            for j1 in range(16):
                rhs = jnp.concatenate([_as_bf16(gmat_u[32 * inverse + 2 * j1 + i]) for i in range(2)], axis=1)
                v = jnp.dot(_as_bf16(bb_u[j1, pl.ds(64 * g, 8 * n), :]), rhs, preferred_element_type=f32)
                for r in range(n):
                    top, bot = v[16 * r:16 * r + 8], v[16 * r + 8:16 * r + 16]
                    if inverse:
                        re, im = _tile(top, 0) + _tile(bot, 1), _tile(bot, 0) - _tile(top, 1)
                    else:
                        re, im = _tile(top, 0) - _tile(bot, 1), _tile(bot, 0) + _tile(top, 1)
                    dst = t_pv[g % 2][0] if inverse else yv_v
                    dst[j1, pl.ds(128 * g + 16 * r, 16), :] = jnp.concatenate([re, im], axis=0)
                    yield re

        lane = jax.lax.broadcasted_iota(jnp.int32, (8, 128), 1)

        def filt(a, j1, g, r):
            if 0:
                return wt_v[16 * a + j1, pl.ds(64 * g + 8 * (r % 8) if g < 4 else 256 + 8 * r, 8), :]
            if g < 4:
                first = (g + 1 if r < 4 else 8 - g) + 72 * (r % 4)
                return wt_v[16 * a + j1, pl.ds(first, 8, stride=9), :]
            if r < 4:
                return wt_v[16 * a + j1, pl.ds(72 * r, 8, stride=9), :]
            return wt_v[16 * a + j1, pl.ds(288, 8), :]

        def filtering(g, j1):
            for r in range(NRG[g]):
                if r % 4 == 0:
                    yield t_yv
                row = 128 * g + 16 * r
                yr, yi = pair_at(yv_v, j1, row)
                if j1 == 0:
                    yr, yi = yr + sa_v[pl.ds(row, 8), :], yi + sa_v[pl.ds(row + 8, 8), :]
                wr, wi = filt(0, j1, g, r), filt(1, j1, g, r)
                bb_v[j1, pl.ds(row, 16), :] = _pack(yr * wr - yi * wi, yr * wi + yi * wr)

        def inverse_butterflies(g, r):
            row = 128 * g + 16 * r
            mid = [[None] * 4 for _ in range(4)]
            for c in range(4):
                yield t_pv[g % 2]
                for a, y in enumerate(_radix4([pair_at(t_pv[g % 2][0], c + 4 * e, row) for e in range(4)], 1)):
                    mid[a][c] = _twiddle(y, a * c, 1)
            for a in range(4):
                for b, y in enumerate(_radix4(mid[a], 1)):
                    bb_v[a + 4 * b, pl.ds(row, 16), :] = _pack(*y)

        bfly = lambda g: [([20, 36, 28, 36], butterflies(g, r)) for r in range(NRG[g])] if g < 5 else []
        filts = lambda g: [([7 * min(4, NRG[g] - q) for q in range(0, NRG[g], 4)], filtering(g, j1)) for j1 in range(16)] if g < 5 else []
        ibfly = lambda g: [([16, 32, 24, 112], inverse_butterflies(g, r)) for r in range(NRG[g])] if g >= 0 else []

        masks = [(lane & (1 << i)) != 0 for i in range(4)]

        def regroup(tiles):
            t = [pltpu.roll(v, b, 1) if b else v for b, v in enumerate(tiles)]
            t = [t[-i % 16] for i in range(16)]
            for i in range(4):
                t = [jnp.where(masks[i], t[(j - (1 << i)) % 16], t[j]) for j in range(16)]
            return t

        def regroup_unit(a, r):
            yield t_wf
            if r < 18:
                tiles = [pltpu.bitcast(wf_v[a, pl.ds(16 * r, 16), pl.ds(128 * b, 128)], u32) for b in range(16)]
                for j1, v in enumerate(regroup(tiles)):
                    wt_v[16 * a + j1, pl.ds(16 * r, 16), :] = _as_bf16(v).astype(f32)
            else:
                last = jnp.broadcast_to(wf_v[a, pl.ds(288, 1), :].astype(f32), (8, S))
                for j1, v in enumerate(regroup([_tile(last, b) for b in range(16)])):
                    wt_v[16 * a + j1, pl.ds(288, 8), :] = v

        t_wf = (wf_v, (2,), 0)
        regroups = lambda h: [([112], regroup_unit(a, r)) for r in range(6 * h, 6 * h + 6 + h // 2) for a in range(2)]
        when = {int(q): h for h, q in enumerate("123")}

        _run(bfly(0))
        for g in range(5):
            if g in when:
                _wait(wf_copies[when[g]])
            if str(g) in "01234":
                tick((bb_v, (16,), 0), jnp.zeros((8, 128), f32))
            paced(token_dft(g, 0), 16 * NRG[g] - 24,
                  _merge(bfly(g + 1) or filts(0), regroups(when[g]) if g in when else [], fine=bool(1)), lead=1)
        first_rows = wide_v.at[pl.ds(0, 4096)]
        _start([copy(w1_hbm.bitcast(u32).at[:, _lanes(j)], wide_v.at[pl.ds(j * STAGE, 1024)], sem.at[_S_WIDE])
                for j in range(4)] + stage_copies(1, w1_hbm, 0, 4) + stage_copies(0, w1_hbm, 0, 8))

        for g in range(5):
            if str(g) in "":
                tick((bb_v, (16,), 0), jnp.zeros((8, 128), f32))
            side = (_merge(filts(g + 1) + ibfly(g - 1)) if 0 == 2 else
                    _merge(filts(g + 1), ibfly(g - 1), fine=bool(0)))
            paced(token_dft(g, 1), 16 * NRG[g] - 8, side, lead=1)
        _wait([dmat_copies[1]] + wmod_copies[2:])
        modulation(9, 18)
        _run(ibfly(4))
        shift = ar_v[pl.ds(3 * D, D), :]
        ar_v[pl.ds(3 * D, D), :] = shift - _colmean(fold(shift.reshape(9, 64, 128).sum(axis=0)))

        for a in range(4):
            rhs = jnp.concatenate([_as_bf16(bb_u[4 * a + b, pl.ds(256, 40), :]) for b in range(4)], axis=1)
            v = jnp.dot(_as_bf16(dmat_u[9, pl.ds(0, 32), pl.ds(0, 80)]), rhs, preferred_element_type=f32)
            for b in range(4):
                ee_v[pl.ds(64 * (4 * a + b), 64), :] = _tile(v, b)

        def phase_c(a, carry):
            acc = [0.0] * 4
            for b in range(4):
                t = 4 * a + b
                v = [jnp.dot(_as_bf16(dmat_u[5 + g]), _as_bf16(bb_u[4 * a + b, pl.ds(64 * g, 64), :]),
                             preferred_element_type=f32) for g in range(4)]
                for r in range(8):
                    if r % 2 == 0:
                        xres = [_as_bf16(io_u[t, pl.ds(32 * i + 4 * r, 8), :]).astype(f32) for i in range(9)]
                    z = [(q[16 * r:16 * r + 8], q[16 * r + 8:16 * r + 16]) for q in v]
                    y = _idft9(ee_v[_rows(64 * (4 * a + b) + 8 * r, 8), :], *z)
                    for i in range(9):
                        row = 64 * i + 8 * r
                        x2 = xres[i][8 * (r % 2):8 * (r % 2) + 8] + ar_v[pl.ds(2 * D + row, 8), :] * y[i]
                        x2_v[_rows(t * D + row, 8), :] = x2
                        acc[b] = acc[b] + x2
                    if r % 2 == 0:
                        tick(t_io, acc[b])
            mean = [_colmean(v) for v in acc]
            sq, lin, sq2 = [0.0] * 4, [0.0] * 4, [0.0] * 4

            def second(b, i):
                d = x2_v[_rows((4 * a + b) * D + 64 * i, 64), :] - mean[b]
                w = d * ar_v[pl.ds(4 * D + 64 * i, 64), :]
                ar_v[pl.ds(_HA + b * D + 64 * i, 64), :] = w
                sq[b], lin[b] = sq[b] + fold(d * d), lin[b] + fold(w)
                return sq[b], lin[b]

            chained([lambda b=b, i=i: second(b, i) for b in range(4) for i in range(9)], t_x2, lag=5)
            rstd = [jax.lax.rsqrt(_colmean(v) + 1e-5) for v in sq]
            mean = [_colmean(v) for v in lin]

            def third(b, i):
                h = ((ar_v[pl.ds(_HA + b * D + 64 * i, 64), :] - mean[b]) * rstd[b]
                     + ar_v[pl.ds(3 * D + 64 * i, 64), :])
                uu_v[pl.ds(b * D + 64 * i, 64), :] = h
                sq2[b] = sq2[b] + fold(h * h)
                return sq2[b],

            chained([lambda b=b, i=i: third(b, i) for b in range(4) for i in range(9)], t_ar, lag=5)
            rstd = [jax.lax.rsqrt(_colmean(v) + 1e-5) for v in sq2]

            def operands(r):
                blk = [[uu_v[pl.ds(k * D + i * MB + 16 * r, 16), :] * rstd[k] for k in range(4)] for i in range(4)]
                for p1, t1 in enumerate(_A_TERMS):
                    x = _outer_operand(lambda i, k: blk[i][k], t1)
                    for p2, t2 in enumerate(_A_TERMS):
                        v = _inner_operand(x, t2)
                        ac_v[4 * (7 * p1 + p2) + a, pl.ds(16 * r, 16), :] = v.astype(bf16)
                    if p1 == 2:
                        late = v[:8]
                return late,

            chained([lambda r=r: operands(r) for r in range(MB // 16)], t_uu, lag=1)
            return carry

        jax.lax.fori_loop(0, 4, phase_c, 0)

        copy(first_rows, first_rows, sem.at[_S_WIDE]).wait()
        stage_wait(1)
        own = lambda k: (weight_units(0, [((), (_OUTER_ORDER[k],))], source=(wide_v, (), 4 * STAGE))
                         if k < 7 else [])
        ahead = weight_units(1, G['H'])
        product = deep_product(ac_v, lambda p, t: 4 * p + t, bc0, mm0)
        _run(own(0))
        for k, p1 in enumerate(_OUTER_ORDER):
            tick((bc0, (NP,), 0), jnp.zeros((8, 128), f32))
            products(product, [p1], _merge(own(k + 1) + (ahead[4 * k:4 * k + 4] if k < 6 else ahead[24:])))

        def mm1_pair(i, carry):
            c = 2 * i + 1

            @pl.when(i < 3)
            def _():
                _start(stage_copies(1, w1_hbm, 0, 4 * (c + 2)))

            @pl.when(i == 3)
            def _():
                _start(stage_copies(1, w2_hbm, 0, 0))

            copy(w2_hbm.bitcast(u32).at[pl.ds(1024, STAGE), _lanes(i)], wide_v.at[_rows(i * STAGE, STAGE)],
                 sem.at[_S_WIDE]).start()

            def refill():
                _start(stage_copies(0, w1_hbm, 0, 4 * jnp.minimum(c + 3, NCH - 1)))
                stage_wait(1)
                tick((bc0, (NP,), 0), jnp.zeros((8, 128), f32))

            stage_wait(0)
            if 0:
                mm1_step(c, 1, {NP - 1: refill})
            else:
                mm1_step(c, 1)
                pl.when(i < 4)(refill)
            mm1_step(c + 1, 0)
            return carry

        jax.lax.fori_loop(0, 4, mm1_pair, 0)
        stage_wait(0)

    pl.run_scoped(
        first_half,
        pltpu.VMEM((4 * NP, MB, 128), bf16),
        pltpu.VMEM((D, 6 * D), bf16),
        pltpu.VMEM((10, 128, 128), bf16),
        pltpu.VMEM((64, 64, 128), u32),
        pltpu.VMEM((3, DF, S), bf16),
        pltpu.VMEM((32, 296, 128), f32),
        pltpu.VMEM((17, 592, 128), f32),
        pltpu.VMEM((17, 592, 128), f32),
        pltpu.VMEM((17, 592, 128), f32),
        pltpu.VMEM((17, 592, 128), bf16),
        pltpu.VMEM((16 * 64, 128), f32),
        pltpu.VMEM((592, 128), f32),
        pltpu.VMEM((1, D), bf16),
        pltpu.VMEM((F,), bf16),
        pltpu.VMEM((S,), bf16),
    )

    state["zero"] = zero_s[0]

    def quadrant(n, which, r8):
        def finish(i, j, v):
            row = i * MB + 8 * r8
            res = x2_v[_rows((4 * n + j) * D + row, 8), :]
            io_v[4 * n + j, pl.ds(row, 8), :] = (res + ar_v[pl.ds(5 * D + row, 8), :] * v).astype(bf16)

        m = lambda p1: _inner_block(lambda p: mm0[pl.ds(p * MB + 8 * r8, 8), :],
                                    lambda j: bias_v[_rows(8 * (36 + 4 * n + j), 8), :], p1)
        spot = lambda i, j: pl.ds((2 * i + j) * MB + 8 * r8, 8)
        yield t_mm[0]
        if which == 0:
            _finish_block(finish, _add2(m(1), m(3)), 1, 0)
        elif which == 1:
            m3 = m(2)
            _finish_block(finish, _add2(m3, m(4)), 0, 1)
            yield t_mm[0]
            part = _add2(_sub2(m(0), m(1)), m3)
            for i in range(2):
                for j in range(2):
                    uu_v[spot(i, j), :] = part[i][j]
        elif which == 2:
            part = _add2(m(0), m(3))
            yield t_mm[0]
            _finish_block(finish, _add2(_sub2(part, m(4)), m(6)), 0, 0)
        else:
            part = [[uu_v[spot(i, j), :] for j in range(2)] for i in range(2)]
            _finish_block(finish, _add2(part, m(5)), 1, 1)

    def quadrants(n, which):
        return [([[34], [34, 24], [20, 36], [24]][which], quadrant(n, which, r8)) for r8 in range(MB // 8)]

    def out_copies(n, which):
        bi, bj = ((1, 0), (0, 1), (0, 0), (1, 1))[which]
        rows = pl.ds(bi * (D // 2), D // 2)
        return [copy(io_v.at[4 * n + 2 * bj + j, rows], out_hbm.at[rows, _lanes(4 * n + 2 * bj + j)], sem.at[_S_OUT])
                for j in range(2)]

    def mm2_pair(n, carry):
        @pl.when(n < 3)
        def _():
            _start(stage_copies(1, w2_hbm, 0, 4 * n + 4))

        first = deep_product(uc_v, lambda p, t: p * NCH + t, bc1, mm1)

        @pl.when(n == 0)
        def _():
            whole = wide_v.at[pl.ds(0, 4 * STAGE)]
            copy(whole, whole, sem.at[_S_WIDE]).wait()
            products(first, range(7), _merge(weight_units(0, G["S"], (wide_v, (), 4 * STAGE), 5),
                                             hidden_units(NCH - 1, 0),
                                             fine=bool(0)))

        @pl.when(n > 0)
        def _():
            stage_wait(0, 5)
            products(first, range(7), _merge(weight_units(0, G["S"], depth=5), quadrants(n - 1, 3),
                                             fine=bool(1)))
            _start(out_copies(n - 1, 3))

        @pl.when(n < 3)
        def _():
            _start(stage_copies(0, w2_hbm, 1024, 4 * n + 4, 5))
            stage_wait(1)

        second = deep_product(uc_v, lambda p, t: p * NCH + 4 + t, bc0, mm0,
                              lambda p, r: mm1[pl.ds(p * MB + 16 * r, 16), :], depth=5,
                              hooks={7 * _OUTER_ORDER[5]: lambda: _start(out_copies(n, 0)),
                                     7 * _OUTER_ORDER[6]: lambda: _start(out_copies(n, 1))})
        ahead = weight_units(1, G["S"])
        fine = bool(1)
        products(second, _OUTER_ORDER[:2], _merge(ahead[:11]))
        products(second, _OUTER_ORDER[2:5], _merge(ahead[11:25], quadrants(n, 0), fine=fine))
        products(second, _OUTER_ORDER[5:6], _merge(ahead[25:28], quadrants(n, 1), fine=fine))
        products(second, _OUTER_ORDER[6:], _merge(ahead[28:], quadrants(n, 2), fine=fine))
        _start(out_copies(n, 2))
        return carry

    jax.lax.fori_loop(0, 4, mm2_pair, 0)
    _run(quadrants(3, 3))
    _start(out_copies(3, 3))
    copy(out_hbm, out_hbm, sem.at[_S_OUT]).wait()


@jax.jit
def pallas_adaLN_cond__spectral_gfnet__mixer_token_mlp__prompt_kernel(
    A_x: jax.Array,
    A_w_r: jax.Array,
    A_w_i: jax.Array,
    B_x: jax.Array,
    B_w1: jax.Array,
    B_b1: jax.Array,
    B_w2: jax.Array,
    B_b2: jax.Array,
    c: jax.Array,
    w_mod: jax.Array,
):
    del B_x
    hbm = pl.BlockSpec(memory_space=pl.ANY)
    out = pl.pallas_call(
        _kernel,
        out_shape=jax.ShapeDtypeStruct((D, S), bf16),
        in_specs=[hbm] * 11,
        out_specs=hbm,
        scratch_shapes=[
            pltpu.SMEM((1,), jnp.int32),
            pltpu.VMEM((4 * STAGE + 8, 128), u32),
            pltpu.VMEM((4 * STAGE + 8, 128), u32),
            pltpu.VMEM((4 * STAGE + 8, 128), u32),
            pltpu.VMEM((NP * NCH, MB, 128), bf16),
            pltpu.VMEM((NP + 1, 640, 128), bf16),
            pltpu.VMEM((NP, 512, 128), bf16),
            pltpu.VMEM((NP * MB + 8, 128), f32),
            pltpu.VMEM((NP * MB + 8, 128), f32),
            pltpu.VMEM((16 * MB + 8, 128), f32),
            pltpu.VMEM((16 * D + 8, 128), f32),
            pltpu.VMEM((_AR_TICK + 8, 128), f32),
            pltpu.VMEM((8 * 52, 128), f32),
            pltpu.VMEM((25, D, 128), bf16),
            pltpu.SemaphoreType.DMA((_N_SEM,)),
        ],
        compiler_params=pltpu.CompilerParams(vmem_limit_bytes=126 * 1024 * 1024),
        name="adaln_gfnet_mixer",
    )(A_x.reshape(S, D).T, A_w_r.T, A_w_i.T, B_w1, B_b1, B_w2, B_b2, c, w_mod, _DMAT,
      np.zeros((1,), np.int32))
    return out.T.reshape(1, S, D)
```

```python
import numpy as np
import jax
import jax.numpy as jnp
import jax.experimental.pallas as pl
import jax.experimental.pallas.tpu as pltpu

S, D, F = 2048, 576, 4608
DF = D // 2 + 1
NP = 49
MB = D // 4
NCH = F // 512
NRG = (8, 8, 8, 8, 5)
STAGE = 1280

f32, u32, bf16 = jnp.float32, jnp.uint32, jnp.bfloat16


def _interleave(a, b):
    n = a.shape[0] // 8
    return np.stack([a.reshape(n, 8, -1), b.reshape(n, 8, -1)], axis=1).reshape(16 * n, -1)


def _constants():
    d0 = np.arange(64)
    fd = np.zeros((5, 128, 128))
    fi = np.zeros((5, 128, 128))
    scale = 1.0 / (S * D)
    for k1 in range(1, 5):
        k = np.array([k1 + 9 * m for m in range(32)] + [9 - k1 + 9 * m for m in range(32)])
        sg = np.array([1.0] * 32 + [-1.0] * 32)[:, None]
        ang = 2 * np.pi * np.outer(k, d0) / D
        c, s = np.cos(ang), np.sin(ang)
        q = np.sqrt(3.0) / 2 if k1 == 3 else 1.0
        re = _interleave(c.T, (-q * sg * s).T).T
        im = _interleave(-s.T, (-q * sg * c).T).T
        fd[k1 - 1] = _interleave(re, im)
        fi[k1 - 1] = 2 * scale * fd[k1 - 1].T
    ang = 2 * np.pi * np.outer(9 * np.arange(33), d0) / D
    re, im = np.zeros((40, 64)), np.zeros((40, 64))
    re[:33], im[:33] = np.cos(ang), -np.sin(ang)
    im[0] = im[32] = 0.0
    w = np.full((40, 1), 2.0)
    w[0] = w[32] = 1.0
    fd[4, :80, :64] = _interleave(re, im)
    fi[4, :64, :80] = scale * _interleave(w * re, w * im).T
    return np.concatenate([fd, fi]).astype(np.float32).astype(jnp.bfloat16)


_DMAT = _constants()

_C1, _C2, _C4 = (float(np.cos(2 * np.pi * k / 9)) for k in (1, 2, 4))
_S1, _S4, _S3 = float(np.sin(2 * np.pi / 9)), float(np.sin(8 * np.pi / 9)), float(np.sqrt(3.0) / 2)


def _dft9(x):
    e1, e2, e3, e4 = x[1] + x[8], x[2] + x[7], x[3] + x[6], x[4] + x[5]
    o1, o2, o3, o4 = x[1] - x[8], x[2] - x[7], x[3] - x[6], x[4] - x[5]
    t = x[0] - 0.5 * e3
    sm = e1 + e2 + e4
    p = x[0] + e3
    d1, d2 = e1 - e4, e2 - e4
    q1 = _C1 * d1 + _C2 * d2
    q2 = _C2 * d1 + _C4 * d2
    a, b, c = o1 + o2, o2 + o4, o1 - o4
    r1 = _S1 * a + _S4 * b
    r2 = _S1 * c + _S4 * a
    v = _S3 * o3
    return (p + sm, (t + q1, r1 + v), (t + q2, r2 - v), (p - 0.5 * sm, (o1 - o2) + o4),
            ((t - q1) - q2, (r2 - r1) + v))


def _idft9(a0, z1, z2, z3, z4):
    (a1, b1), (a2, b2), (a3, b3), (a4, b4) = z1, z2, z3, z4
    o3 = _S3 * ((b1 - b2) + b4)
    r1, r2 = b1 - b4, b2 + b4
    a, b, c = _S1 * r1 + _S4 * r2, _S4 * r1, _S1 * r2
    o1, o2, o4 = (a + c) + b3, (a + b) - b3, (b - c) + b3
    t = (a1 + a2) + a4
    q1, q2 = a1 - a4, a2 - a4
    d1 = _C1 * q1 + _C2 * q2
    d2 = _C2 * q1 + _C4 * q2
    p, sm = a0 + a3, a0 - 0.5 * a3
    e1, e2, e4 = sm + d1, sm + d2, (sm - d1) - d2
    e3 = p - 0.5 * t
    return [t + p, e1 + o1, e2 + o2, e3 + o3, e4 + o4, e4 - o4, e3 - o3, e2 - o2, e1 - o1]


def _radix4(x, sign):
    t0 = (x[0][0] + x[2][0], x[0][1] + x[2][1])
    t1 = (x[0][0] - x[2][0], x[0][1] - x[2][1])
    t2 = (x[1][0] + x[3][0], x[1][1] + x[3][1])
    t3 = (x[1][0] - x[3][0], x[1][1] - x[3][1])
    plus = (t1[0] - t3[1], t1[1] + t3[0])
    minus = (t1[0] + t3[1], t1[1] - t3[0])
    y1, y3 = (plus, minus) if sign > 0 else (minus, plus)
    return [(t0[0] + t2[0], t0[1] + t2[1]), y1, (t0[0] - t2[0], t0[1] - t2[1]), y3]


def _twiddle(z, n, sign):
    re, im = z
    if n == 0:
        return z
    if n == 4:
        return (-im, re) if sign > 0 else (im, -re)
    c, s = float(np.cos(np.pi * n / 8)), sign * float(np.sin(np.pi * n / 8))
    if n in (2, 6):
        if c * s > 0:
            return (c * (re - im), c * (im + re))
        return (c * (re + im), c * (im - re))
    return (c * re - s * im, c * im + s * re)


_A_TERMS = (((0, 0), 1, (1, 1)), ((1, 0), 1, (1, 1)), ((0, 0), 0, None), ((1, 1), 0, None),
            ((0, 0), 1, (0, 1)), ((1, 0), -1, (0, 0)), ((0, 1), -1, (1, 1)))
_B_TERMS = (((0, 0), 1, (1, 1)), ((0, 0), 0, None), ((0, 1), -1, (1, 1)), ((1, 0), -1, (0, 0)),
            ((1, 1), 0, None), ((0, 0), 1, (0, 1)), ((1, 0), 1, (1, 1)))


def _add2(x, y):
    return [[x[i][j] + y[i][j] for j in range(2)] for i in range(2)]


def _sub2(x, y):
    return [[x[i][j] - y[i][j] for j in range(2)] for i in range(2)]


def _outer_operand(ld, term):
    a, s, b = term
    x = [[ld(2 * a[0] + i, 2 * a[1] + j) for j in range(2)] for i in range(2)]
    if s == 0:
        return x
    y = [[ld(2 * b[0] + i, 2 * b[1] + j) for j in range(2)] for i in range(2)]
    return _add2(x, y) if s > 0 else _sub2(x, y)


def _inner_operand(x, term):
    a, s, b = term
    if s == 0:
        return x[a[0]][a[1]]
    return x[a[0]][a[1]] + x[b[0]][b[1]] if s > 0 else x[a[0]][a[1]] - x[b[0]][b[1]]


def _inner_result(m):
    m1, m4, m2 = m(0), m(3), m(1)
    c21, c22, c11 = m2 + m4, m1 - m2, m1 + m4
    m5, m3 = m(4), m(2)
    c12, c11, c22 = m3 + m5, c11 - m5, c22 + m3
    return [[c11 + m(6), c12], [c21, c22 + m(5)]]


def _inner_block(load, bias, p1):
    def m(p2):
        v = load(7 * p1 + p2)
        if p1 in (3, 2) and p2 in (3, 2):
            v = v + bias(2 * (3 - p1) + (3 - p2))
        return v
    return _inner_result(m)


def _finish_block(finish, c, bi, bj):
    for i in range(2):
        for j in range(2):
            finish(2 * bi + i, 2 * bj + j, c[i][j])


def _recombine(load, bias, finish, tag):
    yield tag
    m2 = _inner_block(load, bias, 1)
    yield tag
    m4 = _inner_block(load, bias, 3)
    _finish_block(finish, _add2(m2, m4), 1, 0)
    yield tag
    m1 = _inner_block(load, bias, 0)
    c22, c11 = _sub2(m1, m2), _add2(m1, m4)
    yield tag
    m5 = _inner_block(load, bias, 4)
    c11 = _sub2(c11, m5)
    yield tag
    m3 = _inner_block(load, bias, 2)
    c22 = _add2(c22, m3)
    _finish_block(finish, _add2(m3, m5), 0, 1)
    yield tag
    _finish_block(finish, _add2(c11, _inner_block(load, bias, 6)), 0, 0)
    yield tag
    _finish_block(finish, _add2(c22, _inner_block(load, bias, 5)), 1, 1)


def _gelu2(x):
    c0 = float(np.sqrt(2.0 / np.pi))
    return x + x * jnp.tanh(x * (c0 + (c0 * 0.044715) * (x * x)))


def _merge(*streams, fine=False):
    streams = [us for us in streams if us]

    def whole():
        order = sorted(((i + 0.5) / len(us), k, i) for k, us in enumerate(streams) for i in range(len(us)))
        for _, k, i in order:
            costs, gen = streams[k][i]
            yield from zip(gen, costs + [None])

    def pieces():
        order = []
        for k, us in enumerate(streams):
            costs = np.array([c for u in us for c in u[0]])
            order += [(float(q) / costs.sum(), k, int(c)) for q, c in zip(np.cumsum(costs) - 0.5 * costs, costs)]
        gens = [(tag for u in us for tag in u[1]) for us in streams]
        heads = [next(g) for g in gens]
        for _, k, c in sorted(order):
            yield heads[k], c
            heads[k] = next(gens[k], None)

    return sum(sum(u[0]) for us in streams for u in us), (pieces() if fine else whole())


def _run(units):
    for _, gen in units:
        for _ in gen:
            pass


def _pack(a, b):
    return jnp.concatenate([a, b], axis=0).astype(bf16)


def _colmean(v):
    return jnp.sum(v, axis=0, keepdims=True) * (1.0 / D)


def _fold(v):
    return v.reshape(8, 8, 128).sum(axis=0)


def _rows(start, n):
    return pl.ds(start if isinstance(start, int) else pl.multiple_of(start, 8), n)


def _lanes(tile):
    return pl.ds(128 * tile if isinstance(tile, int) else pl.multiple_of(128 * tile, 128), 128)


def _as_bf16(v):
    return pltpu.bitcast(v, bf16)


def _tile(v, t):
    return v[:, 128 * t:128 * t + 128]


def _start(copies):
    for cp in copies:
        cp.start()


def _wait(copies):
    for cp in copies:
        cp.wait()


def _operand_costs(terms, groups, unpack):
    out, have = [], set()
    for keep, group in groups:
        have, n = have & set(keep), 0
        for p1 in group:
            a, s, b = terms[p1]
            need = {(2 * q[0] + i, 2 * q[1] + j) for q in ((a, b) if s else (a,)) for i in range(2) for j in range(2)}
            n += unpack * len(need - have) + (8 if s else 0) + 17
            have |= need
        out.append(n)
    return out


def _quad(*blocks):
    return [(2 * a + i, 2 * b + j) for a, b in blocks for i in range(2) for j in range(2)]


_SINGLE = [((), (p,)) for p in range(7)]
_SHARED = [((), (1,)), (_quad((0, 0), (1, 1)), (5,)), (_quad((0, 0), (1, 1), (0, 1)), (4, 2)),
           (_quad((0, 0), (1, 1)), (0, 6)), (_quad((0, 0), (1, 1), (1, 0)), (3,))]
_OUTER_ORDER = (1, 3, 0, 4, 2, 6, 5)

_HA = 6 * D
_AR_TICK = _HA + 4 * D
_S_SMALL, _S_X, _S_MOD, _S_DMAT, _S_WF, _S_STAGE, _S_OUT, _N_SEM = 0, 1, 5, 8, 10, 13, 16, 17


def _kernel(x_hbm, wr_hbm, wi_hbm, w1_hbm, b1_hbm, w2_hbm, b2_hbm, c_hbm, wmod_hbm, dmat_hbm, zero_hbm,
            out_hbm,
            zero_s, st0, st1, st2, uc_v, bc0, bc1, mm0, mm1, uu_v, x2_v, ar_v, bias_v, io_v, sem):
    copy = pltpu.make_async_copy
    state = {}

    def tick(target, val):
        ref, idx, row = target
        where = idx + (_rows(row + state["zero"], 8), pl.ds(0, 128))
        if ref.dtype != bf16:
            ref[where] = pltpu.bitcast(val, ref.dtype)
        elif ref.shape[-2] % 2:
            ref[where] = val.astype(bf16)
        else:
            ref.bitcast(u32)[where] = pltpu.bitcast(val, u32)

    def fence(ref):
        tick((ref, (ref.shape[0] - 1,), 0), jnp.zeros((8, 128), f32))

    def paced(main, points, side, lead):
        total, gen = side
        pending, done = next(gen, None), 0
        for _ in range(lead):
            if pending is not None:
                pending, done = next(gen, None), done + pending[1]
        for pt, v in enumerate(main, 1):
            seen = []
            while pending is not None and done * points < pt * total:
                if not any(pending[0] is t for t in seen):
                    seen.append(pending[0])
                    tick(pending[0], v)
                pending, done = next(gen, None), done + pending[1]
        assert pending is None

    def chained(units, target, lag):
        late = []
        for k, unit in enumerate(units):
            if k >= lag:
                for v in late[k - lag]:
                    tick(target, v)
            late.append(unit())

    t_uu, t_ar = (uu_v, (), 16 * MB), (ar_v, (), _AR_TICK)
    t_mm = [(mm0, (), NP * MB), (mm1, (), NP * MB)]
    t_st = [(ref, (), 4 * STAGE) for ref in (st0, st1, st2)]
    bcs = (bc0, bc1)

    def stage_copies(par, src, row, tile, depth=4):
        return [copy(src.bitcast(u32).at[pl.ds(row, 256 * depth), _lanes(tile + j)],
                     t_st[par][0].at[pl.ds(j * STAGE, 256 * depth)], sem.at[_S_STAGE + par]) for j in range(4)]

    def stage_wait(par, depth=4):
        for j in range(4):
            tile = t_st[par][0].at[pl.ds(j * STAGE, 256 * depth)]
            copy(tile, tile, sem.at[_S_STAGE + par]).wait()

    def operand_unit(target, raw, load, terms, groups, put):
        cache = {}
        for keep, group in groups:
            yield target
            cache = {k: v for k, v in cache.items() if k in keep}

            def ld(i, j):
                if (i, j) not in cache:
                    cache[i, j] = load(i, j)
                return cache[i, j]

            for p1 in group:
                t1 = terms[p1]
                x = _outer_operand(ld, t1)
                for p2, t2 in enumerate(terms):
                    if raw is not None and t1[1] == 0 and t2[1] == 0:
                        put(7 * p1 + p2, raw(2 * t1[0][0] + t2[0][0], 2 * t1[0][1] + t2[0][1]))
                    else:
                        put(7 * p1 + p2, _inner_operand(x, t2).astype(bf16))

    def weight_units(par, bc, groups=_SINGLE, depth=4):
        target = t_st[par]

        def unit(ru):
            def raw(k, j):
                return target[0][pl.ds(j * STAGE + 256 * (ru // 8) + 64 * k + 8 * (ru % 8), 8), :]

            def put(p, v):
                if v.dtype == u32:
                    bc.bitcast(u32)[p, pl.ds(8 * ru, 8), :] = v
                else:
                    bc[p, pl.ds(16 * ru, 16), :] = v
            return operand_unit(target, raw, lambda k, j: _as_bf16(raw(k, j)).astype(f32), _B_TERMS, groups, put)
        return [(_operand_costs(_B_TERMS, groups, 2), unit(ru)) for ru in range(8 * depth)]

    def hidden_units(c, par):
        target, t_hid = t_mm[par], (t_uu, t_ar)
        spot = lambda i, j, r, row, n: pl.ds(_HA * (r % 2) + (4 * i + j) * MB + row, n)

        def first(r8):
            def finish(i, j, v):
                t_hid[r8 // 2 % 2][0][spot(i, j, r8 // 2, 8 * r8, 8), :] = _gelu2(v)
            return _recombine(lambda p: target[0][pl.ds(p * MB + 8 * r8, 8), :],
                              lambda j: bias_v[_rows(8 * (4 * c + j), 8), :], finish, target)

        def second(r):
            def put(p, v):
                uc_v[p * NCH + c, pl.ds(16 * r, 16), :] = v
            return operand_unit(t_hid[r % 2], None, lambda i, j: t_hid[r % 2][0][spot(i, j, r, 16 * r, 16), :],
                                _A_TERMS, _SINGLE, put)

        units, cost = [], [8, 38, 16, 12, 42, 36, 36]
        for r in range(MB // 16 + 1):
            if r < MB // 16:
                units += [(cost, first(2 * r)), (cost, first(2 * r + 1))]
            if r > 0:
                units += [(_operand_costs(_A_TERMS, _SINGLE, 0), second(r - 1))]
        return units

    def products(product, outer, side):
        main = (v for p1 in outer for p2 in range(7) for v in product(7 * p1 + p2))
        points = 7 * len(outer) * (MB // 16)
        paced(main, points - max(2, points // 40), side, lead=2 if len(outer) == 7 else 1)

    def deep_product(lhs_ref, slot, bc, dst, init=None, depth=4, hooks=None):
        lhs_u, bc_u = lhs_ref.bitcast(u32), bc.bitcast(u32)

        def product(p):
            lhs = jnp.concatenate([_as_bf16(lhs_u[slot(p, t)]) for t in range(depth)], axis=1)
            v = jnp.dot(lhs, _as_bf16(bc_u[p, pl.ds(0, 64 * depth), :]), preferred_element_type=f32)
            if hooks and p in hooks:
                hooks[p]()
            for r in range(MB // 16):
                blk = v[16 * r:16 * r + 16]
                if init is not None:
                    blk = blk + init(p, r)
                dst[pl.ds(p * MB + 16 * r, 16), :] = blk
                yield blk[:8]
        return product

    def first_half(ac_v, wmod_v, dmat_v, gmat_u, wf_v, wt_v, uv_v, yv_v, pv_v, bb_v, ee_v, sa_v, c_v, b1_v, b2_v):
        small_copies = [copy(c_hbm, c_v, sem.at[_S_SMALL]), copy(zero_hbm, zero_s, sem.at[_S_SMALL]),
                        copy(b1_hbm, b1_v, sem.at[_S_SMALL]), copy(b2_hbm, b2_v, sem.at[_S_SMALL])]
        x_copies = lambda a: [copy(x_hbm.at[:, _lanes(a + 4 * b)], io_v.at[a + 4 * b], sem.at[_S_X + a])
                              for b in range(4)]
        mod_tiles = ((0, 4), (4, 9), (9, 27))
        wmod_copies = [copy(wmod_hbm.at[:, pl.ds(128 * t0, 128 * (t1 - t0))],
                            wmod_v.at[:, pl.ds(128 * t0, 128 * (t1 - t0))], sem.at[_S_MOD + h])
                       for h, (t0, t1) in enumerate(mod_tiles)]
        dmat_copies = [copy(dmat_hbm.at[pl.ds(5 * h, 5)], dmat_v.at[pl.ds(5 * h, 5)], sem.at[_S_DMAT + h])
                       for h in range(2)]
        wf_rows = ((0, 96), (96, 96), (192, DF - 192))
        wf_copies = [[copy(src.at[pl.ds(*rows)], wf_v.at[a, pl.ds(*rows)], sem.at[_S_WF + h])
                      for a, src in enumerate((wr_hbm, wi_hbm))] for h, rows in enumerate(wf_rows)]

        _start(small_copies + [wmod_copies[1], dmat_copies[0]] + sum((x_copies(a) for a in range(4)), [])
               + [wmod_copies[0]] + sum(wf_copies, []) + [dmat_copies[1], wmod_copies[2]])
        _wait(small_copies)
        state["zero"] = zero_s[0]
        s0 = jax.lax.broadcasted_iota(jnp.int32, (16, 128), 0)
        j0 = jax.lax.broadcasted_iota(jnp.int32, (16, 128), 1)
        j0 = 8 * (j0 & 15) + (j0 >> 4)
        phasor = lambda n, period: (jnp.cos(n.astype(f32) * (-2 * np.pi / period)),
                                    jnp.sin(n.astype(f32) * (-2 * np.pi / period)))
        cmul = lambda x, y: (x[0] * y[0] - x[1] * y[1], x[0] * y[1] + x[1] * y[0])
        base, rot, down = phasor((s0 * j0) & 127, 128), phasor(s0, S), phasor(j0[:1] & 7, 8)

        def generate(i, carry):
            for r in range(2):
                g, rows = carry[:2], _rows(8 * (2 * i + r), 8)
                for j1 in range(16):
                    for q in range(2):
                        v = pltpu.bitcast(g[q].astype(bf16), u32)
                        gmat_u[2 * j1 + q, rows, :] = pltpu.roll(v, j1, 1) if j1 else v
                    g = cmul(g, carry[2:])
                carry = cmul(carry[:2], down) + cmul(carry[2:], (float(np.cos(np.pi / 64)), float(-np.sin(np.pi / 64))))
            return carry

        jax.lax.fori_loop(0, 4, generate, base + rot)
        for t in range(20, 24):
            io_v[t] = jnp.zeros((D, 128), bf16)
        bb_u = bb_v.bitcast(u32)


        cv = c_v[...].astype(f32)
        sc = jnp.broadcast_to(cv * jax.nn.sigmoid(cv), (16, D)).astype(bf16)
        b1 = b1_v[...].astype(f32).reshape(1, F)
        for t in range(36):
            bias_v[pl.ds(8 * t, 8), :] = jnp.broadcast_to(_tile(b1, t), (8, 128))
        b2 = 2.0 * b2_v[...].astype(f32).reshape(1, S)
        for t in range(16):
            bias_v[pl.ds(8 * (36 + t), 8), :] = jnp.broadcast_to(_tile(b2, t), (8, 128))

        def modulation(h):
            t0, t1 = mod_tiles[h]
            m = jnp.dot(sc, wmod_v[:, pl.ds(128 * t0, 128 * (t1 - t0))], preferred_element_type=f32)[:8]
            for t in range(t0, t1):
                col = 128 * t + jax.lax.broadcasted_iota(jnp.int32, (8, 128), 1)
                v = _tile(m, t - t0)
                scale = ((col >= D) & (col < 2 * D)) | ((col >= 4 * D) & (col < 5 * D))
                v = jnp.where(scale, 1.0 + v, v)
                v = jnp.where(col >= 5 * D, 0.5 * v, v)
                ar_v[pl.ds(128 * t, 128), :] = jnp.concatenate([v] * 16, axis=0).T

        wmod_copies[1].wait()
        modulation(1)
        dmat_u, io_u = dmat_v.bitcast(u32), io_v.bitcast(u32)
        t_io, t_uv, t_x2 = (io_v, (24,), 0), (uv_v, (16,), 0), (x2_v, (), 16 * D)

        def dft9_tiles(h, r, held):
            z = _dft9(h)
            out = [(128 * g + 16 * r, _pack(*z[g + 1])) for g in range(4)]
            if r % 2:
                out.append((512 + 8 * (r - 1), _pack(held.pop(), z[0])))
            else:
                held.append(z[0])
            return out

        def put(slot, tiles):
            for row, v in tiles:
                io_v[slot, pl.ds(row, 16), :] = v

        def channel_dft(g, slots):
            n = 64 if g < 4 else 32
            lhs = _as_bf16(dmat_u[g] if g < 4 else dmat_u[4, pl.ds(0, 40), pl.ds(0, 64)])
            rhs = jnp.concatenate([_as_bf16(io_u[t, pl.ds(64 * g, n), :]) for t in slots], axis=1)
            return jnp.dot(lhs, rhs, preferred_element_type=f32)

        def spectrum(a, rstd, ordered=True):
            slots = [16 + 4 * (a % 2) + b for b in range(4)]
            nxt = channel_dft(0, slots)
            for g in range(5):
                yield
                v, nxt = nxt, (channel_dft(g + 1, slots) if g < 4 else None)
                for half in range(2):
                    yield
                    for r in range(4 * half, min(4 * half + 4, NRG[g])):
                        z = [(_tile(v[16 * r:16 * r + 8], b) * rstd[b], _tile(v[16 * r + 8:16 * r + 16], b) * rstd[b])
                             for b in range(4)]
                        for c, y in enumerate(_radix4(z, -1)):
                            uv_v[4 * a + c, pl.ds(128 * g + 16 * r, 16), :] = jnp.concatenate(y, axis=0)
                        if ordered and r % 2:
                            tick(t_io, y[1])

        def token_mean(t):
            total = jnp.dot(jnp.ones((16, D), bf16), _as_bf16(io_u[t]), preferred_element_type=f32)
            return total[:8] * (1.0 / D)

        def phase_a(a, rstd_prev):
            _wait(x_copies(a))
            behind = spectrum((a + 3) % 4, rstd_prev)
            mean = [token_mean(a)]
            next(behind)
            sq, queue = [0.0] * 4, []
            for b in range(4):
                held, slot = [], 16 + 4 * (a % 2) + b
                if b:
                    tick(t_ar, sq[b - 1])
                if b < 3:
                    mean.append(token_mean(a + 4 * b + 4))
                for r in range(8):
                    if r % 2 == 0:
                        xp = [io_u[a + 4 * b, pl.ds(32 * i + 4 * r, 8), :] for i in range(9)]
                        for emit in queue:
                            emit()
                        queue = []
                        next(behind, None)
                        xp = [_as_bf16(v).astype(f32) for v in xp]
                    h = []
                    for i in range(9):
                        d = xp[i][8 * (r % 2):8 * (r % 2) + 8] - mean[b]
                        sq[b] = sq[b] + d * d
                        h.append(d * ar_v[pl.ds(D + 64 * i + 8 * r, 8), :])
                    tiles = dft9_tiles(h, r, held)
                    if r % 2 == 0:
                        put(slot, tiles)
                    else:
                        queue.append(lambda slot=slot, tiles=tiles, q=sq[b]: (put(slot, tiles), tick(t_io, q)))
            for _ in behind:
                pass
            for emit in queue:
                emit()
            return tuple(jnp.broadcast_to(jax.lax.rsqrt(_colmean(q) + 1e-5), (8, 128)) for q in sq)

        dmat_copies[0].wait()
        rstd_last = jax.lax.fori_loop(0, 4, phase_a, (jnp.zeros((8, 128), f32),) * 4)
        wmod_copies[0].wait()
        modulation(0)
        for _ in spectrum(3, rstd_last, ordered=False):
            pass
        for q in range(32):
            gmat_u[32 + q] = pltpu.bitcast(_as_bf16(gmat_u[q]).T, u32)
        held = []
        for r in range(8):
            put(16, dft9_tiles([float(S) * ar_v[pl.ds(64 * i + 8 * r, 8), :] for i in range(9)], r, held))
        for g in range(5):
            v = channel_dft(g, [16])
            first = jax.lax.broadcasted_iota(jnp.int32, v.shape, 1) == 0
            sa_v[pl.ds(128 * g, 16 * NRG[g]), :] = jnp.where(first, v, 0.0)


        def pair_at(ref, j, row):
            return ref[j, pl.ds(row, 8), :], ref[j, pl.ds(row + 8, 8), :]

        t_yv, t_pv = (yv_v, (16,), 0), [t_uv, (pv_v, (16,), 0)]

        def butterflies(g, r):
            row = 128 * g + 16 * r
            for c in range(4):
                yield t_uv
                z = [_twiddle(pair_at(uv_v, 4 * a + c, row), a * c, -1) for a in range(4)]
                for e, y in enumerate(_radix4(z, -1)):
                    bb_v[c + 4 * e, pl.ds(row, 16), :] = _pack(*y)

        def token_dft(g, inverse):
            n = NRG[g]
            for j1 in range(16):
                rhs = jnp.concatenate([_as_bf16(gmat_u[32 * inverse + 2 * j1 + i]) for i in range(2)], axis=1)
                v = jnp.dot(_as_bf16(bb_u[j1, pl.ds(64 * g, 8 * n), :]), rhs, preferred_element_type=f32)
                for r in range(n):
                    top, bot = v[16 * r:16 * r + 8], v[16 * r + 8:16 * r + 16]
                    if inverse:
                        re, im = _tile(top, 0) + _tile(bot, 1), _tile(bot, 0) - _tile(top, 1)
                    else:
                        re, im = _tile(top, 0) - _tile(bot, 1), _tile(bot, 0) + _tile(top, 1)
                    dst = t_pv[g % 2][0] if inverse else yv_v
                    dst[j1, pl.ds(128 * g + 16 * r, 16), :] = jnp.concatenate([re, im], axis=0)
                    yield re

        lane = jax.lax.broadcasted_iota(jnp.int32, (8, 128), 1)

        def filt(a, j1, g, r):
            if g < 4:
                first = (g + 1 if r < 4 else 8 - g) + 72 * (r % 4)
                return wt_v[16 * a + j1, pl.ds(first, 8, stride=9), :]
            if r < 4:
                return wt_v[16 * a + j1, pl.ds(72 * r, 8, stride=9), :]
            return wt_v[16 * a + j1, pl.ds(288, 8), :]

        def filtering(g, j1):
            for r in range(NRG[g]):
                if r % 4 == 0:
                    yield t_yv
                row = 128 * g + 16 * r
                yr, yi = pair_at(yv_v, j1, row)
                if j1 == 0:
                    yr, yi = yr + sa_v[pl.ds(row, 8), :], yi + sa_v[pl.ds(row + 8, 8), :]
                wr, wi = filt(0, j1, g, r), filt(1, j1, g, r)
                bb_v[j1, pl.ds(row, 16), :] = _pack(yr * wr - yi * wi, yr * wi + yi * wr)

        def inverse_butterflies(g, r):
            row = 128 * g + 16 * r
            mid = [[None] * 4 for _ in range(4)]
            for c in range(4):
                yield t_pv[g % 2]
                for a, y in enumerate(_radix4([pair_at(t_pv[g % 2][0], c + 4 * e, row) for e in range(4)], 1)):
                    mid[a][c] = _twiddle(y, a * c, 1)
            for a in range(4):
                for b, y in enumerate(_radix4(mid[a], 1)):
                    bb_v[a + 4 * b, pl.ds(row, 16), :] = _pack(*y)

        bfly = lambda g: [([20, 36, 28, 36], butterflies(g, r)) for r in range(NRG[g])] if g < 5 else []
        filts = lambda g: [([28, 7 * (NRG[g] - 4)], filtering(g, j1)) for j1 in range(16)] if g < 5 else []
        ibfly = lambda g: [([16, 32, 24, 112], inverse_butterflies(g, r)) for r in range(NRG[g])] if g >= 0 else []

        masks = [(lane & (1 << i)) != 0 for i in range(4)]

        def regroup(tiles):
            t = [pltpu.roll(v, b, 1) if b else v for b, v in enumerate(tiles)]
            t = [t[-i % 16] for i in range(16)]
            for i in range(4):
                t = [jnp.where(masks[i], t[(j - (1 << i)) % 16], t[j]) for j in range(16)]
            return t

        def regroup_unit(a, r):
            yield t_wf
            if r < 18:
                tiles = [pltpu.bitcast(wf_v[a, pl.ds(16 * r, 16), pl.ds(128 * b, 128)], u32) for b in range(16)]
                for j1, v in enumerate(regroup(tiles)):
                    wt_v[16 * a + j1, pl.ds(16 * r, 16), :] = _as_bf16(v).astype(f32)
            else:
                last = jnp.broadcast_to(wf_v[a, pl.ds(288, 1), :].astype(f32), (8, S))
                for j1, v in enumerate(regroup([_tile(last, b) for b in range(16)])):
                    wt_v[16 * a + j1, pl.ds(288, 8), :] = v

        t_wf = (wf_v, (2,), 0)
        regroups = lambda h: [([112], regroup_unit(a, r)) for r in range(6 * h, 6 * h + 6 + h // 2) for a in range(2)]

        _run(bfly(0))
        for g in range(5):
            if 1 <= g <= 3:
                _wait(wf_copies[g - 1])
            fence(bb_v)
            paced(token_dft(g, 0), 16 * NRG[g] - 24,
                  _merge(bfly(g + 1) or filts(0), regroups(g - 1) if 1 <= g <= 3 else [], fine=True), lead=1)
        _start(stage_copies(2, w1_hbm, 0, 0) + stage_copies(1, w1_hbm, 0, 4) + stage_copies(0, w1_hbm, 0, 8))
        for g in range(5):
            paced(token_dft(g, 1), 16 * NRG[g] - 8, _merge(filts(g + 1), ibfly(g - 1)), lead=1)
        _wait([dmat_copies[1], wmod_copies[2]])
        modulation(2)
        _run(ibfly(4))
        shift = ar_v[pl.ds(3 * D, D), :]
        ar_v[pl.ds(3 * D, D), :] = shift - _colmean(_fold(shift.reshape(9, 64, 128).sum(axis=0)))

        for a in range(4):
            rhs = jnp.concatenate([_as_bf16(bb_u[4 * a + b, pl.ds(256, 40), :]) for b in range(4)], axis=1)
            v = jnp.dot(_as_bf16(dmat_u[9, pl.ds(0, 32), pl.ds(0, 80)]), rhs, preferred_element_type=f32)
            for b in range(4):
                ee_v[pl.ds(64 * (4 * a + b), 64), :] = _tile(v, b)

        def phase_c(a, carry):
            acc = [0.0] * 4
            for b in range(4):
                t = 4 * a + b
                v = [jnp.dot(_as_bf16(dmat_u[5 + g]), _as_bf16(bb_u[4 * a + b, pl.ds(64 * g, 64), :]),
                             preferred_element_type=f32) for g in range(4)]
                for r in range(8):
                    if r % 2 == 0:
                        xres = [_as_bf16(io_u[t, pl.ds(32 * i + 4 * r, 8), :]).astype(f32) for i in range(9)]
                    z = [(q[16 * r:16 * r + 8], q[16 * r + 8:16 * r + 16]) for q in v]
                    y = _idft9(ee_v[_rows(64 * (4 * a + b) + 8 * r, 8), :], *z)
                    for i in range(9):
                        row = 64 * i + 8 * r
                        x2 = xres[i][8 * (r % 2):8 * (r % 2) + 8] + ar_v[pl.ds(2 * D + row, 8), :] * y[i]
                        x2_v[_rows(t * D + row, 8), :] = x2
                        acc[b] = acc[b] + x2
                    if r % 2 == 0:
                        tick(t_io, acc[b])
            mean = [_colmean(v) for v in acc]
            sq, lin, sq2 = [0.0] * 4, [0.0] * 4, [0.0] * 4

            def second(b, i):
                d = x2_v[_rows((4 * a + b) * D + 64 * i, 64), :] - mean[b]
                w = d * ar_v[pl.ds(4 * D + 64 * i, 64), :]
                ar_v[pl.ds(_HA + b * D + 64 * i, 64), :] = w
                sq[b], lin[b] = sq[b] + _fold(d * d), lin[b] + _fold(w)
                return sq[b], lin[b]

            chained([lambda b=b, i=i: second(b, i) for b in range(4) for i in range(9)], t_x2, lag=5)
            rstd = [jax.lax.rsqrt(_colmean(v) + 1e-5) for v in sq]
            mean = [_colmean(v) for v in lin]

            def third(b, i):
                h = ((ar_v[pl.ds(_HA + b * D + 64 * i, 64), :] - mean[b]) * rstd[b]
                     + ar_v[pl.ds(3 * D + 64 * i, 64), :])
                uu_v[pl.ds(b * D + 64 * i, 64), :] = h
                sq2[b] = sq2[b] + _fold(h * h)
                return sq2[b],

            chained([lambda b=b, i=i: third(b, i) for b in range(4) for i in range(9)], t_ar, lag=5)
            rstd = [jax.lax.rsqrt(_colmean(v) + 1e-5) for v in sq2]

            def operands(r):
                blk = [[uu_v[pl.ds(k * D + i * MB + 16 * r, 16), :] * rstd[k] for k in range(4)] for i in range(4)]
                for p1, t1 in enumerate(_A_TERMS):
                    x = _outer_operand(lambda i, k: blk[i][k], t1)
                    for p2, t2 in enumerate(_A_TERMS):
                        v = _inner_operand(x, t2)
                        ac_v[4 * (7 * p1 + p2) + a, pl.ds(16 * r, 16), :] = v.astype(bf16)
                    if p1 == 2:
                        late = v[:8]
                return late,

            chained([lambda r=r: operands(r) for r in range(MB // 16)], t_uu, lag=1)
            return carry

        jax.lax.fori_loop(0, 4, phase_c, 0)

        stage_wait(2)
        stage_wait(1)
        product = lambda par: deep_product(ac_v, lambda p, t: 4 * p + t, bcs[par], t_mm[par][0])
        own = lambda k: weight_units(2, bc0, [((), (_OUTER_ORDER[k],))]) if k < 7 else []
        ahead = weight_units(1, bc1, _SHARED)
        _run(own(0))
        for k, p1 in enumerate(_OUTER_ORDER):
            fence(bc0)
            products(product(0), [p1], _merge(own(k + 1) + (ahead[4 * k:4 * k + 4] if k < 6 else ahead[24:])))

        def mm1_step(c, par):
            products(product(par), range(7),
                     _merge(weight_units(1 - par, bcs[1 - par]), hidden_units(c - 1, 1 - par)))

        def mm1_pair(i, carry):
            c = 2 * i + 1

            @pl.when(i < 3)
            def _():
                _start(stage_copies(1, w1_hbm, 0, 4 * (c + 2)))

            @pl.when(i == 3)
            def _():
                _start(stage_copies(1, w2_hbm, 0, 0))

            copy(w2_hbm.bitcast(u32).at[pl.ds(1024, STAGE), _lanes(i)], st2.at[_rows(i * STAGE, STAGE)],
                 sem.at[_S_STAGE + 2]).start()
            stage_wait(0)
            mm1_step(c, 1)

            @pl.when(i < 3)
            def _():
                _start(stage_copies(0, w1_hbm, 0, 4 * (c + 3)))

            stage_wait(1)
            mm1_step(c + 1, 0)
            return carry

        jax.lax.fori_loop(0, 4, mm1_pair, 0)

    pl.run_scoped(
        first_half,
        pltpu.VMEM((4 * NP, MB, 128), bf16),
        pltpu.VMEM((D, 6 * D), bf16),
        pltpu.VMEM((10, 128, 128), bf16),
        pltpu.VMEM((64, 64, 128), u32),
        pltpu.VMEM((3, DF, S), bf16),
        pltpu.VMEM((32, 296, 128), f32),
        pltpu.VMEM((17, 592, 128), f32),
        pltpu.VMEM((17, 592, 128), f32),
        pltpu.VMEM((17, 592, 128), f32),
        pltpu.VMEM((17, 592, 128), bf16),
        pltpu.VMEM((16 * 64, 128), f32),
        pltpu.VMEM((592, 128), f32),
        pltpu.VMEM((1, D), bf16),
        pltpu.VMEM((F,), bf16),
        pltpu.VMEM((S,), bf16),
    )

    state["zero"] = zero_s[0]

    def quadrant(n, which, r8):
        def finish(i, j, v):
            row = i * MB + 8 * r8
            res = x2_v[_rows((4 * n + j) * D + row, 8), :]
            io_v[4 * n + j, pl.ds(row, 8), :] = (res + ar_v[pl.ds(5 * D + row, 8), :] * v).astype(bf16)

        m = lambda p1: _inner_block(lambda p: mm0[pl.ds(p * MB + 8 * r8, 8), :],
                                    lambda j: bias_v[_rows(8 * (36 + 4 * n + j), 8), :], p1)
        spot = lambda i, j: pl.ds((2 * i + j) * MB + 8 * r8, 8)
        yield t_mm[0]
        if which == 0:
            _finish_block(finish, _add2(m(1), m(3)), 1, 0)
        elif which == 1:
            m3 = m(2)
            _finish_block(finish, _add2(m3, m(4)), 0, 1)
            yield t_mm[0]
            part = _add2(_sub2(m(0), m(1)), m3)
            for i in range(2):
                for j in range(2):
                    uu_v[spot(i, j), :] = part[i][j]
        elif which == 2:
            part = _add2(m(0), m(3))
            yield t_mm[0]
            _finish_block(finish, _add2(_sub2(part, m(4)), m(6)), 0, 0)
        else:
            part = [[uu_v[spot(i, j), :] for j in range(2)] for i in range(2)]
            _finish_block(finish, _add2(part, m(5)), 1, 1)

    def quadrants(n, which):
        return [([[34], [34, 24], [20, 36], [24]][which], quadrant(n, which, r8)) for r8 in range(MB // 8)]

    def out_copies(n, which):
        bi, bj = ((1, 0), (0, 1), (0, 0), (1, 1))[which]
        rows = pl.ds(bi * (D // 2), D // 2)
        return [copy(io_v.at[4 * n + 2 * bj + j, rows], out_hbm.at[rows, _lanes(4 * n + 2 * bj + j)], sem.at[_S_OUT])
                for j in range(2)]

    def mm2_pair(n, carry):
        @pl.when(n < 3)
        def _():
            _start(stage_copies(1, w2_hbm, 0, 4 * n + 4))

        first = deep_product(uc_v, lambda p, t: p * NCH + t, bc1, mm1)

        @pl.when(n == 0)
        def _():
            stage_wait(2, 5)
            products(first, range(7), _merge(weight_units(2, bc0, depth=5), hidden_units(NCH - 1, 0)))

        @pl.when(n > 0)
        def _():
            stage_wait(0, 5)
            products(first, range(7), _merge(weight_units(0, bc0, depth=5), quadrants(n - 1, 3), fine=True))
            _start(out_copies(n - 1, 3))

        @pl.when(n < 3)
        def _():
            _start(stage_copies(0, w2_hbm, 1024, 4 * n + 4, 5))
            stage_wait(1)

        second = deep_product(uc_v, lambda p, t: p * NCH + 4 + t, bc0, mm0,
                              lambda p, r: mm1[pl.ds(p * MB + 16 * r, 16), :], depth=5,
                              hooks={7 * _OUTER_ORDER[5]: lambda: _start(out_copies(n, 0)),
                                     7 * _OUTER_ORDER[6]: lambda: _start(out_copies(n, 1))})
        ahead = weight_units(1, bc1)
        products(second, _OUTER_ORDER[:2], _merge(ahead[:11]))
        products(second, _OUTER_ORDER[2:5], _merge(ahead[11:25], quadrants(n, 0), fine=True))
        products(second, _OUTER_ORDER[5:6], _merge(ahead[25:28], quadrants(n, 1), fine=True))
        products(second, _OUTER_ORDER[6:], _merge(ahead[28:], quadrants(n, 2), fine=True))
        _start(out_copies(n, 2))
        return carry

    jax.lax.fori_loop(0, 4, mm2_pair, 0)
    _run(quadrants(3, 3))
    _start(out_copies(3, 3))
    _wait([cp for n in range(4) for which in range(4) for cp in out_copies(n, which)])


@jax.jit
def pallas_adaLN_cond__spectral_gfnet__mixer_token_mlp__prompt_kernel(
    A_x: jax.Array,
    A_w_r: jax.Array,
    A_w_i: jax.Array,
    B_x: jax.Array,
    B_w1: jax.Array,
    B_b1: jax.Array,
    B_w2: jax.Array,
    B_b2: jax.Array,
    c: jax.Array,
    w_mod: jax.Array,
):
    del B_x
    hbm = pl.BlockSpec(memory_space=pl.ANY)
    out = pl.pallas_call(
        _kernel,
        out_shape=jax.ShapeDtypeStruct((D, S), bf16),
        in_specs=[hbm] * 11,
        out_specs=hbm,
        scratch_shapes=[
            pltpu.SMEM((1,), jnp.int32),
            pltpu.VMEM((4 * STAGE + 8, 128), u32),
            pltpu.VMEM((4 * STAGE + 8, 128), u32),
            pltpu.VMEM((4 * STAGE + 8, 128), u32),
            pltpu.VMEM((NP * NCH, MB, 128), bf16),
            pltpu.VMEM((NP + 1, 640, 128), bf16),
            pltpu.VMEM((NP, 512, 128), bf16),
            pltpu.VMEM((NP * MB + 8, 128), f32),
            pltpu.VMEM((NP * MB + 8, 128), f32),
            pltpu.VMEM((16 * MB + 8, 128), f32),
            pltpu.VMEM((16 * D + 8, 128), f32),
            pltpu.VMEM((_AR_TICK + 8, 128), f32),
            pltpu.VMEM((8 * 52, 128), f32),
            pltpu.VMEM((25, D, 128), bf16),
            pltpu.SemaphoreType.DMA((_N_SEM,)),
        ],
        compiler_params=pltpu.CompilerParams(vmem_limit_bytes=126 * 1024 * 1024),
        name="adaln_gfnet_mixer",
    )(A_x.reshape(S, D).T, A_w_r.T, A_w_i.T, B_w1, B_b1, B_w2, B_b2, c, w_mod, _DMAT,
      np.zeros((1,), np.int32))
    return out.T.reshape(1, S, D)
```

```python
import numpy as np
import jax
import jax.numpy as jnp
import jax.experimental.pallas as pl
import jax.experimental.pallas.tpu as pltpu

S, D, F = 2048, 576, 4608
DF = D // 2 + 1
NP = 49
MB = D // 4
NCH = F // 512
NRG = (8, 8, 8, 8, 5)
STAGE = 1280

f32, u32, bf16 = jnp.float32, jnp.uint32, jnp.bfloat16


def _interleave(a, b):
    n = a.shape[0] // 8
    return np.stack([a.reshape(n, 8, -1), b.reshape(n, 8, -1)], axis=1).reshape(16 * n, -1)


def _constants():
    d0 = np.arange(64)
    fd = np.zeros((5, 128, 128))
    fi = np.zeros((5, 128, 128))
    scale = 1.0 / (S * D)
    for k1 in range(1, 5):
        k = np.array([k1 + 9 * m for m in range(32)] + [9 - k1 + 9 * m for m in range(32)])
        sg = np.array([1.0] * 32 + [-1.0] * 32)[:, None]
        ang = 2 * np.pi * np.outer(k, d0) / D
        c, s = np.cos(ang), np.sin(ang)
        q = np.sqrt(3.0) / 2 if k1 == 3 else 1.0
        re = _interleave(c.T, (-q * sg * s).T).T
        im = _interleave(-s.T, (-q * sg * c).T).T
        fd[k1 - 1] = _interleave(re, im)
        fi[k1 - 1] = 2 * scale * fd[k1 - 1].T
    ang = 2 * np.pi * np.outer(9 * np.arange(33), d0) / D
    re, im = np.zeros((40, 64)), np.zeros((40, 64))
    re[:33], im[:33] = np.cos(ang), -np.sin(ang)
    im[0] = im[32] = 0.0
    w = np.full((40, 1), 2.0)
    w[0] = w[32] = 1.0
    fd[4, :80, :64] = _interleave(re, im)
    fi[4, :64, :80] = scale * _interleave(w * re, w * im).T
    return np.concatenate([fd, fi]).astype(np.float32).astype(jnp.bfloat16)


_DMAT = _constants()

_C1, _C2, _C4 = (float(np.cos(2 * np.pi * k / 9)) for k in (1, 2, 4))
_S1, _S4, _S3 = float(np.sin(2 * np.pi / 9)), float(np.sin(8 * np.pi / 9)), float(np.sqrt(3.0) / 2)


def _dft9(x):
    e1, e2, e3, e4 = x[1] + x[8], x[2] + x[7], x[3] + x[6], x[4] + x[5]
    o1, o2, o3, o4 = x[1] - x[8], x[2] - x[7], x[3] - x[6], x[4] - x[5]
    t = x[0] - 0.5 * e3
    sm = e1 + e2 + e4
    p = x[0] + e3
    d1, d2 = e1 - e4, e2 - e4
    q1 = _C1 * d1 + _C2 * d2
    q2 = _C2 * d1 + _C4 * d2
    a, b, c = o1 + o2, o2 + o4, o1 - o4
    r1 = _S1 * a + _S4 * b
    r2 = _S1 * c + _S4 * a
    v = _S3 * o3
    return (p + sm, (t + q1, r1 + v), (t + q2, r2 - v), (p - 0.5 * sm, (o1 - o2) + o4),
            ((t - q1) - q2, (r2 - r1) + v))


def _idft9(a0, z1, z2, z3, z4):
    (a1, b1), (a2, b2), (a3, b3), (a4, b4) = z1, z2, z3, z4
    o3 = _S3 * ((b1 - b2) + b4)
    r1, r2 = b1 - b4, b2 + b4
    a, b, c = _S1 * r1 + _S4 * r2, _S4 * r1, _S1 * r2
    o1, o2, o4 = (a + c) + b3, (a + b) - b3, (b - c) + b3
    t = (a1 + a2) + a4
    q1, q2 = a1 - a4, a2 - a4
    d1 = _C1 * q1 + _C2 * q2
    d2 = _C2 * q1 + _C4 * q2
    p, sm = a0 + a3, a0 - 0.5 * a3
    e1, e2, e4 = sm + d1, sm + d2, (sm - d1) - d2
    e3 = p - 0.5 * t
    return [t + p, e1 + o1, e2 + o2, e3 + o3, e4 + o4, e4 - o4, e3 - o3, e2 - o2, e1 - o1]


def _radix4(x, sign):
    t0 = (x[0][0] + x[2][0], x[0][1] + x[2][1])
    t1 = (x[0][0] - x[2][0], x[0][1] - x[2][1])
    t2 = (x[1][0] + x[3][0], x[1][1] + x[3][1])
    t3 = (x[1][0] - x[3][0], x[1][1] - x[3][1])
    plus = (t1[0] - t3[1], t1[1] + t3[0])
    minus = (t1[0] + t3[1], t1[1] - t3[0])
    y1, y3 = (plus, minus) if sign > 0 else (minus, plus)
    return [(t0[0] + t2[0], t0[1] + t2[1]), y1, (t0[0] - t2[0], t0[1] - t2[1]), y3]


def _twiddle(z, n, sign):
    re, im = z
    if n == 0:
        return z
    if n == 4:
        return (-im, re) if sign > 0 else (im, -re)
    c, s = float(np.cos(np.pi * n / 8)), sign * float(np.sin(np.pi * n / 8))
    if n in (2, 6):
        if c * s > 0:
            return (c * (re - im), c * (im + re))
        return (c * (re + im), c * (im - re))
    return (c * re - s * im, c * im + s * re)


_A_TERMS = (((0, 0), 1, (1, 1)), ((1, 0), 1, (1, 1)), ((0, 0), 0, None), ((1, 1), 0, None),
            ((0, 0), 1, (0, 1)), ((1, 0), -1, (0, 0)), ((0, 1), -1, (1, 1)))
_B_TERMS = (((0, 0), 1, (1, 1)), ((0, 0), 0, None), ((0, 1), -1, (1, 1)), ((1, 0), -1, (0, 0)),
            ((1, 1), 0, None), ((0, 0), 1, (0, 1)), ((1, 0), 1, (1, 1)))


def _add2(x, y):
    return [[x[i][j] + y[i][j] for j in range(2)] for i in range(2)]


def _sub2(x, y):
    return [[x[i][j] - y[i][j] for j in range(2)] for i in range(2)]


def _outer_operand(ld, term):
    a, s, b = term
    x = [[ld(2 * a[0] + i, 2 * a[1] + j) for j in range(2)] for i in range(2)]
    if s == 0:
        return x
    y = [[ld(2 * b[0] + i, 2 * b[1] + j) for j in range(2)] for i in range(2)]
    return _add2(x, y) if s > 0 else _sub2(x, y)


def _inner_operand(x, term):
    a, s, b = term
    if s == 0:
        return x[a[0]][a[1]]
    return x[a[0]][a[1]] + x[b[0]][b[1]] if s > 0 else x[a[0]][a[1]] - x[b[0]][b[1]]


def _inner_result(m):
    m1, m4, m2 = m(0), m(3), m(1)
    c21, c22, c11 = m2 + m4, m1 - m2, m1 + m4
    m5, m3 = m(4), m(2)
    c12, c11, c22 = m3 + m5, c11 - m5, c22 + m3
    return [[c11 + m(6), c12], [c21, c22 + m(5)]]


def _inner_block(load, bias, p1):
    def m(p2):
        v = load(7 * p1 + p2)
        if p1 in (3, 2) and p2 in (3, 2):
            v = v + bias(2 * (3 - p1) + (3 - p2))
        return v
    return _inner_result(m)


def _finish_block(finish, c, bi, bj):
    for i in range(2):
        for j in range(2):
            finish(2 * bi + i, 2 * bj + j, c[i][j])


def _recombine(load, bias, finish, tag):
    yield tag
    m2 = _inner_block(load, bias, 1)
    yield tag
    m4 = _inner_block(load, bias, 3)
    _finish_block(finish, _add2(m2, m4), 1, 0)
    yield tag
    m1 = _inner_block(load, bias, 0)
    c22, c11 = _sub2(m1, m2), _add2(m1, m4)
    yield tag
    m5 = _inner_block(load, bias, 4)
    c11 = _sub2(c11, m5)
    yield tag
    m3 = _inner_block(load, bias, 2)
    c22 = _add2(c22, m3)
    _finish_block(finish, _add2(m3, m5), 0, 1)
    yield tag
    _finish_block(finish, _add2(c11, _inner_block(load, bias, 6)), 0, 0)
    yield tag
    _finish_block(finish, _add2(c22, _inner_block(load, bias, 5)), 1, 1)


def _gelu2(x):
    c0 = float(np.sqrt(2.0 / np.pi))
    return x + x * jnp.tanh(x * (c0 + (c0 * 0.044715) * (x * x)))


def _merge(*streams, fine=False):
    streams = [us for us in streams if us]

    def whole():
        order = sorted(((i + 0.5) / len(us), k, i) for k, us in enumerate(streams) for i in range(len(us)))
        for _, k, i in order:
            costs, gen = streams[k][i]
            yield from zip(gen, costs + [None])

    def pieces():
        order = []
        for k, us in enumerate(streams):
            costs = np.array([c for u in us for c in u[0]])
            order += [(float(q) / costs.sum(), k, int(c)) for q, c in zip(np.cumsum(costs) - 0.5 * costs, costs)]
        gens = [(tag for u in us for tag in u[1]) for us in streams]
        heads = [next(g) for g in gens]
        for _, k, c in sorted(order):
            yield heads[k], c
            heads[k] = next(gens[k], None)

    return sum(sum(u[0]) for us in streams for u in us), (pieces() if fine else whole())


def _run(units):
    for _, gen in units:
        for _ in gen:
            pass


def _pack(a, b):
    return jnp.concatenate([a, b], axis=0).astype(bf16)


def _colmean(v):
    return jnp.sum(v, axis=0, keepdims=True) * (1.0 / D)


def _fold(v):
    return v.reshape(8, 8, 128).sum(axis=0)


def _rows(start, n):
    return pl.ds(start if isinstance(start, int) else pl.multiple_of(start, 8), n)


def _lanes(tile):
    return pl.ds(128 * tile if isinstance(tile, int) else pl.multiple_of(128 * tile, 128), 128)


def _as_bf16(v):
    return pltpu.bitcast(v, bf16)


def _tile(v, t):
    return v[:, 128 * t:128 * t + 128]


def _start(copies):
    for cp in copies:
        cp.start()


def _wait(copies):
    for cp in copies:
        cp.wait()


def _operand_costs(terms, groups, unpack):
    out, have = [], set()
    for keep, group in groups:
        have, n = have & set(keep), 0
        for p1 in group:
            a, s, b = terms[p1]
            need = {(2 * q[0] + i, 2 * q[1] + j) for q in ((a, b) if s else (a,)) for i in range(2) for j in range(2)}
            n += unpack * len(need - have) + (8 if s else 0) + 17
            have |= need
        out.append(n)
    return out


def _quad(*blocks):
    return [(2 * a + i, 2 * b + j) for a, b in blocks for i in range(2) for j in range(2)]


_SINGLE = [((), (p,)) for p in range(7)]
_SHARED = [((), (1,)), (_quad((0, 0), (1, 1)), (5,)), (_quad((0, 0), (1, 1), (0, 1)), (4, 2)),
           (_quad((0, 0), (1, 1)), (0, 6)), (_quad((0, 0), (1, 1), (1, 0)), (3,))]
_OUTER_ORDER = (1, 3, 0, 4, 2, 6, 5)

_HA = 6 * D
_AR_TICK = _HA + 4 * D
_S_SMALL, _S_X, _S_MOD, _S_DMAT, _S_WF, _S_STAGE, _S_OUT, _N_SEM = 0, 1, 5, 8, 10, 13, 16, 17


def _kernel(x_hbm, wr_hbm, wi_hbm, w1_hbm, b1_hbm, w2_hbm, b2_hbm, c_hbm, wmod_hbm, dmat_hbm, zero_hbm,
            out_hbm,
            zero_s, st0, st1, st2, uc_v, bc0, bc1, mm0, mm1, uu_v, x2_v, ar_v, bias_v, io_v, sem):
    copy = pltpu.make_async_copy
    state = {}

    def tick(target, val):
        ref, idx, row = target
        where = idx + (_rows(row + state["zero"], 8), pl.ds(0, 128))
        if ref.dtype != bf16:
            ref[where] = pltpu.bitcast(val, ref.dtype)
        elif ref.shape[-2] % 2:
            ref[where] = val.astype(bf16)
        else:
            ref.bitcast(u32)[where] = pltpu.bitcast(val, u32)

    def fence(ref):
        tick((ref, (ref.shape[0] - 1,), 0), jnp.zeros((8, 128), f32))

    def paced(main, points, side, lead):
        total, gen = side
        pending, done = next(gen, None), 0
        for _ in range(lead):
            if pending is not None:
                pending, done = next(gen, None), done + pending[1]
        for pt, v in enumerate(main, 1):
            seen = []
            while pending is not None and done * points < pt * total:
                if not any(pending[0] is t for t in seen):
                    seen.append(pending[0])
                    tick(pending[0], v)
                pending, done = next(gen, None), done + pending[1]
        assert pending is None

    def chained(units, target, lag):
        late = []
        for k, unit in enumerate(units):
            if k >= lag:
                for v in late[k - lag]:
                    tick(target, v)
            late.append(unit())

    t_uu, t_ar = (uu_v, (), 16 * MB), (ar_v, (), _AR_TICK)
    t_mm = [(mm0, (), NP * MB), (mm1, (), NP * MB)]
    t_st = [(ref, (), 4 * STAGE) for ref in (st0, st1, st2)]
    bcs = (bc0, bc1)

    def stage_copies(par, src, row, tile, depth=4):
        return [copy(src.bitcast(u32).at[pl.ds(row, 256 * depth), _lanes(tile + j)],
                     t_st[par][0].at[pl.ds(j * STAGE, 256 * depth)], sem.at[_S_STAGE + par]) for j in range(4)]

    def stage_wait(par, depth=4):
        for j in range(4):
            tile = t_st[par][0].at[pl.ds(j * STAGE, 256 * depth)]
            copy(tile, tile, sem.at[_S_STAGE + par]).wait()

    def operand_unit(target, raw, load, terms, groups, put):
        cache = {}
        for keep, group in groups:
            yield target
            cache = {k: v for k, v in cache.items() if k in keep}

            def ld(i, j):
                if (i, j) not in cache:
                    cache[i, j] = load(i, j)
                return cache[i, j]

            for p1 in group:
                t1 = terms[p1]
                x = _outer_operand(ld, t1)
                for p2, t2 in enumerate(terms):
                    if raw is not None and t1[1] == 0 and t2[1] == 0:
                        put(7 * p1 + p2, raw(2 * t1[0][0] + t2[0][0], 2 * t1[0][1] + t2[0][1]))
                    else:
                        put(7 * p1 + p2, _inner_operand(x, t2).astype(bf16))

    def weight_units(par, bc, groups=_SINGLE, depth=4):
        target = t_st[par]

        def unit(ru):
            def raw(k, j):
                return target[0][pl.ds(j * STAGE + 256 * (ru // 8) + 64 * k + 8 * (ru % 8), 8), :]

            def put(p, v):
                if v.dtype == u32:
                    bc.bitcast(u32)[p, pl.ds(8 * ru, 8), :] = v
                else:
                    bc[p, pl.ds(16 * ru, 16), :] = v
            return operand_unit(target, raw, lambda k, j: _as_bf16(raw(k, j)).astype(f32), _B_TERMS, groups, put)
        return [(_operand_costs(_B_TERMS, groups, 2), unit(ru)) for ru in range(8 * depth)]

    def hidden_units(c, par):
        target, t_hid = t_mm[par], (t_uu, t_ar)
        spot = lambda i, j, r, row, n: pl.ds(_HA * (r % 2) + (4 * i + j) * MB + row, n)

        def first(r8):
            def finish(i, j, v):
                t_hid[r8 // 2 % 2][0][spot(i, j, r8 // 2, 8 * r8, 8), :] = _gelu2(v)
            return _recombine(lambda p: target[0][pl.ds(p * MB + 8 * r8, 8), :],
                              lambda j: bias_v[_rows(8 * (4 * c + j), 8), :], finish, target)

        def second(r):
            def put(p, v):
                uc_v[p * NCH + c, pl.ds(16 * r, 16), :] = v
            return operand_unit(t_hid[r % 2], None, lambda i, j: t_hid[r % 2][0][spot(i, j, r, 16 * r, 16), :],
                                _A_TERMS, _SINGLE, put)

        units, cost = [], [8, 38, 16, 12, 42, 36, 36]
        for r in range(MB // 16 + 1):
            if r < MB // 16:
                units += [(cost, first(2 * r)), (cost, first(2 * r + 1))]
            if r > 0:
                units += [(_operand_costs(_A_TERMS, _SINGLE, 0), second(r - 1))]
        return units

    def products(product, outer, side):
        main = (v for p1 in outer for p2 in range(7) for v in product(7 * p1 + p2))
        points = 7 * len(outer) * (MB // 16)
        paced(main, points - max(2, points // 40), side, lead=2 if len(outer) == 7 else 1)

    def deep_product(lhs_ref, slot, bc, dst, init=None, depth=4, hooks=None):
        lhs_u, bc_u = lhs_ref.bitcast(u32), bc.bitcast(u32)

        def product(p):
            lhs = jnp.concatenate([_as_bf16(lhs_u[slot(p, t)]) for t in range(depth)], axis=1)
            v = jnp.dot(lhs, _as_bf16(bc_u[p, pl.ds(0, 64 * depth), :]), preferred_element_type=f32)
            if hooks and p in hooks:
                hooks[p]()
            for r in range(MB // 16):
                blk = v[16 * r:16 * r + 16]
                if init is not None:
                    blk = blk + init(p, r)
                dst[pl.ds(p * MB + 16 * r, 16), :] = blk
                yield blk[:8] if lhs_ref is uc_v else blk[8:]
        return product

    def first_half(ac_v, wmod_v, dmat_v, gmat_u, wf_v, wt_v, uv_v, yv_v, pv_v, bb_v, ee_v, sa_v, c_v, b1_v, b2_v):
        small_copies = [copy(c_hbm, c_v, sem.at[_S_SMALL]), copy(zero_hbm, zero_s, sem.at[_S_SMALL]),
                        copy(b1_hbm, b1_v, sem.at[_S_SMALL]), copy(b2_hbm, b2_v, sem.at[_S_SMALL])]
        x_copies = lambda a: [copy(x_hbm.at[:, _lanes(a + 4 * b)], io_v.at[a + 4 * b], sem.at[_S_X + a])
                              for b in range(4)]
        mod_tiles = ((0, 4), (4, 9), (9, 27))
        wmod_copies = [copy(wmod_hbm.at[:, pl.ds(128 * t0, 128 * (t1 - t0))],
                            wmod_v.at[:, pl.ds(128 * t0, 128 * (t1 - t0))], sem.at[_S_MOD + h])
                       for h, (t0, t1) in enumerate(mod_tiles)]
        dmat_copies = [copy(dmat_hbm.at[pl.ds(5 * h, 5)], dmat_v.at[pl.ds(5 * h, 5)], sem.at[_S_DMAT + h])
                       for h in range(2)]
        wf_rows = ((0, 96), (96, 96), (192, DF - 192))
        wf_copies = [[copy(src.at[pl.ds(*rows)], wf_v.at[a, pl.ds(*rows)], sem.at[_S_WF + h])
                      for a, src in enumerate((wr_hbm, wi_hbm))] for h, rows in enumerate(wf_rows)]

        _start(small_copies + [wmod_copies[1]] + x_copies(0) + [dmat_copies[0]] + x_copies(1) + x_copies(2)
               + x_copies(3) + [wmod_copies[0]] + sum(wf_copies, []) + [dmat_copies[1], wmod_copies[2]])
        _wait(small_copies)
        state["zero"] = zero_s[0]
        s0 = jax.lax.broadcasted_iota(jnp.int32, (16, 128), 0)
        j0 = jax.lax.broadcasted_iota(jnp.int32, (16, 128), 1)
        j0 = 8 * (j0 & 15) + (j0 >> 4)
        phasor = lambda n, period: (jnp.cos(n.astype(f32) * (-2 * np.pi / period)),
                                    jnp.sin(n.astype(f32) * (-2 * np.pi / period)))
        cmul = lambda x, y: (x[0] * y[0] - x[1] * y[1], x[0] * y[1] + x[1] * y[0])
        base, rot, down = phasor((s0 * j0) & 127, 128), phasor(s0, S), phasor(j0[:1] & 7, 8)

        def generate(i, carry):
            for r in range(4):
                g, rows = carry[:2], _rows(8 * (4 * i + r), 8)
                for j1 in range(16):
                    for q in range(2):
                        v = pltpu.bitcast(g[q].astype(bf16), u32)
                        gmat_u[2 * j1 + q, rows, :] = pltpu.roll(v, j1, 1) if j1 else v
                    g = cmul(g, carry[2:])
                carry = cmul(carry[:2], down) + cmul(carry[2:], (float(np.cos(np.pi / 64)), float(-np.sin(np.pi / 64))))
            return carry

        jax.lax.fori_loop(0, 2, generate, base + rot)
        bb_u = bb_v.bitcast(u32)

        cv = c_v[...].astype(f32)
        sc = jnp.broadcast_to(cv * jax.nn.sigmoid(cv), (16, D)).astype(bf16)
        b1 = b1_v[...].astype(f32).reshape(1, F)
        for t in range(36):
            bias_v[pl.ds(8 * t, 8), :] = jnp.broadcast_to(_tile(b1, t), (8, 128))
        b2 = 2.0 * b2_v[...].astype(f32).reshape(1, S)
        for t in range(16):
            bias_v[pl.ds(8 * (36 + t), 8), :] = jnp.broadcast_to(_tile(b2, t), (8, 128))

        def modulation(h):
            t0, t1 = mod_tiles[h]
            m = jnp.dot(sc, wmod_v[:, pl.ds(128 * t0, 128 * (t1 - t0))], preferred_element_type=f32)[:8]
            for t in range(t0, t1):
                col = 128 * t + jax.lax.broadcasted_iota(jnp.int32, (8, 128), 1)
                v = _tile(m, t - t0)
                scale = ((col >= D) & (col < 2 * D)) | ((col >= 4 * D) & (col < 5 * D))
                v = jnp.where(scale, 1.0 + v, v)
                v = jnp.where(col >= 5 * D, 0.5 * v, v)
                ar_v[pl.ds(128 * t, 128), :] = jnp.concatenate([v] * 16, axis=0).T

        wmod_copies[1].wait()
        modulation(1)
        dmat_u, io_u = dmat_v.bitcast(u32), io_v.bitcast(u32)
        t_io, t_uv, t_x2 = (io_v, (24,), 0), (uv_v, (16,), 0), (x2_v, (), 16 * D)

        def dft9_tiles(h, r, held):
            z = _dft9(h)
            out = [(128 * g + 16 * r, _pack(*z[g + 1])) for g in range(4)]
            if r % 2:
                out.append((512 + 8 * (r - 1), _pack(held.pop(), z[0])))
            else:
                held.append(z[0])
            return out

        def put(slot, tiles):
            for row, v in tiles:
                io_v[slot, pl.ds(row, 16), :] = v

        def channel_dft(g, slots):
            n = 64 if g < 4 else 32
            lhs = _as_bf16(dmat_u[g] if g < 4 else dmat_u[4, pl.ds(0, 40), pl.ds(0, 64)])
            rhs = jnp.concatenate([_as_bf16(io_u[t, pl.ds(64 * g, n), :]) for t in slots], axis=1)
            return jnp.dot(lhs, rhs, preferred_element_type=f32)

        def spectrum(a, rstd, ordered=True):
            slots = [16 + 4 * (a % 2) + b for b in range(4)]
            nxt = channel_dft(0, slots)
            for g in range(5):
                yield
                v, nxt = nxt, (channel_dft(g + 1, slots) if g < 4 else None)
                for half in range(2):
                    yield
                    for r in range(4 * half, min(4 * half + 4, NRG[g])):
                        z = [(_tile(v[16 * r:16 * r + 8], b) * rstd[b], _tile(v[16 * r + 8:16 * r + 16], b) * rstd[b])
                             for b in range(4)]
                        for c, y in enumerate(_radix4(z, -1)):
                            uv_v[4 * a + c, pl.ds(128 * g + 16 * r, 16), :] = jnp.concatenate(y, axis=0)
                        if ordered and r % 2:
                            tick(t_io, y[1])

        def token_mean(t):
            total = jnp.dot(jnp.ones((16, D), bf16), _as_bf16(io_u[t]), preferred_element_type=f32)
            return total[:8] * (1.0 / D)

        def phase_a(a, rstd_prev):
            _wait(x_copies(a))
            behind = iter(()) if rstd_prev is None else spectrum(a - 1, rstd_prev)
            mean = [token_mean(a)]
            next(behind, None)
            sq, queue = [0.0] * 4, []
            for b in range(4):
                held, slot = [], 16 + 4 * (a % 2) + b
                if b:
                    tick(t_ar, sq[b - 1])
                if b < 3:
                    mean.append(token_mean(a + 4 * b + 4))
                for r in range(8):
                    if r % 2 == 0:
                        xp = [io_u[a + 4 * b, pl.ds(32 * i + 4 * r, 8), :] for i in range(9)]
                        for emit in queue:
                            emit()
                        queue = []
                        next(behind, None)
                        xp = [_as_bf16(v).astype(f32) for v in xp]
                    h = []
                    for i in range(9):
                        d = xp[i][8 * (r % 2):8 * (r % 2) + 8] - mean[b]
                        sq[b] = sq[b] + d * d
                        h.append(d * ar_v[pl.ds(D + 64 * i + 8 * r, 8), :])
                    tiles = dft9_tiles(h, r, held)
                    if r % 2 == 0:
                        put(slot, tiles)
                    else:
                        queue.append(lambda slot=slot, tiles=tiles, q=sq[b]: (put(slot, tiles), tick(t_io, q)))
            for _ in behind:
                pass
            for emit in queue:
                emit()
            return tuple(jnp.broadcast_to(jax.lax.rsqrt(_colmean(q) + 1e-5), (8, 128)) for q in sq)

        rstd_first = phase_a(0, None)
        dmat_copies[0].wait()
        rstd_last = jax.lax.fori_loop(1, 4, phase_a, rstd_first)

        wmod_copies[0].wait()
        modulation(0)
        for _ in spectrum(3, rstd_last, ordered=False):
            pass
        for q in range(32):
            gmat_u[32 + q] = pltpu.bitcast(_as_bf16(gmat_u[q]).T, u32)
        held = []
        for r in range(8):
            put(16, dft9_tiles([float(S) * ar_v[pl.ds(64 * i + 8 * r, 8), :] for i in range(9)], r, held))
        for g in range(5):
            v = channel_dft(g, [16])
            first = jax.lax.broadcasted_iota(jnp.int32, v.shape, 1) == 0
            sa_v[pl.ds(128 * g, 16 * NRG[g]), :] = jnp.where(first, v, 0.0)


        def pair_at(ref, j, row):
            return ref[j, pl.ds(row, 8), :], ref[j, pl.ds(row + 8, 8), :]

        t_yv, t_pv = (yv_v, (16,), 0), [t_uv, (pv_v, (16,), 0)]

        def butterflies(g, r):
            row = 128 * g + 16 * r
            for c in range(4):
                yield t_uv
                z = [_twiddle(pair_at(uv_v, 4 * a + c, row), a * c, -1) for a in range(4)]
                for e, y in enumerate(_radix4(z, -1)):
                    bb_v[c + 4 * e, pl.ds(row, 16), :] = _pack(*y)

        def token_dft(g, inverse):
            n = NRG[g]
            for j1 in range(16):
                rhs = jnp.concatenate([_as_bf16(gmat_u[32 * inverse + 2 * j1 + i]) for i in range(2)], axis=1)
                v = jnp.dot(_as_bf16(bb_u[j1, pl.ds(64 * g, 8 * n), :]), rhs, preferred_element_type=f32)
                for r in range(n):
                    top, bot = v[16 * r:16 * r + 8], v[16 * r + 8:16 * r + 16]
                    if inverse:
                        re, im = _tile(top, 0) + _tile(bot, 1), _tile(bot, 0) - _tile(top, 1)
                    else:
                        re, im = _tile(top, 0) - _tile(bot, 1), _tile(bot, 0) + _tile(top, 1)
                    dst = t_pv[g % 2][0] if inverse else yv_v
                    dst[j1, pl.ds(128 * g + 16 * r, 16), :] = jnp.concatenate([re, im], axis=0)
                    yield re

        lane = jax.lax.broadcasted_iota(jnp.int32, (8, 128), 1)

        def filt(a, j1, g, r):
            if g < 4:
                first = (g + 1 if r < 4 else 8 - g) + 72 * (r % 4)
                return wt_v[16 * a + j1, pl.ds(first, 8, stride=9), :]
            if r < 4:
                return wt_v[16 * a + j1, pl.ds(72 * r, 8, stride=9), :]
            return wt_v[16 * a + j1, pl.ds(288, 8), :]

        def filtering(g, j1):
            for r in range(NRG[g]):
                if r % 4 == 0:
                    yield t_yv
                row = 128 * g + 16 * r
                yr, yi = pair_at(yv_v, j1, row)
                if j1 == 0:
                    yr, yi = yr + sa_v[pl.ds(row, 8), :], yi + sa_v[pl.ds(row + 8, 8), :]
                wr, wi = filt(0, j1, g, r), filt(1, j1, g, r)
                bb_v[j1, pl.ds(row, 16), :] = _pack(yr * wr - yi * wi, yr * wi + yi * wr)

        def inverse_butterflies(g, r):
            row = 128 * g + 16 * r
            mid = [[None] * 4 for _ in range(4)]
            for c in range(4):
                yield t_pv[g % 2]
                for a, y in enumerate(_radix4([pair_at(t_pv[g % 2][0], c + 4 * e, row) for e in range(4)], 1)):
                    mid[a][c] = _twiddle(y, a * c, 1)
            for a in range(4):
                for b, y in enumerate(_radix4(mid[a], 1)):
                    bb_v[a + 4 * b, pl.ds(row, 16), :] = _pack(*y)

        bfly = lambda g: [([20, 36, 28, 36], butterflies(g, r)) for r in range(NRG[g])] if g < 5 else []
        filts = lambda g: [([28, 7 * (NRG[g] - 4)], filtering(g, j1)) for j1 in range(16)] if g < 5 else []
        ibfly = lambda g: [([16, 32, 24, 112], inverse_butterflies(g, r)) for r in range(NRG[g])] if g >= 0 else []

        masks = [(lane & (1 << i)) != 0 for i in range(4)]

        def regroup(tiles):
            t = [pltpu.roll(v, b, 1) if b else v for b, v in enumerate(tiles)]
            t = [t[-i % 16] for i in range(16)]
            for i in range(4):
                t = [jnp.where(masks[i], t[(j - (1 << i)) % 16], t[j]) for j in range(16)]
            return t

        def regroup_unit(a, r):
            yield t_wf
            if r < 18:
                tiles = [pltpu.bitcast(wf_v[a, pl.ds(16 * r, 16), pl.ds(128 * b, 128)], u32) for b in range(16)]
                for j1, v in enumerate(regroup(tiles)):
                    wt_v[16 * a + j1, pl.ds(16 * r, 16), :] = _as_bf16(v).astype(f32)
            else:
                last = jnp.broadcast_to(wf_v[a, pl.ds(288, 1), :].astype(f32), (8, S))
                for j1, v in enumerate(regroup([_tile(last, b) for b in range(16)])):
                    wt_v[16 * a + j1, pl.ds(288, 8), :] = v

        t_wf = (wf_v, (2,), 0)
        regroups = lambda h: [([112], regroup_unit(a, r)) for r in range(6 * h, 6 * h + 6 + h // 2) for a in range(2)]

        _run(bfly(0))
        for g in range(5):
            if 1 <= g <= 3:
                _wait(wf_copies[g - 1])
            fence(bb_v)
            paced(token_dft(g, 0), 16 * NRG[g] - 24,
                  _merge(bfly(g + 1) or filts(0), regroups(g - 1) if 1 <= g <= 3 else [], fine=True), lead=1)
        _start(stage_copies(2, w1_hbm, 0, 0) + stage_copies(1, w1_hbm, 0, 4) + stage_copies(0, w1_hbm, 0, 8))
        for g in range(5):
            paced(token_dft(g, 1), 16 * NRG[g] - 8, _merge(filts(g + 1), ibfly(g - 1)), lead=1)
        _wait([dmat_copies[1], wmod_copies[2]])
        modulation(2)
        _run(ibfly(4))
        shift = ar_v[pl.ds(3 * D, D), :]
        ar_v[pl.ds(3 * D, D), :] = shift - _colmean(_fold(shift.reshape(9, 64, 128).sum(axis=0)))

        for a in range(4):
            rhs = jnp.concatenate([_as_bf16(bb_u[4 * a + b, pl.ds(256, 40), :]) for b in range(4)], axis=1)
            v = jnp.dot(_as_bf16(dmat_u[9, pl.ds(0, 32), pl.ds(0, 80)]), rhs, preferred_element_type=f32)
            for b in range(4):
                ee_v[pl.ds(64 * (4 * a + b), 64), :] = _tile(v, b)

        def phase_c(a, carry):
            acc = [0.0] * 4
            for b in range(4):
                t = 4 * a + b
                v = [jnp.dot(_as_bf16(dmat_u[5 + g]), _as_bf16(bb_u[4 * a + b, pl.ds(64 * g, 64), :]),
                             preferred_element_type=f32) for g in range(4)]
                for r in range(8):
                    if r % 2 == 0:
                        xres = [_as_bf16(io_u[t, pl.ds(32 * i + 4 * r, 8), :]).astype(f32) for i in range(9)]
                    z = [(q[16 * r:16 * r + 8], q[16 * r + 8:16 * r + 16]) for q in v]
                    y = _idft9(ee_v[_rows(64 * (4 * a + b) + 8 * r, 8), :], *z)
                    for i in range(9):
                        row = 64 * i + 8 * r
                        x2 = xres[i][8 * (r % 2):8 * (r % 2) + 8] + ar_v[pl.ds(2 * D + row, 8), :] * y[i]
                        x2_v[_rows(t * D + row, 8), :] = x2
                        acc[b] = acc[b] + x2
                    if r % 2 == 0:
                        tick(t_io, acc[b])
            mean = [_colmean(v) for v in acc]
            sq, lin, sq2 = [0.0] * 4, [0.0] * 4, [0.0] * 4

            def second(b, i):
                d = x2_v[_rows((4 * a + b) * D + 64 * i, 64), :] - mean[b]
                w = d * ar_v[pl.ds(4 * D + 64 * i, 64), :]
                ar_v[pl.ds(_HA + b * D + 64 * i, 64), :] = w
                sq[b], lin[b] = sq[b] + _fold(d * d), lin[b] + _fold(w)
                return sq[b], lin[b]

            chained([lambda b=b, i=i: second(b, i) for b in range(4) for i in range(9)], t_x2, lag=5)
            rstd = [jax.lax.rsqrt(_colmean(v) + 1e-5) for v in sq]
            mean = [_colmean(v) for v in lin]

            def third(b, i):
                h = ((ar_v[pl.ds(_HA + b * D + 64 * i, 64), :] - mean[b]) * rstd[b]
                     + ar_v[pl.ds(3 * D + 64 * i, 64), :])
                uu_v[pl.ds(b * D + 64 * i, 64), :] = h
                sq2[b] = sq2[b] + _fold(h * h)
                return sq2[b],

            chained([lambda b=b, i=i: third(b, i) for b in range(4) for i in range(9)], t_ar, lag=5)
            rstd = [jax.lax.rsqrt(_colmean(v) + 1e-5) for v in sq2]

            def operands(r):
                blk = [[uu_v[pl.ds(k * D + i * MB + 16 * r, 16), :] * rstd[k] for k in range(4)] for i in range(4)]
                for p1, t1 in enumerate(_A_TERMS):
                    x = _outer_operand(lambda i, k: blk[i][k], t1)
                    for p2, t2 in enumerate(_A_TERMS):
                        v = _inner_operand(x, t2)
                        ac_v[4 * (7 * p1 + p2) + a, pl.ds(16 * r, 16), :] = v.astype(bf16)
                    if p1 == 2:
                        late = v[:8]
                return late,

            chained([lambda r=r: operands(r) for r in range(MB // 16)], t_uu, lag=1)
            return carry

        jax.lax.fori_loop(0, 4, phase_c, 0)

        stage_wait(2)
        stage_wait(1)
        product = lambda par: deep_product(ac_v, lambda p, t: 4 * p + t, bcs[par], t_mm[par][0])
        own = lambda k: weight_units(2, bc0, [((), (_OUTER_ORDER[k],))]) if k < 7 else []
        ahead = weight_units(1, bc1, _SHARED)
        _run(own(0))
        for k, p1 in enumerate(_OUTER_ORDER):
            fence(bc0)
            products(product(0), [p1], _merge(own(k + 1) + (ahead[4 * k:4 * k + 4] if k < 6 else ahead[24:])))

        def mm1_step(c, par):
            products(product(par), range(7),
                     _merge(weight_units(1 - par, bcs[1 - par]), hidden_units(c - 1, 1 - par)))

        def mm1_pair(i, carry):
            c = 2 * i + 1

            @pl.when(i < 3)
            def _():
                _start(stage_copies(1, w1_hbm, 0, 4 * (c + 2)))

            @pl.when(i == 3)
            def _():
                _start(stage_copies(1, w2_hbm, 0, 0))

            copy(w2_hbm.bitcast(u32).at[pl.ds(1024, STAGE), _lanes(i)], st2.at[_rows(i * STAGE, STAGE)],
                 sem.at[_S_STAGE + 2]).start()
            stage_wait(0)
            mm1_step(c, 1)

            @pl.when(i < 3)
            def _():
                _start(stage_copies(0, w1_hbm, 0, 4 * (c + 3)))

            stage_wait(1)
            mm1_step(c + 1, 0)
            return carry

        jax.lax.fori_loop(0, 4, mm1_pair, 0)

    pl.run_scoped(
        first_half,
        pltpu.VMEM((4 * NP, MB, 128), bf16),
        pltpu.VMEM((D, 6 * D), bf16),
        pltpu.VMEM((10, 128, 128), bf16),
        pltpu.VMEM((64, 64, 128), u32),
        pltpu.VMEM((3, DF, S), bf16),
        pltpu.VMEM((32, 296, 128), f32),
        pltpu.VMEM((17, 592, 128), f32),
        pltpu.VMEM((17, 592, 128), f32),
        pltpu.VMEM((17, 592, 128), f32),
        pltpu.VMEM((17, 592, 128), bf16),
        pltpu.VMEM((16 * 64, 128), f32),
        pltpu.VMEM((592, 128), f32),
        pltpu.VMEM((1, D), bf16),
        pltpu.VMEM((F,), bf16),
        pltpu.VMEM((S,), bf16),
    )

    state["zero"] = zero_s[0]

    def quadrant(n, which, r8):
        def finish(i, j, v):
            row = i * MB + 8 * r8
            res = x2_v[_rows((4 * n + j) * D + row, 8), :]
            io_v[4 * n + j, pl.ds(row, 8), :] = (res + ar_v[pl.ds(5 * D + row, 8), :] * v).astype(bf16)

        m = lambda p1: _inner_block(lambda p: mm0[pl.ds(p * MB + 8 * r8, 8), :],
                                    lambda j: bias_v[_rows(8 * (36 + 4 * n + j), 8), :], p1)
        spot = lambda i, j: pl.ds((2 * i + j) * MB + 8 * r8, 8)
        yield t_mm[0]
        if which == 0:
            _finish_block(finish, _add2(m(1), m(3)), 1, 0)
        elif which == 1:
            m3 = m(2)
            _finish_block(finish, _add2(m3, m(4)), 0, 1)
            yield t_mm[0]
            part = _add2(_sub2(m(0), m(1)), m3)
            for i in range(2):
                for j in range(2):
                    uu_v[spot(i, j), :] = part[i][j]
        elif which == 2:
            part = _add2(m(0), m(3))
            yield t_mm[0]
            _finish_block(finish, _add2(_sub2(part, m(4)), m(6)), 0, 0)
        else:
            part = [[uu_v[spot(i, j), :] for j in range(2)] for i in range(2)]
            _finish_block(finish, _add2(part, m(5)), 1, 1)

    def quadrants(n, which):
        return [([[34], [34, 24], [20, 36], [24]][which], quadrant(n, which, r8)) for r8 in range(MB // 8)]

    def out_copies(n, which):
        bi, bj = ((1, 0), (0, 1), (0, 0), (1, 1))[which]
        rows = pl.ds(bi * (D // 2), D // 2)
        return [copy(io_v.at[4 * n + 2 * bj + j, rows], out_hbm.at[rows, _lanes(4 * n + 2 * bj + j)], sem.at[_S_OUT])
                for j in range(2)]

    def mm2_pair(n, carry):
        @pl.when(n < 3)
        def _():
            _start(stage_copies(1, w2_hbm, 0, 4 * n + 4))

        first = deep_product(uc_v, lambda p, t: p * NCH + t, bc1, mm1)

        @pl.when(n == 0)
        def _():
            stage_wait(2, 5)
            products(first, range(7), _merge(weight_units(2, bc0, depth=5), hidden_units(NCH - 1, 0)))

        @pl.when(n > 0)
        def _():
            stage_wait(0, 5)
            products(first, range(7), _merge(weight_units(0, bc0, depth=5), quadrants(n - 1, 3), fine=True))
            _start(out_copies(n - 1, 3))

        @pl.when(n < 3)
        def _():
            _start(stage_copies(0, w2_hbm, 1024, 4 * n + 4, 5))
            stage_wait(1)

        second = deep_product(uc_v, lambda p, t: p * NCH + 4 + t, bc0, mm0,
                              lambda p, r: mm1[pl.ds(p * MB + 16 * r, 16), :], depth=5,
                              hooks={7 * _OUTER_ORDER[5]: lambda: _start(out_copies(n, 0)),
                                     7 * _OUTER_ORDER[6]: lambda: _start(out_copies(n, 1))})
        ahead = weight_units(1, bc1)
        products(second, _OUTER_ORDER[:2], _merge(ahead[:11]))
        products(second, _OUTER_ORDER[2:5], _merge(ahead[11:25], quadrants(n, 0), fine=True))
        products(second, _OUTER_ORDER[5:6], _merge(ahead[25:28], quadrants(n, 1), fine=True))
        products(second, _OUTER_ORDER[6:], _merge(ahead[28:], quadrants(n, 2), fine=True))
        _start(out_copies(n, 2))
        return carry

    jax.lax.fori_loop(0, 4, mm2_pair, 0)
    _run(quadrants(3, 3))
    _start(out_copies(3, 3))
    _wait([cp for n in range(4) for which in range(4) for cp in out_copies(n, which)])


@jax.jit
def pallas_adaLN_cond__spectral_gfnet__mixer_token_mlp__prompt_kernel(
    A_x: jax.Array,
    A_w_r: jax.Array,
    A_w_i: jax.Array,
    B_x: jax.Array,
    B_w1: jax.Array,
    B_b1: jax.Array,
    B_w2: jax.Array,
    B_b2: jax.Array,
    c: jax.Array,
    w_mod: jax.Array,
):
    del B_x
    hbm = pl.BlockSpec(memory_space=pl.ANY)
    out = pl.pallas_call(
        _kernel,
        out_shape=jax.ShapeDtypeStruct((D, S), bf16),
        in_specs=[hbm] * 11,
        out_specs=hbm,
        scratch_shapes=[
            pltpu.SMEM((1,), jnp.int32),
            pltpu.VMEM((4 * STAGE + 8, 128), u32),
            pltpu.VMEM((4 * STAGE + 8, 128), u32),
            pltpu.VMEM((4 * STAGE + 8, 128), u32),
            pltpu.VMEM((NP * NCH, MB, 128), bf16),
            pltpu.VMEM((NP + 1, 640, 128), bf16),
            pltpu.VMEM((NP, 512, 128), bf16),
            pltpu.VMEM((NP * MB + 8, 128), f32),
            pltpu.VMEM((NP * MB + 8, 128), f32),
            pltpu.VMEM((16 * MB + 8, 128), f32),
            pltpu.VMEM((16 * D + 8, 128), f32),
            pltpu.VMEM((_AR_TICK + 8, 128), f32),
            pltpu.VMEM((8 * 52, 128), f32),
            pltpu.VMEM((25, D, 128), bf16),
            pltpu.SemaphoreType.DMA((_N_SEM,)),
        ],
        compiler_params=pltpu.CompilerParams(vmem_limit_bytes=126 * 1024 * 1024),
        name="adaln_gfnet_mixer",
    )(A_x.reshape(S, D).T, A_w_r.T, A_w_i.T, B_w1, B_b1, B_w2, B_b2, c, w_mod, _DMAT,
      np.zeros((1,), np.int32))
    return out.T.reshape(1, S, D)
```
